```python
import os as _os
_os.environ.setdefault('JAX_PLATFORMS', 'cpu')
import jax
import jax.numpy as jnp

def _softmax(x, axis=-1):
    return jax.nn.softmax(x, axis=axis)

def _gelu(x):
    return jax.nn.gelu(x, approximate=True)

def _silu(x):
    return jax.nn.silu(x)

def _sigmoid(x):
    return jax.nn.sigmoid(x)

def _layernorm(x, axis=-1, eps=1e-05):
    m = jnp.mean(x, axis=axis, keepdims=True)
    v = jnp.var(x, axis=axis, keepdims=True)
    return (x - m) / jnp.sqrt(v + eps)

def _scatter_add(tgt, idx, src, axis=0):
    return tgt.at[idx].add(src)

def _segment_sum(src, seg, n):
    return jax.ops.segment_sum(src, seg, n)

class _Rng:

    def __init__(self, key):
        self._k = key

    def _next(self):
        self._k, sub = jax.random.split(self._k)
        return sub

    def normal(self, shape):
        return jax.random.normal(self._next(), shape, dtype=jnp.bfloat16)

    def randint(self, lo, hi, shape):
        return jax.random.randint(self._next(), shape, lo, hi, dtype=jnp.int32)

    def uniform(self, shape, lo=0.0, hi=1.0):
        return jax.random.uniform(self._next(), shape, jnp.bfloat16, lo, hi)

    def permutation(self, n):
        return jax.random.permutation(self._next(), n)
kernel_name = 'standalone__autoregressive_conv_wavenet__speech'

def setup_inputs():
    _rng = _Rng(jax.random.key(int.from_bytes(__import__("os").urandom(4), "little")))
    _w = lambda a: (lambda t: t.astype(jnp.bfloat16) if jnp.issubdtype(t.dtype, jnp.floating) else t)(jnp.asarray(a))
    B, T, D, K = (2, 4000, 512, 31)
    return {'x': _w((lambda *s: _rng.normal(s) * 0.05)(B, T, D)), 'w': _w((lambda *s: _rng.normal(s) * 0.05)(K, D, 2 * D)), 'w_o': _w((lambda *s: _rng.normal(s) * 0.05)(D, D))}

def reference(x, w, w_o):
    B, T, D = x.shape
    K = w.shape[0]
    dil = 2
    pad = (K - 1) * dil
    xp = jnp.pad(x, ((0, 0), (pad, 0), (0, 0)))
    h = jnp.einsum('btc,cd->btd', xp[:, pad:pad + T, :], w[0])
    for i in range(1, K):
        off = pad - i * dil
        h = h + jnp.einsum('btc,cd->btd', xp[:, off:off + T, :], w[i])
    f = h[..., :D].copy()
    g = h[..., D:].copy()
    z = jnp.tanh(f) * _sigmoid(g)
    return z @ w_o
```

```python
import functools
import jax
import jax.numpy as jnp
import numpy as np
from jax.experimental import pallas as pl
from jax.experimental.pallas import tpu as pltpu

NF = 64
HOP = 34
NPROD = 95


def _fwd_coef(q, nm):
    m = 4 * np.arange(nm) + q
    c = np.zeros((16, nm))
    c[0] = 1.0
    th8 = -2 * np.pi * 8 * m / NF
    c[1] = np.sin(th8) if q == 2 else np.cos(th8)
    for kp in range(1, 8):
        th = -2 * np.pi * kp * m / NF
        c[2 * kp] = np.cos(th)
        c[2 * kp + 1] = np.sin(th)
    return c


def _inv_coef(q):
    ns = [n for n in range(30, NF) if n % 4 == q]
    c = np.zeros((9, 16))
    for r, n in enumerate(ns):
        sgn = (-1.0) ** (n // 4)
        c[r, 0] = 1.0 / NF
        c[r, 1] = (2.0, np.sqrt(2.0), -2.0, -np.sqrt(2.0))[q] * sgn / NF
        for kp in range(1, 8):
            th = 2 * np.pi * kp * n / NF
            c[r, 2 * kp] = 2.0 / NF * np.cos(th)
            c[r, 2 * kp + 1] = -2.0 / NF * np.sin(th)
    return c, ns


def _snap(c):
    c = np.where(np.abs(c) < 1e-12, 0.0, c)
    return c


def _constants(taps):
    lw, lx, ly = [], [], []
    for q in range(4):
        cw = _fwd_coef(q, 8)
        for mp in range(8):
            if 4 * mp + q >= taps:
                cw[:, mp] = 0.0
        lw.append(np.kron(_snap(cw), np.eye(16)))
        lx.append(np.kron(_snap(_fwd_coef(q, 16)), np.eye(8)))
        ly.append(np.kron(_snap(_inv_coef(q)[0]), np.eye(8)))
    f = lambda a: np.asarray(np.stack(a), dtype=np.float32).astype(jnp.bfloat16)
    return f(lw), f(lx), f(ly)


def _fwd_butterfly(T):
    ops = []

    def cplx(re, im):
        ops.extend([re + im, re, im])

    u0, u1 = T[0][0] + T[2][0], T[0][0] - T[2][0]
    v0, v1n = T[1][0] + T[3][0], T[3][0] - T[1][0]
    ops.append(u0 + v0)
    ops.append(u0 - v0)
    cplx(u1, v1n)
    a0, a1, b2, a3 = T[0][1], T[1][1], T[2][1], T[3][1]
    s, d = a1 + a3, a3 - a1
    cplx(a0 + s, b2 + d)
    cplx(a0 - s, d - b2)
    for kp in range(1, 8):
        t = [(T[q][2 * kp], T[q][2 * kp + 1]) for q in range(4)]
        u0 = (t[0][0] + t[2][0], t[0][1] + t[2][1])
        u1 = (t[0][0] - t[2][0], t[0][1] - t[2][1])
        v0 = (t[1][0] + t[3][0], t[1][1] + t[3][1])
        v1 = (t[1][0] - t[3][0], t[1][1] - t[3][1])
        cplx(u0[0] + v0[0], u0[1] + v0[1])
        cplx(u1[0] + v1[1], u1[1] - v1[0])
        cplx(u0[0] - v0[0], u0[1] - v0[1])
        cplx(u1[0] - v1[1], u1[1] + v1[0])
    return ops


def _inv_butterfly(P):
    def cplx(i):
        p1, p2, p3 = P(i), P(i + 1), P(i + 2)
        return (p2 - p3, (p1 - p2) - p3)

    A = [[None] * 16 for _ in range(4)]
    y0, y32 = P(0), P(1)
    y16, y8, y24 = cplx(2), cplx(5), cplx(8)
    e, o = y0 + y32, y0 - y32
    r2, i2 = y16[0] + y16[0], y16[1] + y16[1]
    A[0][0], A[2][0] = e + r2, e - r2
    A[1][0], A[3][0] = o - i2, o + i2
    A[0][1] = y8[0] + y24[0]
    A[2][1] = y8[1] - y24[1]
    dr, si = y8[0] - y24[0], y24[1] + y8[1]
    A[1][1], A[3][1] = dr - si, dr + si
    for kp in range(1, 8):
        b = 11 + 12 * (kp - 1)
        Y = [cplx(b + 3 * j) for j in range(4)]
        e0 = (Y[0][0] + Y[2][0], Y[0][1] + Y[2][1])
        e1 = (Y[0][0] - Y[2][0], Y[0][1] - Y[2][1])
        f0 = (Y[1][0] + Y[3][0], Y[1][1] + Y[3][1])
        f1 = (Y[1][0] - Y[3][0], Y[1][1] - Y[3][1])
        A[0][2 * kp], A[0][2 * kp + 1] = e0[0] + f0[0], e0[1] + f0[1]
        A[2][2 * kp], A[2][2 * kp + 1] = e0[0] - f0[0], e0[1] - f0[1]
        A[1][2 * kp], A[1][2 * kp + 1] = e1[0] - f1[1], e1[1] + f1[0]
        A[3][2 * kp], A[3][2 * kp + 1] = e1[0] + f1[1], e1[1] - f1[0]
    return A


def _pack(v):
    return pltpu.bitcast(v.astype(jnp.bfloat16), jnp.uint32)


def _unpack(v):
    return pltpu.bitcast(v, jnp.bfloat16)


def make(UW=2, UC=19, UY=1, UX=1, RC=400):
    B, T, D, K = 2, 4000, 512, 31
    NB = 60
    PITCH = NB * HOP
    TH = T // 2
    NG = B * NB // 8
    OFF = 32
    XROWS = 4128
    NCT = D // 128

    def kernel(x_hbm, w_hbm, wo_ref, lw_ref, lx_ref, ly_ref, o_hbm,
               xs, wbuf, xh, wh, yh, tf, ost, xsem, wsem, osem):
        xs_bf = xs.bitcast(jnp.bfloat16)

        def x_copy(b, ct):
            return pltpu.make_async_copy(
                x_hbm.at[b, :, pl.ds(ct * 128, 128)],
                xs_bf.at[ct, pl.ds(2 * (OFF + b * PITCH), T), :],
                xsem.at[b * NCT + ct])

        def col_of(j):
            return (j % 2) * D + (j // 2) * 128

        def w_copy(j, slot):
            return pltpu.make_async_copy(
                w_hbm.at[:, :, pl.ds(pl.multiple_of(col_of(j), 128), 128)],
                wbuf.at[slot], wsem.at[slot])

        w_copy(0, 0).start()
        for b in range(B):
            for ct in range(NCT):
                x_copy(b, ct).start()

        for ct in range(NCT):
            xs[ct, 0:OFF, :] = jnp.zeros((OFF, 128), jnp.uint32)
            for b in range(B):
                lo = OFF + b * PITCH + TH
                hi = OFF + (b + 1) * PITCH if b + 1 < B else XROWS
                xs[ct, lo:hi, :] = jnp.zeros((hi - lo, 128), jnp.uint32)

        def w_stage(slot):
            wv = wbuf.bitcast(jnp.uint32)

            def body(cg, _):
                r0 = pl.multiple_of(cg * 8, 8)
                Tq = []
                for q in range(4):
                    rows = [wv[slot, min(4 * m + q, K - 1), pl.ds(r0, 8), :] for m in range(8)]
                    rhs = _unpack(jnp.concatenate(rows, axis=0))
                    res = jnp.dot(lw_ref[q], rhs, preferred_element_type=jnp.float32)
                    Tq.append([res[16 * j:16 * j + 16] for j in range(16)])
                ops = _fwd_butterfly(Tq)
                for p in range(NPROD):
                    wh[p, pl.ds(r0, 8), :] = _pack(ops[p])
                return 0
            jax.lax.fori_loop(0, D // 16, body, 0, unroll=UW)

        def x_stage():
            def body(i, _):
                g = i // NCT
                ct = i % NCT
                base = g * (8 * HOP) + (OFF - 30)
                xf = [_unpack(xs[ct, pl.ds(base + m, 8, stride=HOP), :]).astype(jnp.float32)
                      for m in range(NF)]
                Tq = []
                for q in range(4):
                    halves = []
                    for h in range(2):
                        rhs = jnp.concatenate([xf[4 * m + q][8 * h:8 * h + 8] for m in range(16)], axis=0)
                        halves.append(jnp.dot(lx_ref[q], rhs.astype(jnp.bfloat16),
                                              preferred_element_type=jnp.float32))
                    Tq.append([jnp.concatenate([halves[0][8 * j:8 * j + 8], halves[1][8 * j:8 * j + 8]], axis=0)
                               for j in range(16)])
                ops = _fwd_butterfly(Tq)
                r0 = pl.multiple_of(g * 8, 8)
                c0 = pl.multiple_of(ct * 128, 128)
                for p in range(NPROD):
                    xh[p, pl.ds(r0, 8), pl.ds(c0, 128)] = _pack(ops[p])
                return 0
            jax.lax.fori_loop(0, NG * NCT, body, 0, unroll=UX)

        def c_stage():
            def body(p, _):
                yh[p] = jnp.dot(_unpack(xh[p]), _unpack(wh[p]), preferred_element_type=jnp.float32)
                return 0
            jax.lax.fori_loop(0, NPROD, body, 0, unroll=UC)

        def y_stage(is_g, ct):
            def body(g, _):
                r0 = pl.multiple_of(g * 16, 16)
                A = _inv_butterfly(lambda p: yh[p, pl.ds(r0, 16), :])
                hs = {}
                for q in range(4):
                    ns = _inv_coef(q)[1]
                    halves = []
                    for h in range(2):
                        rhs = jnp.concatenate([A[q][j][8 * h:8 * h + 8] for j in range(16)], axis=0)
                        halves.append(jnp.dot(ly_ref[q], rhs.astype(jnp.bfloat16),
                                              preferred_element_type=jnp.float32))
                    for r, n in enumerate(ns):
                        hs[n - 30] = jnp.concatenate(
                            [halves[0][8 * r:8 * r + 8], halves[1][8 * r:8 * r + 8]], axis=0)
                if is_g:
                    zb = g * (8 * HOP)
                    for t in range(HOP):
                        z = tf[t, pl.ds(r0, 16), :] * jax.nn.sigmoid(hs[t])
                        xs[ct, pl.ds(zb + t, 8, stride=HOP), :] = _pack(z)
                else:
                    for t in range(HOP):
                        tf[t, pl.ds(r0, 16), :] = jnp.tanh(hs[t])
                return 0
            jax.lax.fori_loop(0, NG, body, 0, unroll=UY)

        w_copy(0, 0).wait()
        w_copy(1, 1).start()
        w_stage(0)
        for b in range(B):
            for ct in range(NCT):
                x_copy(b, ct).wait()
        x_stage()
        c_stage()
        y_stage(False, 0)

        def pair(jj, _):
            w_copy(2 * jj + 1, 1).wait()

            @pl.when(jj + 1 < NCT)
            def _():
                w_copy(2 * jj + 2, 0).start()
            w_stage(1)
            c_stage()
            y_stage(True, jj)

            @pl.when(jj + 1 < NCT)
            def _():
                w_copy(2 * jj + 2, 0).wait()
                w_copy(2 * jj + 3, 1).start()
                w_stage(0)
                c_stage()
                y_stage(False, 0)
            return 0
        jax.lax.fori_loop(0, NCT, pair, 0)

        nch = TH // RC

        def o_copy(b, i, slot):
            return pltpu.make_async_copy(ost.at[slot], o_hbm.at[b, pl.ds(2 * i * RC, 2 * RC), :], osem.at[slot])

        idx = 0
        for b in range(B):
            for i in range(nch):
                slot = idx % 2
                if idx >= 2:
                    pb, pi = divmod(idx - 2, nch)
                    o_copy(pb, pi, slot).wait()
                r0 = b * PITCH + i * RC
                z = jnp.concatenate([_unpack(xs[ct, r0:r0 + RC, :]) for ct in range(NCT)], axis=1)
                ost[slot] = jnp.dot(z, wo_ref[...], preferred_element_type=jnp.float32).astype(jnp.bfloat16)
                o_copy(b, i, slot).start()
                idx += 1
        for k in (idx - 2, idx - 1):
            pb, pi = divmod(k, nch)
            o_copy(pb, pi, k % 2).wait()

    def f(x, w, w_o):
        lw, lx, ly = _constants(K)
        vm = pl.BlockSpec(memory_space=pltpu.VMEM)
        anyspec = pl.BlockSpec(memory_space=pl.ANY)
        return pl.pallas_call(
            kernel,
            in_specs=[anyspec, anyspec, vm, vm, vm, vm],
            out_specs=anyspec,
            out_shape=jax.ShapeDtypeStruct((B, T, D), jnp.bfloat16),
            scratch_shapes=[
                pltpu.VMEM((NCT, XROWS, 128), jnp.uint32),
                pltpu.VMEM((2, K, D, 128), jnp.bfloat16),
                pltpu.VMEM((NPROD, NG * 8, D), jnp.uint32),
                pltpu.VMEM((NPROD, D // 2, 128), jnp.uint32),
                pltpu.VMEM((NPROD, NG * 16, 128), jnp.float32),
                pltpu.VMEM((HOP, NG * 16, 128), jnp.float32),
                pltpu.VMEM((2, 2 * RC, D), jnp.bfloat16),
                pltpu.SemaphoreType.DMA((B * NCT,)),
                pltpu.SemaphoreType.DMA((2,)),
                pltpu.SemaphoreType.DMA((2,)),
            ],
            compiler_params=pltpu.CompilerParams(vmem_limit_bytes=100 * 2**20),
        )(x, w, w_o, lw, lx, ly)
    return jax.jit(f)


_kernel = make()


@jax.jit
def pallas_standalone__autoregressive_conv_wavenet__speech_kernel(x, w, w_o):
    return _kernel(x, w, w_o)
```

```python
import functools
import jax
import jax.numpy as jnp
import numpy as np
from jax.experimental import pallas as pl
from jax.experimental.pallas import tpu as pltpu

NF = 64
HOP = 34
NPROD = 95


def _fwd_coef(q, nm):
    m = 4 * np.arange(nm) + q
    c = np.zeros((16, nm))
    c[0] = 1.0
    th8 = -2 * np.pi * 8 * m / NF
    c[1] = np.sin(th8) if q == 2 else np.cos(th8)
    for kp in range(1, 8):
        th = -2 * np.pi * kp * m / NF
        c[2 * kp] = np.cos(th)
        c[2 * kp + 1] = np.sin(th)
    return c


def _inv_coef(q):
    ns = [n for n in range(30, NF) if n % 4 == q]
    c = np.zeros((9, 16))
    for r, n in enumerate(ns):
        sgn = (-1.0) ** (n // 4)
        c[r, 0] = 1.0 / NF
        c[r, 1] = (2.0, np.sqrt(2.0), -2.0, -np.sqrt(2.0))[q] * sgn / NF
        for kp in range(1, 8):
            th = 2 * np.pi * kp * n / NF
            c[r, 2 * kp] = 2.0 / NF * np.cos(th)
            c[r, 2 * kp + 1] = -2.0 / NF * np.sin(th)
    return c, ns


def _snap(c):
    c = np.where(np.abs(c) < 1e-12, 0.0, c)
    return c


def _pair_cols(a):
    r, c = a.shape
    return a.reshape(r, c // 16, 2, 8).transpose(0, 1, 3, 2).reshape(r, c)


def _to_words(a):
    b = np.asarray(a, dtype=np.float32).astype(jnp.bfloat16).view(np.uint16).astype(np.uint32)
    return b[..., 0::2, :] | (b[..., 1::2, :] << 16)


def _constants(taps):
    lw, lx, ly = [], [], []
    for q in range(4):
        cw = _fwd_coef(q, 8)
        for mp in range(8):
            if 4 * mp + q >= taps:
                cw[:, mp] = 0.0
        lw.append(np.kron(_snap(cw), np.eye(16)))
        lx.append(_pair_cols(np.kron(_snap(_fwd_coef(q, 16)), np.eye(8))))
        ly.append(_pair_cols(np.kron(_snap(np.pad(_inv_coef(q)[0], ((0, 1), (0, 0)))), np.eye(8))))
    return _to_words(np.stack(lw)), _to_words(np.stack(lx)), _to_words(np.stack(ly))


def _fwd_butterfly(T, is_w):
    ops = []

    def cplx(re, im):
        ops.extend([re, im - re, re + im] if is_w else [re + im, re, im])

    u0, u1 = T[0][0] + T[2][0], T[0][0] - T[2][0]
    v0, v1n = T[1][0] + T[3][0], T[3][0] - T[1][0]
    ops.append(u0 + v0)
    ops.append(u0 - v0)
    cplx(u1, v1n)
    a0, a1, b2, a3 = T[0][1], T[1][1], T[2][1], T[3][1]
    s, d = a1 + a3, a3 - a1
    cplx(a0 + s, b2 + d)
    cplx(a0 - s, d - b2)
    for kp in range(1, 8):
        t = [(T[q][2 * kp], T[q][2 * kp + 1]) for q in range(4)]
        u0 = (t[0][0] + t[2][0], t[0][1] + t[2][1])
        u1 = (t[0][0] - t[2][0], t[0][1] - t[2][1])
        v0 = (t[1][0] + t[3][0], t[1][1] + t[3][1])
        v1 = (t[1][0] - t[3][0], t[1][1] - t[3][1])
        cplx(u0[0] + v0[0], u0[1] + v0[1])
        cplx(u1[0] + v1[1], u1[1] - v1[0])
        cplx(u0[0] - v0[0], u0[1] - v0[1])
        cplx(u1[0] - v1[1], u1[1] + v1[0])
    return ops


def _inv_butterfly(P):
    def cplx(b):
        return (P(2 * b), P(2 * b + 1))

    A = [[None] * 16 for _ in range(4)]
    y0, y32 = P(0), P(1)
    y16, y8, y24 = cplx(1), cplx(2), cplx(3)
    e, o = y0 + y32, y0 - y32
    r2, i2 = y16[0] + y16[0], y16[1] + y16[1]
    A[0][0], A[2][0] = e + r2, e - r2
    A[1][0], A[3][0] = o - i2, o + i2
    A[0][1] = y8[0] + y24[0]
    A[2][1] = y8[1] - y24[1]
    dr, si = y8[0] - y24[0], y24[1] + y8[1]
    A[1][1], A[3][1] = dr - si, dr + si
    for kp in range(1, 8):
        b = 4 + 4 * (kp - 1)
        Y = [cplx(b + j) for j in range(4)]
        e0 = (Y[0][0] + Y[2][0], Y[0][1] + Y[2][1])
        e1 = (Y[0][0] - Y[2][0], Y[0][1] - Y[2][1])
        f0 = (Y[1][0] + Y[3][0], Y[1][1] + Y[3][1])
        f1 = (Y[1][0] - Y[3][0], Y[1][1] - Y[3][1])
        A[0][2 * kp], A[0][2 * kp + 1] = e0[0] + f0[0], e0[1] + f0[1]
        A[2][2 * kp], A[2][2 * kp + 1] = e0[0] - f0[0], e0[1] - f0[1]
        A[1][2 * kp], A[1][2 * kp + 1] = e1[0] - f1[1], e1[1] + f1[0]
        A[3][2 * kp], A[3][2 * kp + 1] = e1[0] + f1[1], e1[1] - f1[0]
    return A


def _pack2(a, b):
    return pltpu.pack_elementwise([a, b], packed_dtype=jnp.bfloat16)


def _half(v, i):
    return pltpu.unpack_elementwise(v, index=i, packed_dtype=jnp.bfloat16, unpacked_dtype=jnp.float32)


def _rhs_from_pairs(vs):
    return _unpack(jnp.concatenate([_pack2(vs[2 * u], vs[2 * u + 1]) for u in range(8)], axis=0))


def _unpack(v):
    return pltpu.bitcast(v, jnp.bfloat16)


import contextlib
def make(UW=2, UC=6, UY=1, UX=1, RC=400, scopes=False):
    sc = (lambda n: jax.named_scope(n)) if scopes else (lambda n: contextlib.nullcontext())
    B, T, D, K = 2, 4000, 512, 31
    NB = 60
    PITCH = NB * HOP
    TH = T // 2
    NG = B * NB // 8
    OFF = 32
    XROWS = 4128
    NCT = D // 128

    def kernel(x_hbm, w_hbm, wo_ref, lw_ref, lx_ref, ly_ref, o_hbm,
               xs, wbuf, xh, wh, yh, tf, ost, xsem, wsem, osem):
        xs_bf = xs.bitcast(jnp.bfloat16)

        def x_copy(b, ct):
            return pltpu.make_async_copy(
                x_hbm.at[b, :, pl.ds(pl.multiple_of(ct * 128, 128), 128)],
                xs_bf.at[ct, pl.ds(2 * (OFF + b * PITCH), T), :],
                xsem.at[b, ct])

        def col_of(j):
            return (j % 2) * D + (j // 2) * 128

        def w_copy(j, slot):
            return pltpu.make_async_copy(
                w_hbm.at[:, :, pl.ds(pl.multiple_of(col_of(j), 128), 128)],
                wbuf.at[slot], wsem.at[slot])

        for ct in range(NCT):
            for b in range(B):
                x_copy(b, ct).start()
        w_copy(0, 0).start()

        for ct in range(NCT):
            xs[ct, 0:OFF, :] = jnp.zeros((OFF, 128), jnp.uint32)
            for b in range(B):
                lo = OFF + b * PITCH + TH
                hi = OFF + (b + 1) * PITCH if b + 1 < B else XROWS
                xs[ct, lo:hi, :] = jnp.zeros((hi - lo, 128), jnp.uint32)

        def w_stage(slot):
            wv = wbuf.bitcast(jnp.uint32)

            def body(cg, _):
                r0 = pl.multiple_of(cg * 8, 8)
                Tq = []
                for q in range(4):
                    rows = [wv[slot, min(4 * m + q, K - 1), pl.ds(r0, 8), :] for m in range(8)]
                    rhs = _unpack(jnp.concatenate(rows, axis=0))
                    res = jnp.dot(_unpack(lw_ref[q]), rhs, preferred_element_type=jnp.float32)
                    Tq.append([res[16 * j:16 * j + 16] for j in range(16)])
                ops = _fwd_butterfly(Tq, True)
                r1 = pl.multiple_of(cg * 16, 16)
                for p in range(NPROD):
                    wh[p, pl.ds(r1, 16), :] = ops[p].astype(jnp.bfloat16)
                return 0
            with sc('W'):
                jax.lax.fori_loop(0, D // 16, body, 0, unroll=UW)

        def x_stage(ct):
            def body(g, _):
                base = g * (8 * HOP) + (OFF - 30)
                Tq = []
                for q in range(4):
                    xw = [xs[ct, pl.ds(base + 4 * m + q, 8, stride=HOP), :] for m in range(16)]
                    halves = []
                    for h in range(2):
                        rhs = _rhs_from_pairs([_half(v, h) for v in xw])
                        halves.append(jnp.dot(_unpack(lx_ref[q]), rhs, preferred_element_type=jnp.float32))
                    Tq.append([jnp.concatenate([halves[0][8 * j:8 * j + 8], halves[1][8 * j:8 * j + 8]], axis=0)
                               for j in range(16)])
                ops = _fwd_butterfly(Tq, False)
                r0 = pl.multiple_of(g * 16, 16)
                for p in range(NPROD):
                    xh[p, ct, pl.ds(r0, 16), :] = ops[p].astype(jnp.bfloat16)
                return 0
            with sc('X'):
                jax.lax.fori_loop(0, NG, body, 0, unroll=UX)

        def c_stage():
            def prod(p):
                lhs = jnp.concatenate([xh[p, ct] for ct in range(NCT)], axis=1)
                return jnp.dot(lhs, wh[p], preferred_element_type=jnp.float32)

            def cbin(b):
                p = 3 * b - 1
                k1 = prod(p)
                yh[2 * b] = k1 - prod(p + 2)
                yh[2 * b + 1] = k1 + prod(p + 1)

            def body(b, _):
                cbin(b)
                return 0
            with sc('C'):
                yh[0] = prod(0)
                yh[1] = prod(1)
                cbin(1)
                jax.lax.fori_loop(2, NF // 2, body, 0, unroll=UC)

        def y_stage(is_g, ct):
            def body(g, _):
                r0 = pl.multiple_of(g * 16, 16)
                A = _inv_butterfly(lambda p: yh[p, pl.ds(r0, 16), :])
                hs = {}
                for q in range(4):
                    ns = _inv_coef(q)[1]
                    halves = []
                    for h in range(2):
                        rhs = _rhs_from_pairs([A[q][j][8 * h:8 * h + 8] for j in range(16)])
                        halves.append(jnp.dot(_unpack(ly_ref[q]), rhs, preferred_element_type=jnp.float32))
                    for r, n in enumerate(ns):
                        hs[n - 30] = jnp.concatenate(
                            [halves[0][8 * r:8 * r + 8], halves[1][8 * r:8 * r + 8]], axis=0)
                if is_g:
                    zb = g * (8 * HOP)
                    for t in range(HOP):
                        th = jnp.tanh(0.5 * hs[t])
                        hf = tf[t, pl.ds(r0, 16), :]
                        z = hf + hf * th
                        xs[ct, pl.ds(zb + t, 8, stride=HOP), :] = _pack2(z[0:8], z[8:16])
                else:
                    for t in range(HOP):
                        tf[t, pl.ds(r0, 16), :] = 0.5 * jnp.tanh(hs[t])
                return 0
            with sc('Yg' if is_g else 'Yf'):
                jax.lax.fori_loop(0, NG, body, 0, unroll=UY)

        def x_all(ct, _):
            for b in range(B):
                x_copy(b, ct).wait()
            x_stage(ct)
            return 0
        jax.lax.fori_loop(0, NCT, x_all, 0)
        w_copy(0, 0).wait()
        w_copy(1, 1).start()
        w_stage(0)
        c_stage()
        y_stage(False, 0)

        def pair(jj, _):
            w_copy(2 * jj + 1, 1).wait()

            @pl.when(jj + 1 < NCT)
            def _():
                w_copy(2 * jj + 2, 0).start()
            w_stage(1)
            c_stage()
            y_stage(True, jj)

            @pl.when(jj + 1 < NCT)
            def _():
                w_copy(2 * jj + 2, 0).wait()
                w_copy(2 * jj + 3, 1).start()
                w_stage(0)
                c_stage()
                y_stage(False, 0)
            return 0
        jax.lax.fori_loop(0, NCT, pair, 0)

        nch = TH // RC

        def o_copy(i, slot):
            b = i // nch
            r = pl.multiple_of((i % nch) * (2 * RC), 16)
            return pltpu.make_async_copy(ost.at[slot], o_hbm.at[b, pl.ds(r, 2 * RC), :], osem.at[slot])

        def o_body(i, _):
            slot = i % 2

            @pl.when(i >= 2)
            def _():
                o_copy(i - 2, slot).wait()
            r0 = pl.multiple_of((i // nch) * PITCH + (i % nch) * RC, 8)
            z = jnp.concatenate([_unpack(xs[ct, pl.ds(r0, RC), :]) for ct in range(NCT)], axis=1)
            ost[slot] = jnp.dot(z, wo_ref[...], preferred_element_type=jnp.float32).astype(jnp.bfloat16)
            o_copy(i, slot).start()
            return 0
        with sc('O'):
            jax.lax.fori_loop(0, B * nch, o_body, 0)
        for k in (B * nch - 2, B * nch - 1):
            o_copy(k, k % 2).wait()

    def f(x, w, w_o):
        lw, lx, ly = _constants(K)
        vm = pl.BlockSpec(memory_space=pltpu.VMEM)
        anyspec = pl.BlockSpec(memory_space=pl.ANY)
        return pl.pallas_call(
            kernel,
            in_specs=[anyspec, anyspec, vm, vm, vm, vm],
            out_specs=anyspec,
            out_shape=jax.ShapeDtypeStruct((B, T, D), jnp.bfloat16),
            scratch_shapes=[
                pltpu.VMEM((NCT, XROWS, 128), jnp.uint32),
                pltpu.VMEM((2, K, D, 128), jnp.bfloat16),
                pltpu.VMEM((NPROD, NCT, NG * 16, 128), jnp.bfloat16),
                pltpu.VMEM((NPROD, D, 128), jnp.bfloat16),
                pltpu.VMEM((NF, NG * 16, 128), jnp.float32),
                pltpu.VMEM((HOP, NG * 16, 128), jnp.float32),
                pltpu.VMEM((2, 2 * RC, D), jnp.bfloat16),
                pltpu.SemaphoreType.DMA((B, NCT)),
                pltpu.SemaphoreType.DMA((2,)),
                pltpu.SemaphoreType.DMA((2,)),
            ],
            compiler_params=pltpu.CompilerParams(vmem_limit_bytes=100 * 2**20),
        )(x, w, w_o, lw, lx, ly)
    return jax.jit(f)


_kernel = make(UW=8, UX=5, UY=5, UC=15)


@jax.jit
def pallas_standalone__autoregressive_conv_wavenet__speech_kernel(x, w, w_o):
    return _kernel(x, w, w_o)
```

```python
import contextlib
import jax
import jax.numpy as jnp
import numpy as np
from jax.experimental import pallas as pl
from jax.experimental.pallas import tpu as pltpu

NF = 64
HOP = 34
NPROD = 96


class _V:
    def __init__(self, a, s=1):
        self.a = a
        self.s = s


_Z = _V(None)


def _add(x, y):
    if x.a is None:
        return y
    if y.a is None:
        return x
    if x.s == y.s:
        return _V(x.a + y.a, x.s)
    return _V(x.a - y.a) if x.s > 0 else _V(y.a - x.a)


def _neg(x):
    return x if x.a is None else _V(x.a, -x.s)


def _sub(x, y):
    return _add(x, _neg(y))


def _mul(x, c):
    if x.a is None or c == 0:
        return _Z
    if c == 1:
        return x
    if c == -1:
        return _neg(x)
    return _V(x.a * float(c * x.s))


def _val(x, like=None):
    if x.a is None:
        return jnp.zeros_like(like)
    return x.a if x.s > 0 else -x.a


def _cadd(x, y):
    return (_add(x[0], y[0]), _add(x[1], y[1]))


def _csub(x, y):
    return (_sub(x[0], y[0]), _sub(x[1], y[1]))


def _conj(x):
    return (x[0], _neg(x[1]))


def _ctw(x, k, n):
    k %= n
    a, b = x
    if k == 0:
        return x
    if 4 * k == n:
        return (b, _neg(a))
    if 2 * k == n:
        return (_neg(a), _neg(b))
    if 4 * k == 3 * n:
        return (_neg(b), a)
    c, s = np.cos(2 * np.pi * k / n), -np.sin(2 * np.pi * k / n)
    if (8 * k) % n == 0:
        pa, pb = (a if c > 0 else _neg(a)), (b if c > 0 else _neg(b))
        qa, qb = (a if s > 0 else _neg(a)), (b if s > 0 else _neg(b))
        r = float(np.sqrt(0.5))
        return (_mul(_sub(pa, qb), r), _mul(_add(qa, pb), r))
    return (_sub(_mul(a, c), _mul(b, s)), _add(_mul(a, s), _mul(b, c)))


def _cdft(x):
    n = len(x)
    if n == 1:
        return list(x)
    if n == 2:
        return [_cadd(x[0], x[1]), _csub(x[0], x[1])]
    ev, o1, o3 = _cdft(x[0::2]), _cdft(x[1::4]), _cdft(x[3::4])
    out = [None] * n
    for k in range(n // 4):
        a, b = _ctw(o1[k], k, n), _ctw(o3[k], 3 * k, n)
        p, m = _cadd(a, b), _csub(a, b)
        mi = (m[1], _neg(m[0]))
        out[k], out[k + n // 2] = _cadd(ev[k], p), _csub(ev[k], p)
        out[k + n // 4], out[k + 3 * n // 4] = _cadd(ev[k + n // 4], mi), _csub(ev[k + n // 4], mi)
    return out


def _rdft(x):
    n = len(x)
    if n == 2:
        return {0: (_add(x[0], x[1]), _Z), 1: (_sub(x[0], x[1]), _Z)}
    h, q = n // 2, n // 4
    s = [_add(x[i], x[i + h]) for i in range(h)]
    d = [_sub(x[i], x[i + h]) for i in range(h)]
    out = {2 * k: v for k, v in _rdft(s).items()}
    u = _cdft([_ctw((d[i], _neg(d[i + q])), i, n) for i in range(q)])
    for k in range(q):
        out[4 * k + 1] = u[k]
    return out


def _pass1(i2, a, b, c, d):
    s1, s2, d1, d2 = _add(a, c), _add(b, d), _sub(a, c), _sub(b, d)
    r = float(np.sqrt(0.5))
    t1, t2 = _mul(d2, r), _mul(s2, r)
    g1 = (_add(a, t1), _neg(_add(c, t2)))
    g2 = (d1, _neg(d2))
    g3 = (_sub(a, t1), _sub(c, t2))
    out = [_add(s1, s2), _sub(s1, s2)]
    for k, g in ((1, g1), (2, g2), (3, g3)):
        out.extend(_ctw(g, i2 * k, NF))
    return out


def _pass2(k1, v):
    if k1 == 0:
        return {8 * k: x for k, x in _rdft([v(i, 0) for i in range(8)]).items()}
    if k1 == 4:
        g = [v(i, 1) for i in range(8)]
        u = _cdft([_ctw((g[i], _neg(g[i + 4])), i, 16) for i in range(4)])
        return {4 + 16 * k: u[k] for k in range(4)}
    u = _cdft([(v(i, 2 * k1), v(i, 2 * k1 + 1)) for i in range(8)])
    return {k1 + 8 * k: u[k] for k in range(8)}


def _bin_keys():
    keys = sorted(k for k1 in range(5) for k in _pass2(k1, lambda i, j: _Z))
    rep = {}
    for k in keys:
        rep[k if k <= NF // 2 else NF - k] = k
    return [rep[k] for k in range(NF // 2 + 1)]


_REP = _bin_keys()


def _fwd_coef(q, nm):
    m = 4 * np.arange(nm) + q
    c = np.zeros((16, nm))
    c[0] = 1.0
    th8 = -2 * np.pi * 8 * m / NF
    c[1] = np.sin(th8) if q == 2 else np.cos(th8)
    for kp in range(1, 8):
        th = -2 * np.pi * kp * m / NF
        c[2 * kp] = np.cos(th)
        c[2 * kp + 1] = np.sin(th)
    return c


def _inv_coef(q):
    ns = [n for n in range(30, NF) if n % 4 == q]
    c = np.zeros((len(ns), 16))
    for r, n in enumerate(ns):
        sgn = (-1.0) ** (n // 4)
        c[r, 0] = 1.0 / NF
        c[r, 1] = (2.0, np.sqrt(2.0), -2.0, -np.sqrt(2.0))[q] * sgn / NF
        for kp in range(1, 8):
            th = 2 * np.pi * kp * n / NF
            c[r, 2 * kp] = 2.0 / NF * np.cos(th)
            c[r, 2 * kp + 1] = -2.0 / NF * np.sin(th)
    return c, ns


def _snap(c):
    return np.where(np.abs(c) < 1e-12, 0.0, c)


def _pair_cols(a):
    r, c = a.shape
    return a.reshape(r, c // 16, 2, 8).transpose(0, 1, 3, 2).reshape(r, c)


def _to_words(a):
    b = np.asarray(a, dtype=np.float32).astype(jnp.bfloat16).view(np.uint16).astype(np.uint32)
    return b[..., 0::2, :] | (b[..., 1::2, :] << 16)


def _constants(taps):
    lw, lx, ly = [], [], []
    for q in range(4):
        cw = _fwd_coef(q, 8)
        for mp in range(8):
            if 4 * mp + q >= taps:
                cw[:, mp] = 0.0
        lw.append(np.kron(_snap(cw), np.eye(16)))
        lx.append(_pair_cols(np.kron(_snap(_fwd_coef(q, 16)), np.eye(8))))
        cy = _inv_coef(q)[0]
        cy = np.pad(cy, ((0, 10 - cy.shape[0]), (0, 0)))
        ly.append(_pair_cols(np.kron(_snap(cy), np.eye(8))))
    return _to_words(np.stack(lw)), _to_words(np.stack(lx)), _to_words(np.stack(ly))


def _fwd_bins(T):
    t0 = [_V(T[q][0]) for q in range(4)]
    u0, u1 = _add(t0[0], t0[2]), _sub(t0[0], t0[2])
    v0, v1 = _add(t0[1], t0[3]), _sub(t0[1], t0[3])
    out = {0: (_add(u0, v0), _Z), 32: (_sub(u0, v0), _Z), 16: (u1, _neg(v1))}
    a0, a1, b2, a3 = (_V(T[q][1]) for q in range(4))
    s, d = _add(a1, a3), _sub(a3, a1)
    out[8] = (_add(a0, s), _add(b2, d))
    out[24] = (_sub(a0, s), _sub(d, b2))
    for kp in range(1, 8):
        t = [(_V(T[q][2 * kp]), _V(T[q][2 * kp + 1])) for q in range(4)]
        u0, u1 = _cadd(t[0], t[2]), _csub(t[0], t[2])
        v0, v1 = _cadd(t[1], t[3]), _csub(t[1], t[3])
        mi = (v1[1], _neg(v1[0]))
        out[kp] = _cadd(u0, v0)
        out[kp + 16] = _cadd(u1, mi)
        out[kp + 32] = _csub(u0, v0)
        out[kp + 48] = _csub(u1, mi)
    return out


def _rep_bin(bins, kappa):
    k = _REP[kappa]
    return bins[k] if k in bins else _conj(bins[NF - k])


def _operands(bins, is_w, like):
    ops = []
    for kappa in range(NF // 2):
        if kappa == 0:
            r0, r32 = bins[0][0], bins[NF // 2][0]
            forms = [_Z, r32, _neg(r0)] if is_w else [_Z, r32, r0]
        else:
            re, im = _rep_bin(bins, kappa)
            forms = [re, _sub(im, re), _add(re, im)] if is_w else [_add(re, im), re, im]
        ops.extend(_val(v, like) for v in forms)
    return ops


def _inv_butterfly(Y):
    A = [[None] * 16 for _ in range(4)]
    y0, y32 = Y(0)
    y16, y8, y24 = Y(16), Y(8), Y(24)
    e, o = _add(y0, y32), _sub(y0, y32)
    r2, i2 = _add(y16[0], y16[0]), _add(y16[1], y16[1])
    A[0][0], A[2][0] = _add(e, r2), _sub(e, r2)
    A[1][0], A[3][0] = _sub(o, i2), _add(o, i2)
    A[0][1] = _add(y8[0], y24[0])
    A[2][1] = _sub(y8[1], y24[1])
    dr, si = _sub(y8[0], y24[0]), _add(y24[1], y8[1])
    A[1][1], A[3][1] = _sub(dr, si), _add(dr, si)
    for kp in range(1, 8):
        ys = [Y(kp), Y(kp + 16), _conj(Y(32 - kp)), _conj(Y(16 - kp))]
        e0, e1 = _cadd(ys[0], ys[2]), _csub(ys[0], ys[2])
        f0, f1 = _cadd(ys[1], ys[3]), _csub(ys[1], ys[3])
        pi = (_neg(f1[1]), f1[0])
        for q, v in enumerate([_cadd(e0, f0), _cadd(e1, pi), _csub(e0, f0), _csub(e1, pi)]):
            A[q][2 * kp], A[q][2 * kp + 1] = v
    return [[_val(v) for v in row] for row in A]


def _pack2(a, b):
    return pltpu.pack_elementwise([a, b], packed_dtype=jnp.bfloat16)


def _half(v, i):
    return pltpu.unpack_elementwise(v, index=i, packed_dtype=jnp.bfloat16, unpacked_dtype=jnp.float32)


def _unpack(v):
    return pltpu.bitcast(v, jnp.bfloat16)


def _rhs_from_pairs(vs):
    return _unpack(jnp.concatenate([_pack2(vs[2 * u], vs[2 * u + 1]) for u in range(8)], axis=0))


def make(UW=8, UC=4, UY=5, UX=5, RC=400, scopes=False, WV=True, VMEM=100):
    sc = (lambda n: jax.named_scope(n)) if scopes else (lambda n: contextlib.nullcontext())
    B, T, D, K = 2, 4000, 512, 31
    NB = 60
    PITCH = NB * HOP
    TH = T // 2
    NG = B * NB // 8
    OFF = 32
    XROWS = 4128
    NCT = D // 128

    def kernel(x_hbm, w_hbm, wo_ref, lw_ref, lx_ref, ly_ref, o_hbm,
               xs, wbuf, xh, wh0, wh1, yh, tf, wtmp, zref, ost, xsem, wsem, osem):
        whs = (wh0, wh1)
        xs_bf = xs.bitcast(jnp.bfloat16)
        wv = wbuf.bitcast(jnp.uint32)

        def x_copy(b, ct):
            return pltpu.make_async_copy(
                x_hbm.at[b, :, pl.ds(pl.multiple_of(ct * 128, 128), 128)],
                xs_bf.at[ct, pl.ds(2 * (OFF + b * PITCH), T), :],
                xsem.at[b, ct])

        def col_of(j):
            return (j % 2) * D + (j // 2) * 128

        def w_copy(j, ):
            return pltpu.make_async_copy(
                w_hbm.at[:, :, pl.ds(pl.multiple_of(col_of(j), 128), 128)],
                wbuf.at[j % 2], wsem.at[j % 2])

        for ct in range(NCT):
            for b in range(B):
                x_copy(b, ct).start()
        w_copy(0).start()

        for ct in range(NCT):
            xs[ct, 0:OFF, :] = jnp.zeros((OFF, 128), jnp.uint32)
            for b in range(B):
                lo = OFF + b * PITCH + TH
                hi = OFF + (b + 1) * PITCH if b + 1 < B else XROWS
                xs[ct, lo:hi, :] = jnp.zeros((hi - lo, 128), jnp.uint32)

        def w_stage_mxu():
            def body(cg, _):
                r0 = pl.multiple_of(cg * 8, 8)
                Tq = []
                for q in range(4):
                    rows = [wv[0, min(4 * m + q, K - 1), pl.ds(r0, 8), :] for m in range(8)]
                    rhs = _unpack(jnp.concatenate(rows, axis=0))
                    res = jnp.dot(_unpack(lw_ref[q]), rhs, preferred_element_type=jnp.float32)
                    Tq.append([res[16 * j:16 * j + 16] for j in range(16)])
                ops = _operands(_fwd_bins(Tq), True, Tq[0][0])
                r1 = pl.multiple_of(cg * 16, 16)
                for p in range(NPROD):
                    wh0[p, pl.ds(r1, 16), :] = ops[p].astype(jnp.bfloat16)
                return 0
            with sc('W'):
                jax.lax.fori_loop(0, D // 16, body, 0, unroll=UW)

        def w_pass1(cg, src, tb, i2, dep=None):
            r0 = pl.multiple_of(cg * 8, 8)
            words = [wv[src, i, pl.ds(r0, 8), :] if i < K else None for i in range(i2, 32, 8)]
            if dep is not None:
                words = [v if v is None else v | dep for v in words]
            for h in range(2):
                vals = _pass1(i2, *[_Z if v is None else _V(_half(v, h)) for v in words])
                for j in range(8):
                    wtmp[tb, h, i2, j] = _val(vals[j])

        def w_pass2(cg, whu, tb, k1, dep=None):
            r0 = pl.multiple_of(cg * 8, 8)
            forms = []

            def ld(h, i, j):
                v = wtmp[tb, h, i, j]
                if dep is not None:
                    v = pltpu.bitcast(pltpu.bitcast(v, jnp.uint32) | dep, jnp.float32)
                return _V(v)
            for h in range(2):
                bins = _pass2(k1, lambda i, j: ld(h, i, j))
                fh = {}
                for kappa in range(NF // 2 + 1):
                    if _REP[kappa] in bins:
                        re, im = bins[_REP[kappa]]
                        if kappa == 0:
                            fh[2] = _val(_neg(re))
                        elif kappa == NF // 2:
                            fh[1] = _val(re)
                        else:
                            fh[3 * kappa] = _val(re)
                            fh[3 * kappa + 1] = _val(_sub(im, re))
                            fh[3 * kappa + 2] = _val(_add(re, im))
                forms.append(fh)
            for p in forms[0]:
                whu[p, pl.ds(r0, 8), :] = _pack2(forms[0][p], forms[1][p])

        def x_stage(ct):
            def body(g, _):
                base = g * (8 * HOP) + (OFF - 30)
                Tq = []
                for q in range(4):
                    xw = [xs[ct, pl.ds(base + 4 * m + q, 8, stride=HOP), :] for m in range(16)]
                    halves = []
                    for h in range(2):
                        rhs = _rhs_from_pairs([_half(v, h) for v in xw])
                        halves.append(jnp.dot(_unpack(lx_ref[q]), rhs, preferred_element_type=jnp.float32))
                    Tq.append([jnp.concatenate([halves[0][8 * j:8 * j + 8], halves[1][8 * j:8 * j + 8]], axis=0)
                               for j in range(16)])
                ops = _operands(_fwd_bins(Tq), False, Tq[0][0])
                r0 = pl.multiple_of(g * 16, 16)
                for p in range(NPROD):
                    xh[p, ct, pl.ds(r0, 16), :] = ops[p].astype(jnp.bfloat16)
                return 0
            with sc('X'):
                jax.lax.fori_loop(0, NG, body, 0, unroll=UX)

        def cw_stage(par):
            xhu = xh.bitcast(jnp.uint32)
            whc = whs[par].bitcast(jnp.uint32)
            whn = whs[1 - par].bitcast(jnp.uint32)
            src = 1 - par

            def prod(p, r):
                lhs = jnp.concatenate([_unpack(xhu[p, ct, r // 2:(r + MC) // 2, :]) for ct in range(NCT)], axis=1)
                return jnp.dot(lhs, _unpack(whc[p]), preferred_element_type=jnp.float32)

            def w_tasks(b, tb):
                t = [lambda dep, k1=k1: w_pass2(b, whn, tb, k1, dep) for k1 in (1, 2, 3, 0, 4)]
                t += [lambda dep, i2=i2: w_pass1((b + 1) % 32, src, 1 - tb, i2, dep) for i2 in range(8)]
                order = [0, 5, 6, 1, 7, 8, 2, 9, 10, 3, 11, 4, 12]
                return [t[i] for i in order] if WV else []

            def body(i, _):
                zero = zref[...]
                for u in range(UC):
                    b = i * UC + u
                    p = 3 * b
                    tasks = w_tasks(b, u % 2)
                    nv = 3 * NG * 2
                    state = [0, 0]

                    def seen(k):
                        for v in range(k.shape[0] // 8):
                            if state[1] < len(tasks) and state[0] >= (state[1] * nv) // len(tasks):
                                dep = (pltpu.bitcast(k[8 * v:8 * v + 8], jnp.uint32) & zero) if DEP else None
                                tasks[state[1]](dep)
                                state[1] += 1
                            state[0] += 1
                        return k
                    for r in range(0, NG * 16, MC):
                        k1 = seen(prod(p, r))
                        yh[2 * b, r:r + MC, :] = k1 - seen(prod(p + 2, r))
                        yh[2 * b + 1, r:r + MC, :] = k1 + seen(prod(p + 1, r))
                return 0
            with sc('C'):
                if WV:
                    for i2 in range(8):
                        w_pass1(0, src, 0, i2)
                jax.lax.fori_loop(0, (NF // 2) // UC, body, 0)

        def y_stage(is_g, ct):
            def body(g, _):
                zs = []
                for h in range(2):
                    r0 = pl.multiple_of(g * 16 + 8 * h, 8)

                    def Y(kappa):
                        if kappa == 0:
                            return (_V(yh[0, pl.ds(r0, 8), :]), _V(yh[1, pl.ds(r0, 8), :]))
                        re, im = _V(yh[2 * kappa, pl.ds(r0, 8), :]), _V(yh[2 * kappa + 1, pl.ds(r0, 8), :])
                        return (re, im) if _REP[kappa] == kappa else (re, _neg(im))
                    A = _inv_butterfly(Y)
                    z = {}
                    for q in range(4):
                        ns = _inv_coef(q)[1]
                        nr = 8 * (len(ns) + len(ns) % 2)
                        res = jnp.dot(_unpack(ly_ref[q, 0:nr // 2, :]), _rhs_from_pairs(A[q]),
                                      preferred_element_type=jnp.float32)
                        for r, n in enumerate(ns):
                            t = n - 30
                            hv = res[8 * r:8 * r + 8]
                            if is_g:
                                hf = tf[t, pl.ds(r0, 8), :]
                                z[t] = hf + hf * jnp.tanh(0.5 * hv)
                            else:
                                tf[t, pl.ds(r0, 8), :] = 0.5 * jnp.tanh(hv)
                    zs.append(z)
                if is_g:
                    zb = g * (8 * HOP)
                    for t in range(HOP):
                        xs[ct, pl.ds(zb + t, 8, stride=HOP), :] = _pack2(zs[0][t], zs[1][t])
                return 0
            with sc('Yg' if is_g else 'Yf'):
                jax.lax.fori_loop(0, NG, body, 0, unroll=UY)

        def x_all(ct, _):
            for b in range(B):
                x_copy(b, ct).wait()
            x_stage(ct)
            return 0
        jax.lax.fori_loop(0, NCT, x_all, 0)
        w_copy(0).wait()
        w_copy(1).start()
        wh0[0] = jnp.zeros((D, 128), jnp.bfloat16)
        wh1[0] = jnp.zeros((D, 128), jnp.bfloat16)
        zref[...] = jnp.zeros((8, 128), jnp.uint32)
        w_stage_mxu()

        def tile(jj, _):
            @pl.when(jj + 1 < NCT)
            def _():
                w_copy(2 * jj + 2).start()
            w_copy(2 * jj + 1).wait()
            cw_stage(0)
            y_stage(False, 0)

            @pl.when(jj + 1 < NCT)
            def _():
                w_copy(2 * jj + 3).start()
                w_copy(2 * jj + 2).wait()
            cw_stage(1)
            y_stage(True, jj)
            return 0
        jax.lax.fori_loop(0, NCT, tile, 0)

        nch = TH // RC

        def o_copy(i, slot):
            b = i // nch
            r = pl.multiple_of((i % nch) * (2 * RC), 16)
            return pltpu.make_async_copy(ost.at[slot], o_hbm.at[b, pl.ds(r, 2 * RC), :], osem.at[slot])

        def o_body(i, _):
            slot = i % 2

            @pl.when(i >= 2)
            def _():
                o_copy(i - 2, slot).wait()
            r0 = pl.multiple_of((i // nch) * PITCH + (i % nch) * RC, 8)
            z = jnp.concatenate([_unpack(xs[ct, pl.ds(r0, RC), :]) for ct in range(NCT)], axis=1)
            ost[slot] = jnp.dot(z, wo_ref[...], preferred_element_type=jnp.float32).astype(jnp.bfloat16)
            o_copy(i, slot).start()
            return 0
        with sc('O'):
            jax.lax.fori_loop(0, B * nch, o_body, 0)
        for k in (B * nch - 2, B * nch - 1):
            o_copy(k, k % 2).wait()

    def f(x, w, w_o):
        lw, lx, ly = _constants(K)
        vm = pl.BlockSpec(memory_space=pltpu.VMEM)
        anyspec = pl.BlockSpec(memory_space=pl.ANY)
        return pl.pallas_call(
            kernel,
            in_specs=[anyspec, anyspec, vm, vm, vm, vm],
            out_specs=anyspec,
            out_shape=jax.ShapeDtypeStruct((B, T, D), jnp.bfloat16),
            scratch_shapes=[
                pltpu.VMEM((NCT, XROWS, 128), jnp.uint32),
                pltpu.VMEM((2, K, D, 128), jnp.bfloat16),
                pltpu.VMEM((NPROD, NCT, NG * 16, 128), jnp.bfloat16),
                pltpu.VMEM((NPROD, D, 128), jnp.bfloat16),
                pltpu.VMEM((NPROD, D, 128), jnp.bfloat16),
                pltpu.VMEM((NF, NG * 16, 128), jnp.float32),
                pltpu.VMEM((HOP, NG * 16, 128), jnp.float32),
                pltpu.VMEM((2, 2, 8, 8, 8, 128), jnp.float32),
                pltpu.VMEM((8, 128), jnp.uint32),
                pltpu.VMEM((2, 2 * RC, D), jnp.bfloat16),
                pltpu.SemaphoreType.DMA((B, NCT)),
                pltpu.SemaphoreType.DMA((2,)),
                pltpu.SemaphoreType.DMA((2,)),
            ],
            compiler_params=pltpu.CompilerParams(vmem_limit_bytes=VMEM * 2**20),
        )(x, w, w_o, lw, lx, ly)
    return jax.jit(f)


_kernel = make(UC=8)


@jax.jit
def pallas_standalone__autoregressive_conv_wavenet__speech_kernel(x, w, w_o):
    return _kernel(x, w, w_o)
```

```python
import contextlib
import jax
import jax.numpy as jnp
import numpy as np
from jax.experimental import pallas as pl
from jax.experimental.pallas import tpu as pltpu

NF = 64
HOP = 34
NPROD = 96


class _V:
    def __init__(self, a, s=1):
        self.a = a
        self.s = s


_Z = _V(None)


def _add(x, y):
    if x.a is None:
        return y
    if y.a is None:
        return x
    if x.s == y.s:
        return _V(x.a + y.a, x.s)
    return _V(x.a - y.a) if x.s > 0 else _V(y.a - x.a)


def _neg(x):
    return x if x.a is None else _V(x.a, -x.s)


def _sub(x, y):
    return _add(x, _neg(y))


def _mul(x, c):
    if x.a is None or c == 0:
        return _Z
    if c == 1:
        return x
    if c == -1:
        return _neg(x)
    return _V(x.a * float(c * x.s))


def _val(x, like=None):
    if x.a is None:
        return jnp.zeros_like(like)
    return x.a if x.s > 0 else -x.a


def _cadd(x, y):
    return (_add(x[0], y[0]), _add(x[1], y[1]))


def _csub(x, y):
    return (_sub(x[0], y[0]), _sub(x[1], y[1]))


def _conj(x):
    return (x[0], _neg(x[1]))


def _ctw(x, k, n):
    k %= n
    a, b = x
    if k == 0:
        return x
    if 4 * k == n:
        return (b, _neg(a))
    if 2 * k == n:
        return (_neg(a), _neg(b))
    if 4 * k == 3 * n:
        return (_neg(b), a)
    c, s = np.cos(2 * np.pi * k / n), -np.sin(2 * np.pi * k / n)
    if (8 * k) % n == 0:
        pa, pb = (a if c > 0 else _neg(a)), (b if c > 0 else _neg(b))
        qa, qb = (a if s > 0 else _neg(a)), (b if s > 0 else _neg(b))
        r = float(np.sqrt(0.5))
        return (_mul(_sub(pa, qb), r), _mul(_add(qa, pb), r))
    return (_sub(_mul(a, c), _mul(b, s)), _add(_mul(a, s), _mul(b, c)))


def _cdft(x):
    n = len(x)
    if n == 1:
        return list(x)
    if n == 2:
        return [_cadd(x[0], x[1]), _csub(x[0], x[1])]
    ev, o1, o3 = _cdft(x[0::2]), _cdft(x[1::4]), _cdft(x[3::4])
    out = [None] * n
    for k in range(n // 4):
        a, b = _ctw(o1[k], k, n), _ctw(o3[k], 3 * k, n)
        p, m = _cadd(a, b), _csub(a, b)
        mi = (m[1], _neg(m[0]))
        out[k], out[k + n // 2] = _cadd(ev[k], p), _csub(ev[k], p)
        out[k + n // 4], out[k + 3 * n // 4] = _cadd(ev[k + n // 4], mi), _csub(ev[k + n // 4], mi)
    return out


def _rdft(x):
    n = len(x)
    if n == 2:
        return {0: (_add(x[0], x[1]), _Z), 1: (_sub(x[0], x[1]), _Z)}
    h, q = n // 2, n // 4
    s = [_add(x[i], x[i + h]) for i in range(h)]
    d = [_sub(x[i], x[i + h]) for i in range(h)]
    out = {2 * k: v for k, v in _rdft(s).items()}
    u = _cdft([_ctw((d[i], _neg(d[i + q])), i, n) for i in range(q)])
    for k in range(q):
        out[4 * k + 1] = u[k]
    return out


def _pass1(i2, a, b, c, d):
    s1, s2, d1, d2 = _add(a, c), _add(b, d), _sub(a, c), _sub(b, d)
    r = float(np.sqrt(0.5))
    t1, t2 = _mul(d2, r), _mul(s2, r)
    g1 = (_add(a, t1), _neg(_add(c, t2)))
    g2 = (d1, _neg(d2))
    g3 = (_sub(a, t1), _sub(c, t2))
    out = [_add(s1, s2), _sub(s1, s2)]
    for k, g in ((1, g1), (2, g2), (3, g3)):
        out.extend(_ctw(g, i2 * k, NF))
    return out


def _pass2(k1, v):
    if k1 == 0:
        return {8 * k: x for k, x in _rdft([v(i, 0) for i in range(8)]).items()}
    if k1 == 4:
        g = [v(i, 1) for i in range(8)]
        u = _cdft([_ctw((g[i], _neg(g[i + 4])), i, 16) for i in range(4)])
        return {4 + 16 * k: u[k] for k in range(4)}
    k1, par = k1 % 8, k1 // 8
    x = [(lambda i=i: (v(i, 2 * k1), v(i, 2 * k1 + 1))) for i in range(8)]
    if par == 0:
        u = _cdft([_cadd(x[n](), x[n + 4]()) for n in range(4)])
    else:
        u = _cdft([_ctw(_csub(x[n](), x[n + 4]()), n, 8) for n in range(4)])
    return {k1 + 8 * (2 * k + par): u[k] for k in range(4)}


_PASS2 = (1, 9, 2, 10, 3, 11, 0, 4)


def _bin_keys():
    keys = sorted(k for k1 in (0, 1, 2, 3, 4, 9, 10, 11) for k in _pass2(k1, lambda i, j: _Z))
    rep = {}
    for k in keys:
        rep[k if k <= NF // 2 else NF - k] = k
    return [rep[k] for k in range(NF // 2 + 1)]


_REP = _bin_keys()


def _fwd_coef(q, nm):
    m = 4 * np.arange(nm) + q
    c = np.zeros((16, nm))
    c[0] = 1.0
    th8 = -2 * np.pi * 8 * m / NF
    c[1] = np.sin(th8) if q == 2 else np.cos(th8)
    for kp in range(1, 8):
        th = -2 * np.pi * kp * m / NF
        c[2 * kp] = np.cos(th)
        c[2 * kp + 1] = np.sin(th)
    return c


def _snap(c):
    return np.where(np.abs(c) < 1e-12, 0.0, c)


def _pair_cols(a):
    r, c = a.shape
    return a.reshape(r, c // 16, 2, 8).transpose(0, 1, 3, 2).reshape(r, c)


def _to_words(a):
    b = np.asarray(a, dtype=np.float32).astype(jnp.bfloat16).view(np.uint16).astype(np.uint32)
    return b[..., 0::2, :] | (b[..., 1::2, :] << 16)


def _constants(taps):
    lw, lx = [], []
    for q in range(4):
        cw = _fwd_coef(q, 8)
        for mp in range(8):
            if 4 * mp + q >= taps:
                cw[:, mp] = 0.0
        lw.append(np.kron(_snap(cw), np.eye(16)))
        lx.append(_pair_cols(np.kron(_snap(_fwd_coef(q, 16)) * (2.0 / NF), np.eye(8))))
    return _to_words(np.stack(lw)), _to_words(np.stack(lx))


def _fwd_bins(T):
    t0 = [_V(T[q][0]) for q in range(4)]
    u0, u1 = _add(t0[0], t0[2]), _sub(t0[0], t0[2])
    v0, v1 = _add(t0[1], t0[3]), _sub(t0[1], t0[3])
    out = {0: (_add(u0, v0), _Z), 32: (_sub(u0, v0), _Z), 16: (u1, _neg(v1))}
    a0, a1, b2, a3 = (_V(T[q][1]) for q in range(4))
    s, d = _add(a1, a3), _sub(a3, a1)
    out[8] = (_add(a0, s), _add(b2, d))
    out[24] = (_sub(a0, s), _sub(d, b2))
    for kp in range(1, 8):
        t = [(_V(T[q][2 * kp]), _V(T[q][2 * kp + 1])) for q in range(4)]
        u0, u1 = _cadd(t[0], t[2]), _csub(t[0], t[2])
        v0, v1 = _cadd(t[1], t[3]), _csub(t[1], t[3])
        mi = (v1[1], _neg(v1[0]))
        out[kp] = _cadd(u0, v0)
        out[kp + 16] = _cadd(u1, mi)
        out[kp + 32] = _csub(u0, v0)
        out[kp + 48] = _csub(u1, mi)
    return out


def _rep_bin(bins, kappa):
    k = _REP[kappa]
    return bins[k] if k in bins else _conj(bins[NF - k])


def _operands(bins, is_w, like):
    ops = []
    for kappa in range(NF // 2):
        if kappa == 0:
            r0, r32 = bins[0][0], bins[NF // 2][0]
            forms = [_Z, r32, _neg(r0)] if is_w else [_Z, _mul(r32, 0.5), _mul(r0, 0.5)]
        else:
            re, im = _rep_bin(bins, kappa)
            forms = [re, _sub(im, re), _add(re, im)] if is_w else [_add(re, im), re, im]
        ops.extend(_val(v, like) for v in forms)
    return ops


def _icdft(x):
    return [_conj(v) for v in _cdft([_conj(v) for v in x])]


def _inv_pass_a(k1, y):
    if k1 == 0:
        (g0, _), (g4, _) = y(0), y(32)
        out = _inv_real8(g0, g4, y(8), y(16), _conj(y(40)), range(8))
        return {(i, 0): out[i] for i in range(8)}
    if k1 == 4:
        s = _icdft([y(4 + 16 * k) for k in range(4)])
        out = {}
        for i in range(4):
            re, im = _conj(_ctw(_conj(s[i]), i, 16))
            out[(i, 1)], out[(i + 4, 1)] = re, _neg(im)
        return out
    k1, par = k1 % 8, k1 // 8
    x = [y(k1 + 8 * k2) for k2 in range(8)]
    if par == 0:
        u = _icdft([_cadd(x[n], x[n + 4]) for n in range(4)])
    else:
        u = _icdft([_ctw(_csub(x[n], x[n + 4]), -n, 8) for n in range(4)])
    out = {}
    for k in range(4):
        out[(2 * k + par, 2 * k1)], out[(2 * k + par, 2 * k1 + 1)] = u[k]
    return out


def _inv_real8(g0, g4, t1, t2, t3, outs):
    r = float(np.sqrt(0.5))
    a, b = _add(g0, g4), _sub(g0, g4)
    p, s = _sub(t1[0], t3[0]), _add(t1[1], t3[1])
    base = [_add(a, t2[0]), _sub(b, t2[1]), _sub(a, t2[0]), _add(b, t2[1])]
    lazy = [lambda: _add(t1[0], t3[0]), lambda: _mul(_sub(p, s), r),
            lambda: _sub(t3[1], t1[1]), lambda: _neg(_mul(_add(s, p), r))]
    out, cache = {}, {}
    for i in outs:
        if i % 4 not in cache:
            cache[i % 4] = lazy[i % 4]()
        out[i] = _add(base[i % 4], cache[i % 4]) if i < 4 else _sub(base[i % 4], cache[i % 4])
    return out


def _inv_pass_b(i2, v):
    t = [_conj(_ctw(_conj((v[2 * k], v[2 * k + 1])), i2 * k, NF)) for k in (1, 2, 3)]
    outs = [i1 for i1 in range(8) if 8 * i1 + i2 >= NF - HOP]
    y = _inv_real8(v[0], v[1], t[0], t[1], t[2], outs)
    return {8 * i1 + i2 - (NF - HOP): y[i1] for i1 in outs}


def _pack2(a, b):
    return pltpu.pack_elementwise([a, b], packed_dtype=jnp.bfloat16)


def _half(v, i):
    return pltpu.unpack_elementwise(v, index=i, packed_dtype=jnp.bfloat16, unpacked_dtype=jnp.float32)


def _unpack(v):
    return pltpu.bitcast(v, jnp.bfloat16)


def _rhs_from_pairs(vs):
    return _unpack(jnp.concatenate([_pack2(vs[2 * u], vs[2 * u + 1]) for u in range(8)], axis=0))


def make(UW=8, UC=4, UY=5, UX=5, RC=400, scopes=False, WV=True, VMEM=100):
    sc = (lambda n: jax.named_scope(n)) if scopes else (lambda n: contextlib.nullcontext())
    B, T, D, K = 2, 4000, 512, 31
    NB = 60
    PITCH = NB * HOP
    TH = T // 2
    NG = B * NB // 8
    OFF = 32
    XROWS = 4352
    NCT = D // 128

    def kernel(x_hbm, w_hbm, wo_ref, lw_ref, lx_ref, o_hbm,
               xs, wbuf, xh, wh0, wh1, yh0, yh1, tf, wtmp, ytmp, ztmp, zref, ost, xsem, wsem, osem):
        whs = (wh0, wh1)
        xs_bf = xs.bitcast(jnp.bfloat16)
        wv = wbuf.bitcast(jnp.uint32)

        def x_copy(b, ct):
            return pltpu.make_async_copy(
                x_hbm.at[b, :, pl.ds(pl.multiple_of(ct * 128, 128), 128)],
                xs_bf.at[ct, pl.ds(2 * (OFF + b * PITCH), T), :],
                xsem.at[b, ct])

        def col_of(j):
            return (j % 2) * D + (j // 2) * 128

        def w_copy(j, ):
            return pltpu.make_async_copy(
                w_hbm.at[:, :, pl.ds(pl.multiple_of(col_of(j), 128), 128)],
                wbuf.at[j % 2], wsem.at[j % 2])

        with sc('pro0'):
            for ct in range(NCT):
                for b in range(B):
                    x_copy(b, ct).start()
            w_copy(0).start()

            for ct in range(NCT):
                xs[ct, 0:OFF, :] = jnp.zeros((OFF, 128), jnp.uint32)
                for b in range(B):
                    lo = OFF + b * PITCH + TH
                    hi = OFF + (b + 1) * PITCH if b + 1 < B else OFF + B * PITCH + 16
                    xs[ct, lo:hi, :] = jnp.zeros((hi - lo, 128), jnp.uint32)

        def w_stage_mxu():
            def body(cg, _):
                r0 = pl.multiple_of(cg * 8, 8)
                Tq = []
                for q in range(4):
                    rows = [wv[0, min(4 * m + q, K - 1), pl.ds(r0, 8), :] for m in range(8)]
                    rhs = _unpack(jnp.concatenate(rows, axis=0))
                    res = jnp.dot(_unpack(lw_ref[q]), rhs, preferred_element_type=jnp.float32)
                    Tq.append([res[16 * j:16 * j + 16] for j in range(16)])
                ops = _operands(_fwd_bins(Tq), True, Tq[0][0])
                r1 = pl.multiple_of(cg * 16, 16)
                for p in range(NPROD):
                    wh0[p, pl.ds(r1, 16), :] = ops[p].astype(jnp.bfloat16)
                return 0
            with sc('W'):
                jax.lax.fori_loop(0, D // 16, body, 0, unroll=UW)

        def w_pass1(cg, src, tb, i2, dep=None):
            r0 = pl.multiple_of(cg * 8, 8)
            words = [wv[src, i, pl.ds(r0, 8), :] if i < K else None for i in range(i2, 32, 8)]
            if dep is not None:
                words = [v if v is None else v | dep for v in words]
            for h in range(2):
                vals = _pass1(i2, *[_Z if v is None else _V(_half(v, h)) for v in words])
                for j in range(8):
                    last = _val(vals[j])
                    wtmp[tb, h, i2, j] = last
            return pltpu.bitcast(last, jnp.uint32)

        def w_pass2(cg, whu, tb, k1, dep=None):
            r0 = pl.multiple_of(cg * 8, 8)
            forms = []

            def ld(h, i, j):
                v = wtmp[tb, h, i, j]
                if dep is not None and (i < 4 if DEP2 == 1 else DEP2 == 2):
                    v = pltpu.bitcast(pltpu.bitcast(v, jnp.uint32) | dep, jnp.float32)
                return _V(v)
            for h in range(2):
                bins = _pass2(k1, lambda i, j: ld(h, i, j))
                fh = {}
                for kappa in range(NF // 2 + 1):
                    if _REP[kappa] in bins:
                        re, im = bins[_REP[kappa]]
                        if kappa == 0:
                            fh[2] = _val(_neg(re))
                        elif kappa == NF // 2:
                            fh[1] = _val(re)
                        else:
                            fh[3 * kappa] = _val(re)
                            fh[3 * kappa + 1] = _val(_sub(im, re))
                            fh[3 * kappa + 2] = _val(_add(re, im))
                forms.append(fh)
            for p in forms[0]:
                last = _pack2(forms[0][p], forms[1][p])
                whu[p, pl.ds(r0, 8), :] = last
            return last

        def x_stage(ct):
            def body(g, _):
                base = g * (8 * HOP) + (OFF - 30)
                Tq = []
                for q in range(4):
                    xw = [xs[ct, pl.ds(base + 4 * m + q, 8, stride=HOP), :] for m in range(16)]
                    halves = []
                    for h in range(2):
                        rhs = _rhs_from_pairs([_half(v, h) for v in xw])
                        halves.append(jnp.dot(_unpack(lx_ref[q]), rhs, preferred_element_type=jnp.float32))
                    Tq.append([jnp.concatenate([halves[0][8 * j:8 * j + 8], halves[1][8 * j:8 * j + 8]], axis=0)
                               for j in range(16)])
                ops = _operands(_fwd_bins(Tq), False, Tq[0][0])
                r0 = pl.multiple_of(g * 16, 16)
                for p in range(NPROD):
                    xh[p, ct, pl.ds(r0, 16), :] = ops[p].astype(jnp.bfloat16)
                return 0
            with sc('X'):
                jax.lax.fori_loop(0, NG, body, 0, unroll=UX)

        def cw_stage(par, ct):
            xhu = xh.bitcast(jnp.uint32)
            whc = whs[par].bitcast(jnp.uint32)
            whn = whs[1 - par].bitcast(jnp.uint32)
            src = 1 - par
            yh, yprev = (yh0, yh1) if par == 0 else (yh1, yh0)
            is_g = par == 0

            def prod(p, r):
                lhs = jnp.concatenate([_unpack(xhu[p, ct, r // 2:(r + MC) // 2, :]) for ct in range(NCT)], axis=1)
                return jnp.dot(lhs, _unpack(whc[p]), preferred_element_type=jnp.float32)

            def w_tasks(b, tb):
                t2 = [lambda dep, k1=k1: w_pass2(b, whn, tb, k1, dep) for k1 in _PASS2]
                t1 = [lambda dep, i2=i2: w_pass1((b + 1) % 32, src, 1 - tb, i2, dep) for i2 in range(8)]
                tw = [t for pair in zip(t2, t1) for t in pair] if WV else []
                nxt_half = jnp.minimum(b + 1, 2 * NG - 1)
                ya = [lambda dep, k1=k1: y_pass_a(yprev, nxt_half, 1 - tb, k1, dep) for k1 in _PASS2]
                yb = [lambda dep, i2=i2: y_pass_b(is_g, ct, b // 2, tb, tb, i2, dep) for i2 in range(8)]
                ty = [t for pair in zip(yb, ya) for t in pair]
                return [t for pair in zip(tw, ty) for t in pair] if WV else ty

            def body(i, _):
                zero = zref[...]
                outs = []
                for u in range(UC):
                    b = i * UC + u
                    p = 3 * b
                    tasks = w_tasks(b, u % 2)
                    nv = 3 * NG * 2
                    state = [0, 0]

                    def seen(k):
                        for v in range(k.shape[0] // 8):
                            while state[1] < len(tasks) and state[0] >= (state[1] * nv) // len(tasks):
                                bits = pltpu.bitcast(k[8 * v:8 * v + 8], jnp.uint32)
                                if CH and len(outs) >= CH:
                                    bits = bits | outs[-CH]
                                outs.append(tasks[state[1]](bits & zero))
                                state[1] += 1
                            state[0] += 1
                        return k
                    for r in range(0, NG * 16, MC):
                        k1 = seen(prod(p, r))
                        yh[2 * b, r:r + MC, :] = k1 - seen(prod(p + 2, r))
                        yh[2 * b + 1, r:r + MC, :] = k1 + seen(prod(p + 1, r))
                return 0
            with sc('C%d' % par):
                for i2 in range(8):
                    w_pass1(0, src, 0, i2)
                for k1 in _PASS2:
                    y_pass_a(yprev, 0, 0, k1)
                jax.lax.fori_loop(0, (NF // 2) // UC, body, 0)

        def y_pass_a(yh, half, tb, k1, dep=None):
            r0 = pl.multiple_of(half * 8, 8)

            def ld(idx, use_dep):
                v = yh[idx, pl.ds(r0, 8), :]
                if dep is not None and use_dep:
                    v = pltpu.bitcast(pltpu.bitcast(v, jnp.uint32) | dep, jnp.float32)
                return _V(v)

            def y(k):
                lo = k % NF < NF // 2 and (k1 % 8 != 0 or k < 20)
                if k == 0 or k == NF // 2:
                    return (ld(k // 32, lo), _Z)
                kappa = _REP.index(k)
                return (ld(2 * kappa, lo), ld(2 * kappa + 1, lo))
            for (i2, j), v in _inv_pass_a(k1, y).items():
                last = _val(v)
                ytmp[tb, i2, j] = last
            return pltpu.bitcast(last, jnp.uint32)

        def y_pass_b(is_g, ct, g, h, tb, i2, dep=None):
            r0 = pl.multiple_of(g * 16 + 8 * h, 8)
            v = [ytmp[tb, i2, j] for j in range(8)]
            if dep is not None and DEPY:
                v = [x if (j < 2 and DEPY == 1) else pltpu.bitcast(pltpu.bitcast(x, jnp.uint32) | dep, jnp.float32)
                     for j, x in enumerate(v)]
            for t, hv in _inv_pass_b(i2, [_V(x) for x in v]).items():
                if not is_g:
                    z = 0.5 * jnp.tanh(_val(hv))
                    tf[t, pl.ds(r0, 8), :] = z
                    continue
                hf = tf[t, pl.ds(r0, 8), :]
                z = hf + hf * jnp.tanh(_val(_mul(hv, 0.5)))
                if h == 0:
                    ztmp[t] = z
                else:
                    xs[ct, pl.ds(g * (8 * HOP) + t, 8, stride=HOP), :] = _pack2(ztmp[t], z)
            return pltpu.bitcast(z, jnp.uint32)

        def y_tail(ct):
            def body(g, _):
                for h in range(2):
                    for k1 in _PASS2:
                        y_pass_a(yh1, 2 * g + h, h, k1)
                for h in range(2):
                    for i2 in range(8):
                        y_pass_b(True, ct, g, h, h, i2)
                return 0
            with sc('Y'):
                jax.lax.fori_loop(0, NG, body, 0, unroll=UY)

        def x_all(ct, _):
            with sc('xwait'):
                for b in range(B):
                    x_copy(b, ct).wait()
            x_stage(ct)
            return 0
        jax.lax.fori_loop(0, NCT, x_all, 0)
        with sc('w0wait'):
            w_copy(0).wait()
        w_copy(1).start()
        wh0[0] = jnp.zeros((D, 128), jnp.bfloat16)
        wh1[0] = jnp.zeros((D, 128), jnp.bfloat16)
        zref[...] = jnp.zeros((8, 128), jnp.uint32)

        def zero_body(k, _):
            yh1[2 * k] = jnp.zeros((NG * 16, 128), jnp.float32)
            yh1[2 * k + 1] = jnp.zeros((NG * 16, 128), jnp.float32)
            tf[k] = jnp.zeros((NG * 16 + 16, 128), jnp.float32)
            return 0
        jax.lax.fori_loop(0, NF // 2, zero_body, 0)
        tf[32] = jnp.zeros((NG * 16 + 16, 128), jnp.float32)
        tf[33] = jnp.zeros((NG * 16 + 16, 128), jnp.float32)
        w_stage_mxu()

        def tile(jj, _):
            @pl.when(jj + 1 < NCT)
            def _():
                w_copy(2 * jj + 2).start()
            with sc('wwait'):
                w_copy(2 * jj + 1).wait()
            cw_stage(0, jnp.maximum(jj - 1, 0))

            @pl.when(jj + 1 < NCT)
            def _():
                w_copy(2 * jj + 3).start()
                w_copy(2 * jj + 2).wait()
            cw_stage(1, 0)
            return 0
        jax.lax.fori_loop(0, NCT, tile, 0)
        y_tail(NCT - 1)

        nch = TH // RC

        def o_copy(i, slot):
            b = i // nch
            r = pl.multiple_of((i % nch) * (2 * RC), 16)
            return pltpu.make_async_copy(ost.at[slot], o_hbm.at[b, pl.ds(r, 2 * RC), :], osem.at[slot])

        def o_body(i, _):
            slot = i % 2

            @pl.when(i >= 2)
            def _():
                o_copy(i - 2, slot).wait()
            r0 = pl.multiple_of((i // nch) * PITCH + (i % nch) * RC, 8)
            z = jnp.concatenate([_unpack(xs[ct, pl.ds(r0, RC), :]) for ct in range(NCT)], axis=1)
            ost[slot] = jnp.dot(z, wo_ref[...], preferred_element_type=jnp.float32).astype(jnp.bfloat16)
            o_copy(i, slot).start()
            return 0
        with sc('O'):
            jax.lax.fori_loop(0, B * nch, o_body, 0)
        with sc('owait'):
            for k in (B * nch - 2, B * nch - 1):
                o_copy(k, k % 2).wait()

    def f(x, w, w_o):
        lw, lx = _constants(K)
        vm = pl.BlockSpec(memory_space=pltpu.VMEM)
        anyspec = pl.BlockSpec(memory_space=pl.ANY)
        return pl.pallas_call(
            kernel,
            in_specs=[anyspec, anyspec, vm, vm, vm],
            out_specs=anyspec,
            out_shape=jax.ShapeDtypeStruct((B, T, D), jnp.bfloat16),
            scratch_shapes=[
                pltpu.VMEM((NCT, XROWS, 128), jnp.uint32),
                pltpu.VMEM((2, K, D, 128), jnp.bfloat16),
                pltpu.VMEM((NPROD, NCT, NG * 16, 128), jnp.bfloat16),
                pltpu.VMEM((NPROD, D, 128), jnp.bfloat16),
                pltpu.VMEM((NPROD, D, 128), jnp.bfloat16),
                pltpu.VMEM((NF, NG * 16, 128), jnp.float32),
                pltpu.VMEM((NF, NG * 16, 128), jnp.float32),
                pltpu.VMEM((HOP, NG * 16 + 16, 128), jnp.float32),
                pltpu.VMEM((2, 2, 8, 8, 8, 128), jnp.float32),
                pltpu.VMEM((2, 8, 8, 8, 128), jnp.float32),
                pltpu.VMEM((HOP, 8, 128), jnp.float32),
                pltpu.VMEM((8, 128), jnp.uint32),
                pltpu.VMEM((2, 2 * RC, D), jnp.bfloat16),
                pltpu.SemaphoreType.DMA((B, NCT)),
                pltpu.SemaphoreType.DMA((2,)),
                pltpu.SemaphoreType.DMA((2,)),
            ],
            compiler_params=pltpu.CompilerParams(vmem_limit_bytes=VMEM * 2**20),
        )(x, w, w_o, lw, lx)
    return jax.jit(f)


_kernel = make(UC=8, CH=6)


@jax.jit
def pallas_standalone__autoregressive_conv_wavenet__speech_kernel(x, w, w_o):
    return _kernel(x, w, w_o)
```

```python
import contextlib
import jax
import jax.numpy as jnp
import numpy as np
from jax.experimental import pallas as pl
from jax.experimental.pallas import tpu as pltpu

NF = 64
HOP = 34
NPROD = 96


class _V:
    def __init__(self, a, s=1):
        self.a = a
        self.s = s


_Z = _V(None)


def _add(x, y):
    if x.a is None:
        return y
    if y.a is None:
        return x
    if x.s == y.s:
        return _V(x.a + y.a, x.s)
    return _V(x.a - y.a) if x.s > 0 else _V(y.a - x.a)


def _neg(x):
    return x if x.a is None else _V(x.a, -x.s)


def _sub(x, y):
    return _add(x, _neg(y))


def _mul(x, c):
    if x.a is None or c == 0:
        return _Z
    if c == 1:
        return x
    if c == -1:
        return _neg(x)
    return _V(x.a * float(c * x.s))


def _val(x, like=None):
    if x.a is None:
        return jnp.zeros_like(like)
    return x.a if x.s > 0 else -x.a


def _cadd(x, y):
    return (_add(x[0], y[0]), _add(x[1], y[1]))


def _csub(x, y):
    return (_sub(x[0], y[0]), _sub(x[1], y[1]))


def _conj(x):
    return (x[0], _neg(x[1]))


def _ctw(x, k, n):
    k %= n
    a, b = x
    if k == 0:
        return x
    if 4 * k == n:
        return (b, _neg(a))
    if 2 * k == n:
        return (_neg(a), _neg(b))
    if 4 * k == 3 * n:
        return (_neg(b), a)
    c, s = np.cos(2 * np.pi * k / n), -np.sin(2 * np.pi * k / n)
    if (8 * k) % n == 0:
        pa, pb = (a if c > 0 else _neg(a)), (b if c > 0 else _neg(b))
        qa, qb = (a if s > 0 else _neg(a)), (b if s > 0 else _neg(b))
        r = float(np.sqrt(0.5))
        return (_mul(_sub(pa, qb), r), _mul(_add(qa, pb), r))
    return (_sub(_mul(a, c), _mul(b, s)), _add(_mul(a, s), _mul(b, c)))


def _cdft(x):
    n = len(x)
    if n == 1:
        return list(x)
    if n == 2:
        return [_cadd(x[0], x[1]), _csub(x[0], x[1])]
    ev, o1, o3 = _cdft(x[0::2]), _cdft(x[1::4]), _cdft(x[3::4])
    out = [None] * n
    for k in range(n // 4):
        a, b = _ctw(o1[k], k, n), _ctw(o3[k], 3 * k, n)
        p, m = _cadd(a, b), _csub(a, b)
        mi = (m[1], _neg(m[0]))
        out[k], out[k + n // 2] = _cadd(ev[k], p), _csub(ev[k], p)
        out[k + n // 4], out[k + 3 * n // 4] = _cadd(ev[k + n // 4], mi), _csub(ev[k + n // 4], mi)
    return out


def _rdft(x):
    n = len(x)
    if n == 2:
        return {0: (_add(x[0], x[1]), _Z), 1: (_sub(x[0], x[1]), _Z)}
    h, q = n // 2, n // 4
    s = [_add(x[i], x[i + h]) for i in range(h)]
    d = [_sub(x[i], x[i + h]) for i in range(h)]
    out = {2 * k: v for k, v in _rdft(s).items()}
    u = _cdft([_ctw((d[i], _neg(d[i + q])), i, n) for i in range(q)])
    for k in range(q):
        out[4 * k + 1] = u[k]
    return out


def _pass1(i2, a, b, c, d):
    s1, s2, d1, d2 = _add(a, c), _add(b, d), _sub(a, c), _sub(b, d)
    r = float(np.sqrt(0.5))
    t1, t2 = _mul(d2, r), _mul(s2, r)
    g1 = (_add(a, t1), _neg(_add(c, t2)))
    g2 = (d1, _neg(d2))
    g3 = (_sub(a, t1), _sub(c, t2))
    out = [_add(s1, s2), _sub(s1, s2)]
    for k, g in ((1, g1), (2, g2), (3, g3)):
        out.extend(_ctw(g, i2 * k, NF))
    return out


def _pass2(k1, v):
    if k1 == 0:
        return {8 * k: x for k, x in _rdft([v(i, 0) for i in range(8)]).items()}
    if k1 == 4:
        g = [v(i, 1) for i in range(8)]
        u = _cdft([_ctw((g[i], _neg(g[i + 4])), i, 16) for i in range(4)])
        return {4 + 16 * k: u[k] for k in range(4)}
    k1, par = k1 % 8, k1 // 8
    x = [(lambda i=i: (v(i, 2 * k1), v(i, 2 * k1 + 1))) for i in range(8)]
    if par == 0:
        u = _cdft([_cadd(x[n](), x[n + 4]()) for n in range(4)])
    else:
        u = _cdft([_ctw(_csub(x[n](), x[n + 4]()), n, 8) for n in range(4)])
    return {k1 + 8 * (2 * k + par): u[k] for k in range(4)}


_PASS2 = (1, 9, 2, 10, 3, 11, 0, 4)


def _bin_keys():
    keys = sorted(k for k1 in (0, 1, 2, 3, 4, 9, 10, 11) for k in _pass2(k1, lambda i, j: _Z))
    rep = {}
    for k in keys:
        rep[k if k <= NF // 2 else NF - k] = k
    return [rep[k] for k in range(NF // 2 + 1)]


_REP = _bin_keys()


def _fwd_coef(q, nm):
    m = 4 * np.arange(nm) + q
    c = np.zeros((16, nm))
    c[0] = 1.0
    th8 = -2 * np.pi * 8 * m / NF
    c[1] = np.sin(th8) if q == 2 else np.cos(th8)
    for kp in range(1, 8):
        th = -2 * np.pi * kp * m / NF
        c[2 * kp] = np.cos(th)
        c[2 * kp + 1] = np.sin(th)
    return c


def _snap(c):
    return np.where(np.abs(c) < 1e-12, 0.0, c)


def _pair_cols(a):
    r, c = a.shape
    return a.reshape(r, c // 16, 2, 8).transpose(0, 1, 3, 2).reshape(r, c)


def _to_words(a):
    b = np.asarray(a, dtype=np.float32).astype(jnp.bfloat16).view(np.uint16).astype(np.uint32)
    return b[..., 0::2, :] | (b[..., 1::2, :] << 16)


def _constants(taps):
    lw, lx = [], []
    for q in range(4):
        cw = _fwd_coef(q, 8)
        for mp in range(8):
            if 4 * mp + q >= taps:
                cw[:, mp] = 0.0
        lw.append(np.kron(_snap(cw), np.eye(16)))
        lx.append(_pair_cols(np.kron(_snap(_fwd_coef(q, 16)) * (2.0 / NF), np.eye(8))))
    return _to_words(np.stack(lw)), _to_words(np.stack(lx))


def _fwd_bins(T):
    t0 = [_V(T[q][0]) for q in range(4)]
    u0, u1 = _add(t0[0], t0[2]), _sub(t0[0], t0[2])
    v0, v1 = _add(t0[1], t0[3]), _sub(t0[1], t0[3])
    out = {0: (_add(u0, v0), _Z), 32: (_sub(u0, v0), _Z), 16: (u1, _neg(v1))}
    a0, a1, b2, a3 = (_V(T[q][1]) for q in range(4))
    s, d = _add(a1, a3), _sub(a3, a1)
    out[8] = (_add(a0, s), _add(b2, d))
    out[24] = (_sub(a0, s), _sub(d, b2))
    for kp in range(1, 8):
        t = [(_V(T[q][2 * kp]), _V(T[q][2 * kp + 1])) for q in range(4)]
        u0, u1 = _cadd(t[0], t[2]), _csub(t[0], t[2])
        v0, v1 = _cadd(t[1], t[3]), _csub(t[1], t[3])
        mi = (v1[1], _neg(v1[0]))
        out[kp] = _cadd(u0, v0)
        out[kp + 16] = _cadd(u1, mi)
        out[kp + 32] = _csub(u0, v0)
        out[kp + 48] = _csub(u1, mi)
    return out


def _rep_bin(bins, kappa):
    k = _REP[kappa]
    return bins[k] if k in bins else _conj(bins[NF - k])


def _operands(bins, is_w, like):
    ops = []
    for kappa in range(NF // 2):
        if kappa == 0:
            r0, r32 = bins[0][0], bins[NF // 2][0]
            forms = [_Z, r32, _neg(r0)] if is_w else [_Z, _mul(r32, 0.5), _mul(r0, 0.5)]
        else:
            re, im = _rep_bin(bins, kappa)
            forms = [re, _sub(im, re), _add(re, im)] if is_w else [_add(re, im), re, im]
        ops.extend(_val(v, like) for v in forms)
    return ops


def _icdft(x):
    return [_conj(v) for v in _cdft([_conj(v) for v in x])]


def _inv_pass_a(k1, y):
    if k1 == 0:
        (g0, _), (g4, _) = y(0), y(32)
        out = _inv_real8(g0, g4, y(8), y(16), _conj(y(40)), range(8))
        return {(i, 0): out[i] for i in range(8)}
    if k1 == 4:
        s = _icdft([y(4 + 16 * k) for k in range(4)])
        out = {}
        for i in range(4):
            re, im = _conj(_ctw(_conj(s[i]), i, 16))
            out[(i, 1)], out[(i + 4, 1)] = re, _neg(im)
        return out
    k1, par = k1 % 8, k1 // 8
    x = [y(k1 + 8 * k2) for k2 in range(8)]
    if par == 0:
        u = _icdft([_cadd(x[n], x[n + 4]) for n in range(4)])
    else:
        u = _icdft([_ctw(_csub(x[n], x[n + 4]), -n, 8) for n in range(4)])
    out = {}
    for k in range(4):
        out[(2 * k + par, 2 * k1)], out[(2 * k + par, 2 * k1 + 1)] = u[k]
    return out


def _inv_real8(g0, g4, t1, t2, t3, outs):
    r = float(np.sqrt(0.5))
    a, b = _add(g0, g4), _sub(g0, g4)
    p, s = _sub(t1[0], t3[0]), _add(t1[1], t3[1])
    base = [_add(a, t2[0]), _sub(b, t2[1]), _sub(a, t2[0]), _add(b, t2[1])]
    lazy = [lambda: _add(t1[0], t3[0]), lambda: _mul(_sub(p, s), r),
            lambda: _sub(t3[1], t1[1]), lambda: _neg(_mul(_add(s, p), r))]
    out, cache = {}, {}
    for i in outs:
        if i % 4 not in cache:
            cache[i % 4] = lazy[i % 4]()
        out[i] = _add(base[i % 4], cache[i % 4]) if i < 4 else _sub(base[i % 4], cache[i % 4])
    return out


def _inv_pass_b(i2, v):
    t = [_conj(_ctw(_conj((v[2 * k], v[2 * k + 1])), i2 * k, NF)) for k in (1, 2, 3)]
    outs = [i1 for i1 in range(8) if 8 * i1 + i2 >= NF - HOP]
    y = _inv_real8(v[0], v[1], t[0], t[1], t[2], outs)
    return {8 * i1 + i2 - (NF - HOP): y[i1] for i1 in outs}


def _pack2(a, b):
    return pltpu.pack_elementwise([a, b], packed_dtype=jnp.bfloat16)


def _half(v, i):
    return pltpu.unpack_elementwise(v, index=i, packed_dtype=jnp.bfloat16, unpacked_dtype=jnp.float32)


def _unpack(v):
    return pltpu.bitcast(v, jnp.bfloat16)


def _rhs_from_pairs(vs):
    return _unpack(jnp.concatenate([_pack2(vs[2 * u], vs[2 * u + 1]) for u in range(8)], axis=0))


def make(UW=8, UC=4, UY=5, UX=5, RC=400, scopes=False, WV=True, VMEM=100):
    sc = (lambda n: jax.named_scope(n)) if scopes else (lambda n: contextlib.nullcontext())
    B, T, D, K = 2, 4000, 512, 31
    NB = 60
    PITCH = NB * HOP
    TH = T // 2
    NG = B * NB // 8
    OFF = 32
    XROWS = 4352
    NCT = D // 128

    def kernel(x_hbm, w_hbm, wo_hbm, lw_ref, lx_ref, o_hbm,
               xs, wbuf, xh, wh0, wh1, yh0, yh1, tf, wtmp, ytmp, ztmp, zref, ost, wo_ref, xsem, wsem, psem, osem):
        whs = (wh0, wh1)
        xs_bf = xs.bitcast(jnp.bfloat16)
        wv = wbuf.bitcast(jnp.uint32)

        XP = (((0, 0, 1440),), ((0, 1440, TH), (1, 0, 720)), ((1, 720, TH),))

        def x_copies(ct, k):
            return [pltpu.make_async_copy(
                x_hbm.at[b, pl.ds(2 * lo, 2 * (hi - lo)), pl.ds(pl.multiple_of(ct * 128, 128), 128)],
                xs_bf.at[ct, pl.ds(2 * (OFF + b * PITCH + lo), 2 * (hi - lo)), :],
                xsem.at[ct, k, n]) for n, (b, lo, hi) in enumerate(XP[k])]

        def col_of(j):
            return (j % 2) * D + (j // 2) * 128

        def w_copy(j, ):
            return pltpu.make_async_copy(
                w_hbm.at[:, :, pl.ds(pl.multiple_of(col_of(j), 128), 128)],
                wbuf.at[j % 2], wsem.at[j % 2])

        def w_piece(j, lo, n, k):
            return pltpu.make_async_copy(
                w_hbm.at[:, pl.ds(lo, n), pl.ds(col_of(j), 128)],
                wbuf.at[j % 2, :, pl.ds(lo, n), :], psem.at[k])

        W1 = ((0, 272), (272, D - 272))
        wo_copy = pltpu.make_async_copy(wo_hbm, wo_ref, psem.at[6])

        with sc('pro0'):
            for ct in range(NCT):
                for k in range(3):
                    for c in x_copies(ct, k):
                        c.start()
            for k in range(4):
                w_piece(0, 128 * k, 128, k).start()
            for k, (lo, n) in enumerate(W1):
                w_piece(1, lo, n, 4 + k).start()

            for ct in range(NCT):
                xs[ct, 0:OFF, :] = jnp.zeros((OFF, 128), jnp.uint32)
                for b in range(B):
                    lo = OFF + b * PITCH + TH
                    hi = OFF + (b + 1) * PITCH if b + 1 < B else OFF + B * PITCH + 16
                    xs[ct, lo:hi, :] = jnp.zeros((hi - lo, 128), jnp.uint32)

        wh0[0] = jnp.zeros((D, 128), jnp.bfloat16)
        wh1[0] = jnp.zeros((D, 128), jnp.bfloat16)
        zref[...] = jnp.zeros((8, 128), jnp.uint32)
        ytmp[...] = jnp.zeros(ytmp.shape, jnp.float32)
        ztmp[...] = jnp.zeros(ztmp.shape, jnp.float32)

        def zero_body(k, _):
            yh1[2 * k] = jnp.zeros((NG * 16, 128), jnp.float32)
            yh1[2 * k + 1] = jnp.zeros((NG * 16, 128), jnp.float32)
            tf[k] = jnp.zeros((NG * 16 + 16, 128), jnp.float32)
            return 0
        jax.lax.fori_loop(0, NF // 2, zero_body, 0)
        tf[32] = jnp.zeros((NG * 16 + 16, 128), jnp.float32)
        tf[33] = jnp.zeros((NG * 16 + 16, 128), jnp.float32)
        def w_stage_mxu():
            def body(cg, _):
                r0 = pl.multiple_of(cg * 8, 8)
                Tq = []
                for q in range(4):
                    rows = [wv[0, min(4 * m + q, K - 1), pl.ds(r0, 8), :] for m in range(8)]
                    rhs = _unpack(jnp.concatenate(rows, axis=0))
                    res = jnp.dot(_unpack(lw_ref[q]), rhs, preferred_element_type=jnp.float32)
                    Tq.append([res[16 * j:16 * j + 16] for j in range(16)])
                ops = _operands(_fwd_bins(Tq), True, Tq[0][0])
                r1 = pl.multiple_of(cg * 16, 16)
                for p in range(NPROD):
                    wh0[p, pl.ds(r1, 16), :] = ops[p].astype(jnp.bfloat16)
                return 0
            def quarter(k, _):
                with sc('w0wait'):
                    pltpu.make_async_copy(
                        w_hbm.at[:, pl.ds(0, 128), pl.ds(0, 128)],
                        wbuf.at[0, :, pl.ds(pl.multiple_of(k * 128, 128), 128), :], psem.at[k]).wait()
                for cg in range(8):
                    body(k * 8 + cg, 0)
                return 0
            with sc('W'):
                jax.lax.fori_loop(0, 4, quarter, 0)

        def w_pass1(cg, src, tb, i2, dep=None):
            r0 = pl.multiple_of(cg * 8, 8)
            words = [wv[src, i, pl.ds(r0, 8), :] if i < K else None for i in range(i2, 32, 8)]
            if dep is not None:
                words = [v if v is None else v | dep for v in words]
            for h in range(2):
                vals = _pass1(i2, *[_Z if v is None else _V(_half(v, h)) for v in words])
                for j in range(8):
                    last = _val(vals[j])
                    wtmp[tb, h, i2, j] = last
            return pltpu.bitcast(last, jnp.uint32)

        def w_pass2(cg, whu, tb, k1, dep=None):
            r0 = pl.multiple_of(cg * 8, 8)
            forms = []

            def ld(h, i, j):
                v = wtmp[tb, h, i, j]
                if dep is not None and (i < 4 if DEP2 == 1 else DEP2 == 2):
                    v = pltpu.bitcast(pltpu.bitcast(v, jnp.uint32) | dep, jnp.float32)
                return _V(v)
            for h in range(2):
                bins = _pass2(k1, lambda i, j: ld(h, i, j))
                fh = {}
                for kappa in range(NF // 2 + 1):
                    if _REP[kappa] in bins:
                        re, im = bins[_REP[kappa]]
                        if kappa == 0:
                            fh[2] = _val(_neg(re))
                        elif kappa == NF // 2:
                            fh[1] = _val(re)
                        else:
                            fh[3 * kappa] = _val(re)
                            fh[3 * kappa + 1] = _val(_sub(im, re))
                            fh[3 * kappa + 2] = _val(_add(re, im))
                forms.append(fh)
            for p in forms[0]:
                last = _pack2(forms[0][p], forms[1][p])
                whu[p, pl.ds(r0, 8), :] = last
            return last

        def x_stage(ct, k):
            def body(g, _):
                base = g * (8 * HOP) + (OFF - 30)
                Tq = []
                for q in range(4):
                    xw = [xs[ct, pl.ds(base + 4 * m + q, 8, stride=HOP), :] for m in range(16)]
                    halves = []
                    for h in range(2):
                        rhs = _rhs_from_pairs([_half(v, h) for v in xw])
                        halves.append(jnp.dot(_unpack(lx_ref[q]), rhs, preferred_element_type=jnp.float32))
                    Tq.append([jnp.concatenate([halves[0][8 * j:8 * j + 8], halves[1][8 * j:8 * j + 8]], axis=0)
                               for j in range(16)])
                ops = _operands(_fwd_bins(Tq), False, Tq[0][0])
                r0 = pl.multiple_of(g * 16, 16)
                for p in range(NPROD):
                    xh[p, ct, pl.ds(r0, 16), :] = ops[p].astype(jnp.bfloat16)
                return 0
            with sc('X'):
                for gi in range(NG // 3):
                    body(k * (NG // 3) + gi, 0)

        def cw_stage(par, ct, has_next2, wait_next2):
            xhu = xh.bitcast(jnp.uint32)
            whc = whs[par].bitcast(jnp.uint32)
            whn = whs[1 - par].bitcast(jnp.uint32)
            src = 1 - par
            yh, yprev = (yh0, yh1) if par == 0 else (yh1, yh0)
            is_g = par == 0

            def prod(p, r):
                lhs = jnp.concatenate([_unpack(xhu[p, ct, r // 2:(r + MC) // 2, :]) for ct in range(NCT)], axis=1)
                return jnp.dot(lhs, _unpack(whc[p]), preferred_element_type=jnp.float32)

            def w_tasks(b, tb):
                t2 = [lambda dep, k1=k1: w_pass2(b, whn, tb, k1, dep) for k1 in _PASS2]
                src1 = jnp.where(b == NF // 2 - 1, 1 - src, src)
                t1 = [lambda dep, i2=i2: w_pass1((b + 1) % (NF // 2), src1, 1 - tb, i2, dep) for i2 in range(8)]
                tw = [t for pair in zip(t2, t1) for t in pair]
                half_a = jnp.minimum(b, 2 * NG - 1)
                g_b = jnp.where(b == 0, NG, (b - 1) // 2)
                ya = [lambda dep, k1=k1: y_pass_a(yprev, half_a, tb, k1, dep) for k1 in _PASS2]
                yb = [lambda dep, i2=i2: y_pass_b(is_g, ct, g_b, 1 - tb, 1 - tb, i2, dep) for i2 in range(8)]
                ty = [t for pair in zip(yb, ya) for t in pair]
                return [t for pair in zip(tw, ty) for t in pair]

            def body(i, _):
                @pl.when(jnp.logical_and(i == (NF // 2) // UC - 1, has_next2))
                def _():
                    wait_next2()
                zero = zref[...]
                outs = []
                for u in range(UC):
                    b = i * UC + u
                    p = 3 * b
                    tasks = w_tasks(b, u % 2)
                    nv = 3 * NG * 2
                    state = [0, 0]

                    def seen(k):
                        for v in range(k.shape[0] // 8):
                            while state[1] < len(tasks) and state[0] >= (state[1] * nv) // len(tasks):
                                bits = pltpu.bitcast(k[8 * v:8 * v + 8], jnp.uint32)
                                if CH and len(outs) >= CH:
                                    bits = bits | outs[-CH]
                                outs.append(tasks[state[1]](bits & zero))
                                state[1] += 1
                            state[0] += 1
                        return k
                    for r in range(0, NG * 16, MC):
                        k1 = seen(prod(p, r))
                        yh[2 * b, r:r + MC, :] = k1 - seen(prod(p + 2, r))
                        yh[2 * b + 1, r:r + MC, :] = k1 + seen(prod(p + 1, r))
                return 0
            with sc('C%d' % par):
                jax.lax.fori_loop(0, (NF // 2) // UC, body, 0)

        def y_pass_a(yh, half, tb, k1, dep=None):
            r0 = pl.multiple_of(half * 8, 8)

            def ld(idx, use_dep):
                v = yh[idx, pl.ds(r0, 8), :]
                if dep is not None and use_dep:
                    v = pltpu.bitcast(pltpu.bitcast(v, jnp.uint32) | dep, jnp.float32)
                return _V(v)

            def y(k):
                lo = k % NF < NF // 2 and (k1 % 8 != 0 or k < 20)
                if k == 0 or k == NF // 2:
                    return (ld(k // 32, lo), _Z)
                kappa = _REP.index(k)
                return (ld(2 * kappa, lo), ld(2 * kappa + 1, lo))
            for (i2, j), v in _inv_pass_a(k1, y).items():
                last = _val(v)
                ytmp[tb, i2, j] = last
            return pltpu.bitcast(last, jnp.uint32)

        def y_pass_b(is_g, ct, g, h, tb, i2, dep=None):
            r0 = pl.multiple_of(g * 16 + 8 * h, 8)
            v = [ytmp[tb, i2, j] for j in range(8)]
            if dep is not None and DEPY:
                v = [x if (j < 2 and DEPY == 1) else pltpu.bitcast(pltpu.bitcast(x, jnp.uint32) | dep, jnp.float32)
                     for j, x in enumerate(v)]
            for t, hv in _inv_pass_b(i2, [_V(x) for x in v]).items():
                if not is_g:
                    z = 0.5 * jnp.tanh(_val(hv))
                    tf[t, pl.ds(r0, 8), :] = z
                    continue
                hf = tf[t, pl.ds(r0, 8), :]
                z = hf + hf * jnp.tanh(_val(_mul(hv, 0.5)))
                if h == 0:
                    ztmp[t] = z
                else:
                    xs[ct, pl.ds(g * (8 * HOP) + t, 8, stride=HOP), :] = _pack2(ztmp[t], z)
            return pltpu.bitcast(z, jnp.uint32)

        def y_group(ct, g):
            for h in range(2):
                for k1 in _PASS2:
                    y_pass_a(yh1, jnp.minimum(2 * g + h, 2 * NG - 1), h, k1)
            for h in range(2):
                for i2 in range(8):
                    y_pass_b(True, ct, g, h, h, i2)

        def x_all(i, _):
            ct, k = i // 3, i % 3
            with sc('xwait'):
                for kk in range(3):
                    @pl.when(k == kk)
                    def _():
                        for c in x_copies(ct, kk):
                            c.wait()
            x_stage(ct, k)
            return 0
        jax.lax.fori_loop(0, 3 * NCT, x_all, 0)
        w_stage_mxu()

        w_copy(2).start()
        wo_copy.start()
        with sc('w1wait'):
            w_piece(1, *W1[0], 4).wait()
        for i2 in range(8):
            w_pass1(0, 1, 0, i2)

        def wait_next2(jj):
            @pl.when(jj == 0)
            def _():
                w_piece(1, *W1[1], 5).wait()
            w_copy(2 * jj + 2).wait()

        def tile(jj, _):
            cw_stage(0, jnp.maximum(jj - 1, 0), jj + 1 < NCT, lambda: wait_next2(jj))

            @pl.when(jj + 1 < NCT)
            def _():
                w_copy(2 * jj + 3).start()
            cw_stage(1, 0, jj + 1 < NCT, lambda: w_copy(2 * jj + 3).wait())

            @pl.when(jj + 2 < NCT)
            def _():
                w_copy(2 * jj + 4).start()
            return 0
        jax.lax.fori_loop(0, NCT, tile, 0)

        GR = 8 * HOP
        wo_copy.wait()

        def o_copies(g, slot, fn):
            def cp(src_lo, n, b, dst_lo, k):
                return pltpu.make_async_copy(ost.at[slot, pl.ds(src_lo, n), :],
                                             o_hbm.at[b, pl.ds(dst_lo, n), :], osem.at[slot, k])
            gs = PITCH // GR

            @pl.when(g < gs)
            def _():
                fn(cp(0, 2 * GR, 0, pl.multiple_of(2 * GR * g, 16), 0))

            @pl.when(g == gs)
            def _():
                fn(cp(0, T - 2 * GR * gs, 0, 2 * GR * gs, 0))
                fn(cp(2 * (PITCH - GR * gs), 2 * (GR * (gs + 1) - PITCH), 1, 0, 1))

            @pl.when(jnp.logical_and(g > gs, g < NG - 1))
            def _():
                fn(cp(0, 2 * GR, 1, pl.multiple_of(2 * (GR * g - PITCH), 16), 0))

            @pl.when(g == NG - 1)
            def _():
                lo = 2 * (GR * (NG - 1) - PITCH)
                fn(cp(0, T - lo, 1, lo, 0))

        def o_body(g, _):
            slot = g % 2

            @pl.when(g >= 2)
            def _():
                o_copies(g - 2, slot, lambda c: c.wait())
            r0 = pl.multiple_of(g * GR, 8)
            z = jnp.concatenate([_unpack(xs[ct, pl.ds(r0, GR), :]) for ct in range(NCT)], axis=1)
            res = jnp.dot(z, wo_ref[...], preferred_element_type=jnp.float32)
            ost[slot] = res.astype(jnp.bfloat16)
            tasks = [lambda dep, h=h, k1=k1: y_pass_a(yh1, jnp.minimum(2 * g + 2 + h, 2 * NG - 1), h, k1, dep)
                     for h in range(2) for k1 in _PASS2]
            tasks += [lambda dep, h=h, i2=i2: y_pass_b(True, NCT - 1, g + 1, h, h, i2, dep)
                      for h in range(2) for i2 in range(8)]
            zero = zref[...]
            outs = []
            for n, t in enumerate(tasks):
                v = (n * (4 * 2 * HOP)) // len(tasks)
                col, row = divmod(v, 2 * HOP)
                bits = pltpu.bitcast(res[8 * row:8 * row + 8, 128 * col:128 * col + 128], jnp.uint32)
                if len(outs) >= CH:
                    bits = bits | outs[-CH]
                outs.append(t(bits & zero))
            o_copies(g, slot, lambda c: c.start())
            return 0
        with sc('O'):
            y_group(NCT - 1, 0)
            jax.lax.fori_loop(0, NG, o_body, 0, unroll=UO)
        with sc('owait'):
            for k in (NG - 2, NG - 1):
                o_copies(jnp.int32(k), k % 2, lambda c: c.wait())

    def f(x, w, w_o):
        lw, lx = _constants(K)
        vm = pl.BlockSpec(memory_space=pltpu.VMEM)
        anyspec = pl.BlockSpec(memory_space=pl.ANY)
        return pl.pallas_call(
            kernel,
            in_specs=[anyspec, anyspec, anyspec, vm, vm],
            out_specs=anyspec,
            out_shape=jax.ShapeDtypeStruct((B, T, D), jnp.bfloat16),
            scratch_shapes=[
                pltpu.VMEM((NCT, XROWS, 128), jnp.uint32),
                pltpu.VMEM((2, K, D, 128), jnp.bfloat16),
                pltpu.VMEM((NPROD, NCT, NG * 16, 128), jnp.bfloat16),
                pltpu.VMEM((NPROD, D, 128), jnp.bfloat16),
                pltpu.VMEM((NPROD, D, 128), jnp.bfloat16),
                pltpu.VMEM((NF, NG * 16, 128), jnp.float32),
                pltpu.VMEM((NF, NG * 16, 128), jnp.float32),
                pltpu.VMEM((HOP, NG * 16 + 16, 128), jnp.float32),
                pltpu.VMEM((2, 2, 8, 8, 8, 128), jnp.float32),
                pltpu.VMEM((2, 8, 8, 8, 128), jnp.float32),
                pltpu.VMEM((HOP, 8, 128), jnp.float32),
                pltpu.VMEM((8, 128), jnp.uint32),
                pltpu.VMEM((2, 16 * HOP, D), jnp.bfloat16),
                pltpu.VMEM((D, D), jnp.bfloat16),
                pltpu.SemaphoreType.DMA((NCT, 3, 2)),
                pltpu.SemaphoreType.DMA((2,)),
                pltpu.SemaphoreType.DMA((7,)),
                pltpu.SemaphoreType.DMA((2, 2)),
            ],
            compiler_params=pltpu.CompilerParams(vmem_limit_bytes=VMEM * 2**20),
        )(x, w, w_o, lw, lx)
    return jax.jit(f)


_kernel = make(UC=16)


@jax.jit
def pallas_standalone__autoregressive_conv_wavenet__speech_kernel(x, w, w_o):
    return _kernel(x, w, w_o)
```

```python
import contextlib
import jax
import jax.numpy as jnp
import numpy as np
from jax.experimental import pallas as pl
from jax.experimental.pallas import tpu as pltpu

NF = 64
HOP = 34
NPROD = 96


class _V:
    def __init__(self, a, s=1):
        self.a = a
        self.s = s


_Z = _V(None)


def _add(x, y):
    if x.a is None:
        return y
    if y.a is None:
        return x
    if x.s == y.s:
        return _V(x.a + y.a, x.s)
    return _V(x.a - y.a) if x.s > 0 else _V(y.a - x.a)


def _neg(x):
    return x if x.a is None else _V(x.a, -x.s)


def _sub(x, y):
    return _add(x, _neg(y))


def _mul(x, c):
    if x.a is None or c == 0:
        return _Z
    if c == 1:
        return x
    if c == -1:
        return _neg(x)
    return _V(x.a * float(c * x.s))


def _val(x, like=None):
    if x.a is None:
        return jnp.zeros_like(like)
    return x.a if x.s > 0 else -x.a


def _cadd(x, y):
    return (_add(x[0], y[0]), _add(x[1], y[1]))


def _csub(x, y):
    return (_sub(x[0], y[0]), _sub(x[1], y[1]))


def _conj(x):
    return (x[0], _neg(x[1]))


def _ctw(x, k, n):
    k %= n
    a, b = x
    if k == 0:
        return x
    if 4 * k == n:
        return (b, _neg(a))
    if 2 * k == n:
        return (_neg(a), _neg(b))
    if 4 * k == 3 * n:
        return (_neg(b), a)
    c, s = np.cos(2 * np.pi * k / n), -np.sin(2 * np.pi * k / n)
    if (8 * k) % n == 0:
        pa, pb = (a if c > 0 else _neg(a)), (b if c > 0 else _neg(b))
        qa, qb = (a if s > 0 else _neg(a)), (b if s > 0 else _neg(b))
        r = float(np.sqrt(0.5))
        return (_mul(_sub(pa, qb), r), _mul(_add(qa, pb), r))
    return (_sub(_mul(a, c), _mul(b, s)), _add(_mul(a, s), _mul(b, c)))


def _cdft(x):
    n = len(x)
    if n == 1:
        return list(x)
    if n == 2:
        return [_cadd(x[0], x[1]), _csub(x[0], x[1])]
    ev, o1, o3 = _cdft(x[0::2]), _cdft(x[1::4]), _cdft(x[3::4])
    out = [None] * n
    for k in range(n // 4):
        a, b = _ctw(o1[k], k, n), _ctw(o3[k], 3 * k, n)
        p, m = _cadd(a, b), _csub(a, b)
        mi = (m[1], _neg(m[0]))
        out[k], out[k + n // 2] = _cadd(ev[k], p), _csub(ev[k], p)
        out[k + n // 4], out[k + 3 * n // 4] = _cadd(ev[k + n // 4], mi), _csub(ev[k + n // 4], mi)
    return out


def _rdft(x):
    n = len(x)
    if n == 2:
        return {0: (_add(x[0], x[1]), _Z), 1: (_sub(x[0], x[1]), _Z)}
    h, q = n // 2, n // 4
    s = [_add(x[i], x[i + h]) for i in range(h)]
    d = [_sub(x[i], x[i + h]) for i in range(h)]
    out = {2 * k: v for k, v in _rdft(s).items()}
    u = _cdft([_ctw((d[i], _neg(d[i + q])), i, n) for i in range(q)])
    for k in range(q):
        out[4 * k + 1] = u[k]
    return out


def _pass1(i2, a, b, c, d):
    s1, s2, d1, d2 = _add(a, c), _add(b, d), _sub(a, c), _sub(b, d)
    r = float(np.sqrt(0.5))
    t1, t2 = _mul(d2, r), _mul(s2, r)
    g1 = (_add(a, t1), _neg(_add(c, t2)))
    g2 = (d1, _neg(d2))
    g3 = (_sub(a, t1), _sub(c, t2))
    out = [_add(s1, s2), _sub(s1, s2)]
    for k, g in ((1, g1), (2, g2), (3, g3)):
        out.extend(_ctw(g, i2 * k, NF))
    return out


def _pass2(k1, v):
    if k1 == 0:
        return {8 * k: x for k, x in _rdft([v(i, 0) for i in range(8)]).items()}
    if k1 == 4:
        g = [v(i, 1) for i in range(8)]
        u = _cdft([_ctw((g[i], _neg(g[i + 4])), i, 16) for i in range(4)])
        return {4 + 16 * k: u[k] for k in range(4)}
    k1, par = k1 % 8, k1 // 8
    x = [(lambda i=i: (v(i, 2 * k1), v(i, 2 * k1 + 1))) for i in range(8)]
    if par == 0:
        u = _cdft([_cadd(x[n](), x[n + 4]()) for n in range(4)])
    else:
        u = _cdft([_ctw(_csub(x[n](), x[n + 4]()), n, 8) for n in range(4)])
    return {k1 + 8 * (2 * k + par): u[k] for k in range(4)}


_PASS2 = (1, 9, 2, 10, 3, 11, 0, 4)


def _bin_keys():
    keys = sorted(k for k1 in (0, 1, 2, 3, 4, 9, 10, 11) for k in _pass2(k1, lambda i, j: _Z))
    rep = {}
    for k in keys:
        rep[k if k <= NF // 2 else NF - k] = k
    return [rep[k] for k in range(NF // 2 + 1)]


_REP = _bin_keys()


def _fwd_coef(q, nm):
    m = 4 * np.arange(nm) + q
    c = np.zeros((16, nm))
    c[0] = 1.0
    th8 = -2 * np.pi * 8 * m / NF
    c[1] = np.sin(th8) if q == 2 else np.cos(th8)
    for kp in range(1, 8):
        th = -2 * np.pi * kp * m / NF
        c[2 * kp] = np.cos(th)
        c[2 * kp + 1] = np.sin(th)
    return c


def _snap(c):
    return np.where(np.abs(c) < 1e-12, 0.0, c)


def _to_words(a):
    b = np.asarray(a, dtype=np.float32).astype(jnp.bfloat16).view(np.uint16).astype(np.uint32)
    return b[..., 0::2, :] | (b[..., 1::2, :] << 16)


def _constants(taps):
    lw, lx = [], []
    for q in range(4):
        cw = _fwd_coef(q, 8)
        for mp in range(8):
            if 4 * mp + q >= taps:
                cw[:, mp] = 0.0
        lw.append(np.kron(_snap(cw), np.eye(16)))
        lx.append(np.kron(_snap(_fwd_coef(q, 16)) * (2.0 / NF), np.eye(8)))
    return _to_words(np.stack(lw)), _to_words(np.stack(lx))


def _fwd_bins(T):
    t0 = [_V(T[q][0]) for q in range(4)]
    u0, u1 = _add(t0[0], t0[2]), _sub(t0[0], t0[2])
    v0, v1 = _add(t0[1], t0[3]), _sub(t0[1], t0[3])
    out = {0: (_add(u0, v0), _Z), 32: (_sub(u0, v0), _Z), 16: (u1, _neg(v1))}
    a0, a1, b2, a3 = (_V(T[q][1]) for q in range(4))
    s, d = _add(a1, a3), _sub(a3, a1)
    out[8] = (_add(a0, s), _add(b2, d))
    out[24] = (_sub(a0, s), _sub(d, b2))
    for kp in range(1, 8):
        t = [(_V(T[q][2 * kp]), _V(T[q][2 * kp + 1])) for q in range(4)]
        u0, u1 = _cadd(t[0], t[2]), _csub(t[0], t[2])
        v0, v1 = _cadd(t[1], t[3]), _csub(t[1], t[3])
        mi = (v1[1], _neg(v1[0]))
        out[kp] = _cadd(u0, v0)
        out[kp + 16] = _cadd(u1, mi)
        out[kp + 32] = _csub(u0, v0)
        out[kp + 48] = _csub(u1, mi)
    return out


def _rep_bin(bins, kappa):
    k = _REP[kappa]
    return bins[k] if k in bins else _conj(bins[NF - k])


def _operands(bins, is_w, like):
    ops = []
    for kappa in range(NF // 2):
        if kappa == 0:
            r0, r32 = bins[0][0], bins[NF // 2][0]
            forms = [_Z, r32, _neg(r0)] if is_w else [_Z, _mul(r32, 0.5), _mul(r0, 0.5)]
        else:
            re, im = _rep_bin(bins, kappa)
            forms = [re, _sub(im, re), _add(re, im)] if is_w else [_add(re, im), re, im]
        ops.extend(_val(v, like) for v in forms)
    return ops


def _icdft(x):
    return [_conj(v) for v in _cdft([_conj(v) for v in x])]


def _inv_pass_a(k1, y):
    if k1 == 0:
        (g0, _), (g4, _) = y(0), y(32)
        out = _inv_real8(g0, g4, y(8), y(16), _conj(y(40)), range(8))
        return {(i, 0): out[i] for i in range(8)}
    if k1 == 4:
        s = _icdft([y(4 + 16 * k) for k in range(4)])
        out = {}
        for i in range(4):
            re, im = _conj(_ctw(_conj(s[i]), i, 16))
            out[(i, 1)], out[(i + 4, 1)] = re, _neg(im)
        return out
    k1, par = k1 % 8, k1 // 8
    x = [y(k1 + 8 * k2) for k2 in range(8)]
    if par == 0:
        u = _icdft([_cadd(x[n], x[n + 4]) for n in range(4)])
    else:
        u = _icdft([_ctw(_csub(x[n], x[n + 4]), -n, 8) for n in range(4)])
    out = {}
    for k in range(4):
        out[(2 * k + par, 2 * k1)], out[(2 * k + par, 2 * k1 + 1)] = u[k]
    return out


def _inv_real8(g0, g4, t1, t2, t3, outs):
    r = float(np.sqrt(0.5))
    a, b = _add(g0, g4), _sub(g0, g4)
    p, s = _sub(t1[0], t3[0]), _add(t1[1], t3[1])
    base = [_add(a, t2[0]), _sub(b, t2[1]), _sub(a, t2[0]), _add(b, t2[1])]
    lazy = [lambda: _add(t1[0], t3[0]), lambda: _mul(_sub(p, s), r),
            lambda: _sub(t3[1], t1[1]), lambda: _neg(_mul(_add(s, p), r))]
    out, cache = {}, {}
    for i in outs:
        if i % 4 not in cache:
            cache[i % 4] = lazy[i % 4]()
        out[i] = _add(base[i % 4], cache[i % 4]) if i < 4 else _sub(base[i % 4], cache[i % 4])
    return out


def _inv_pass_b(i2, v):
    t = [_conj(_ctw(_conj((v[2 * k], v[2 * k + 1])), i2 * k, NF)) for k in (1, 2, 3)]
    outs = [i1 for i1 in range(8) if 8 * i1 + i2 >= NF - HOP]
    y = _inv_real8(v[0], v[1], t[0], t[1], t[2], outs)
    return {8 * i1 + i2 - (NF - HOP): y[i1] for i1 in outs}


def _rows16(v):
    return pltpu.bitcast(v, jnp.bfloat16).astype(jnp.float32)


def _unpack(v):
    return pltpu.bitcast(v, jnp.bfloat16)


def make(UW=8, UC=4, UY=5, UX=5, RC=400, scopes=False, WV=True, VMEM=100):
    sc = (lambda n: jax.named_scope(n)) if scopes else (lambda n: contextlib.nullcontext())
    B, T, D, K = 2, 4000, 512, 31
    NB = 60
    PITCH = NB * HOP
    TH = T // 2
    NG = B * NB // 8
    OFF = 32
    XROWS = 4392
    NCT = D // 128

    def kernel(x_hbm, w_hbm, wo_hbm, lw_ref, lx_ref, o_hbm,
               xs, wbuf, xh, wh0, wh1, yh0, yh1, tf, wtmp, ytmp, ztmp, zref, ost, wo_ref, xsem, wsem, psem, osem):
        whs = (wh0, wh1)
        xs_bf = xs.bitcast(jnp.bfloat16)
        wv = wbuf.bitcast(jnp.uint32)

        XP = (((0, 0, 1440),), ((0, 1440, TH), (1, 0, 720)), ((1, 720, TH),))

        def x_copies(ct, k):
            return [pltpu.make_async_copy(
                x_hbm.at[b, pl.ds(2 * lo, 2 * (hi - lo)), pl.ds(pl.multiple_of(ct * 128, 128), 128)],
                xs_bf.at[ct, pl.ds(2 * (OFF + b * PITCH + lo), 2 * (hi - lo)), :],
                xsem.at[ct, k, n]) for n, (b, lo, hi) in enumerate(XP[k])]

        def col_of(j):
            return (j % 2) * D + (j // 2) * 128

        def w_copy(j, ):
            return pltpu.make_async_copy(
                w_hbm.at[:, :, pl.ds(pl.multiple_of(col_of(j), 128), 128)],
                wbuf.at[j % 2], wsem.at[j % 2])

        def w_piece(j, lo, n, k):
            return pltpu.make_async_copy(
                w_hbm.at[:, pl.ds(lo, n), pl.ds(col_of(j), 128)],
                wbuf.at[j % 2, :, pl.ds(lo, n), :], psem.at[k])

        W1 = ((0, 272), (272, D - 272))
        wo_copy = pltpu.make_async_copy(wo_hbm, wo_ref, psem.at[6])

        with sc('pro0'):
            for ct in range(NCT):
                for k in range(3):
                    for c in x_copies(ct, k):
                        c.start()
            for k in range(4):
                w_piece(0, 128 * k, 128, k).start()
            for k, (lo, n) in enumerate(W1):
                w_piece(1, lo, n, 4 + k).start()

            for ct in range(NCT):
                xs[ct, 0:OFF, :] = jnp.zeros((OFF, 128), jnp.uint32)
                for b in range(B):
                    lo = OFF + b * PITCH + TH
                    hi = OFF + (b + 1) * PITCH if b + 1 < B else OFF + B * PITCH + 16
                    xs[ct, lo:hi, :] = jnp.zeros((hi - lo, 128), jnp.uint32)

        wh0[0] = jnp.zeros((D, 128), jnp.bfloat16)
        wh1[0] = jnp.zeros((D, 128), jnp.bfloat16)
        zref[...] = jnp.zeros((8, 128), jnp.uint32)
        ytmp[...] = jnp.zeros(ytmp.shape, jnp.float32)
        ztmp[...] = jnp.zeros(ztmp.shape, jnp.float32)


        def w_stage_mxu():
            def body(cg, _):
                r0 = pl.multiple_of(cg * 8, 8)
                Tq = []
                for q in range(4):
                    rows = [wv[0, min(4 * m + q, K - 1), pl.ds(r0, 8), :] for m in range(8)]
                    rhs = _unpack(jnp.concatenate(rows, axis=0))
                    res = jnp.dot(_unpack(lw_ref[q]), rhs, preferred_element_type=jnp.float32)
                    Tq.append([res[16 * j:16 * j + 16] for j in range(16)])
                ops = _operands(_fwd_bins(Tq), True, Tq[0][0])
                r1 = pl.multiple_of(cg * 16, 16)
                for p in range(NPROD):
                    wh0[p, pl.ds(r1, 16), :] = ops[p].astype(jnp.bfloat16)
                return 0
            def quarter(k, _):
                with sc('w0wait'):
                    w_piece(0, pl.multiple_of(k * 128, 128), 128, k).wait()
                for cg in range(8):
                    body(k * 8 + cg, 0)
                return 0
            with sc('W'):
                jax.lax.fori_loop(0, 4, quarter, 0)

        def w_pass1(cg, src, tb, i2, dep=None):
            r0 = pl.multiple_of(cg * 8, 8)
            words = [wv[src, i, pl.ds(r0, 8), :] if i < K else None for i in range(i2, 32, 8)]
            if dep is not None:
                words = [v if v is None else v | dep for v in words]
            rows = [None if v is None else _rows16(v) for v in words]
            for h in range(2):
                vals = _pass1(i2, *[_Z if v is None else _V(v[8 * h:8 * h + 8]) for v in rows])
                for j in range(8):
                    last = _val(vals[j])
                    wtmp[tb, h, i2, j] = last
            return pltpu.bitcast(last, jnp.uint32)

        def w_pass2(cg, whn, tb, k1, dep=None):
            forms = []

            def ld(h, i, j):
                v = wtmp[tb, h, i, j]
                if dep is not None and (i < 4 if DEP2 == 1 else DEP2 == 2):
                    v = pltpu.bitcast(pltpu.bitcast(v, jnp.uint32) | dep, jnp.float32)
                return _V(v)
            for h in range(2):
                bins = _pass2(k1, lambda i, j: ld(h, i, j))
                fh = {}
                for kappa in range(NF // 2 + 1):
                    if _REP[kappa] in bins:
                        re, im = bins[_REP[kappa]]
                        if kappa == 0:
                            fh[2] = _val(_neg(re))
                        elif kappa == NF // 2:
                            fh[1] = _val(re)
                        else:
                            fh[3 * kappa] = _val(re)
                            fh[3 * kappa + 1] = _val(_sub(im, re))
                            fh[3 * kappa + 2] = _val(_add(re, im))
                forms.append(fh)
            r1 = pl.multiple_of(cg * 16, 16)
            for p in forms[0]:
                both = jnp.concatenate([forms[0][p], forms[1][p]], axis=0)
                whn[p, pl.ds(r1, 16), :] = both.astype(jnp.bfloat16)
            return pltpu.bitcast(forms[1][p], jnp.uint32)

        def x_stage(ct, k):
            def body(g, _):
                base = g * (8 * HOP) + (OFF - 30)
                Tq = []
                for q in range(4):
                    xf = [_rows16(xs[ct, pl.ds(base + 4 * m + q, 8, stride=HOP), :]) for m in range(16)]
                    halves = []
                    for h in range(2):
                        rhs = jnp.concatenate([v[8 * h:8 * h + 8] for v in xf], axis=0).astype(jnp.bfloat16)
                        halves.append(jnp.dot(_unpack(lx_ref[q]), rhs, preferred_element_type=jnp.float32))
                    Tq.append([jnp.concatenate([halves[0][8 * j:8 * j + 8], halves[1][8 * j:8 * j + 8]], axis=0)
                               for j in range(16)])
                ops = _operands(_fwd_bins(Tq), False, Tq[0][0])
                r0 = pl.multiple_of(g * 16, 16)
                for p in range(NPROD):
                    xh[p, ct, pl.ds(r0, 16), :] = ops[p].astype(jnp.bfloat16)
                n = ct * NG + g
                yh1[n] = jnp.zeros((NG * 16, 128), jnp.float32)
                tf[jnp.minimum(n, HOP - 1)] = jnp.zeros((NG * 16 + 16, 128), jnp.float32)
                return 0
            with sc('X'):
                for gi in range(NG // 3):
                    body(k * (NG // 3) + gi, 0)

        def cw_stage(par, ct, has_next2, wait_next2):
            xhu = xh.bitcast(jnp.uint32)
            whc = whs[par].bitcast(jnp.uint32)
            whn = whs[1 - par]
            src = 1 - par
            yh, yprev = (yh0, yh1) if par == 0 else (yh1, yh0)
            is_g = par == 0

            def prod(p, r):
                lhs = jnp.concatenate([_unpack(xhu[p, ct, r // 2:(r + MC) // 2, :]) for ct in range(NCT)], axis=1)
                return jnp.dot(lhs, _unpack(whc[p]), preferred_element_type=jnp.float32)

            def w_tasks(b, tb):
                t2 = [lambda dep, k1=k1: w_pass2(b, whn, tb, k1, dep) for k1 in _PASS2]
                src1 = jnp.where(b == NF // 2 - 1, 1 - src, src)
                t1 = [lambda dep, i2=i2: w_pass1((b + 1) % (NF // 2), src1, 1 - tb, i2, dep) for i2 in range(8)]
                tw = [t for pair in zip(t2, t1) for t in pair]
                half_a = jnp.minimum(b, 2 * NG - 1)
                g_b = jnp.where(b == 0, NG, (b - 1) // 2)
                ya = [lambda dep, k1=k1: y_pass_a(yprev, half_a, tb, k1, dep) for k1 in _PASS2]
                yb = [lambda dep, i2=i2: y_pass_b(is_g, ct, g_b, 1 - tb, 1 - tb, i2, dep) for i2 in range(8)]
                ty = [t for pair in zip(yb, ya) for t in pair]
                return [t for pair in zip(tw, ty) for t in pair]

            def body(i, _):
                @pl.when(jnp.logical_and(i == (NF // 2) // UC - 1, has_next2))
                def _():
                    wait_next2()
                zero = zref[...]
                outs = []
                for u in range(UC):
                    b = i * UC + u
                    p = 3 * b
                    tasks = w_tasks(b, u % 2)
                    nv = 3 * NG * 2
                    state = [0, 0]

                    def seen(k):
                        for v in range(k.shape[0] // 8):
                            while state[1] < len(tasks) and state[0] >= (state[1] * nv) // len(tasks):
                                bits = pltpu.bitcast(k[8 * v:8 * v + 8], jnp.uint32)
                                if CH and len(outs) >= CH:
                                    bits = bits | outs[-CH]
                                outs.append(tasks[state[1]](bits & zero))
                                state[1] += 1
                            state[0] += 1
                        return k
                    for r in range(0, NG * 16, MC):
                        k1 = seen(prod(p, r))
                        yh[2 * b, r:r + MC, :] = k1 - seen(prod(p + 2, r))
                        yh[2 * b + 1, r:r + MC, :] = k1 + seen(prod(p + 1, r))
                return 0
            with sc('C%d' % par):
                jax.lax.fori_loop(0, (NF // 2) // UC, body, 0)

        def y_pass_a(yh, half, tb, k1, dep=None):
            r0 = pl.multiple_of(half * 8, 8)

            def ld(idx, use_dep):
                v = yh[idx, pl.ds(r0, 8), :]
                if dep is not None and use_dep:
                    v = pltpu.bitcast(pltpu.bitcast(v, jnp.uint32) | dep, jnp.float32)
                return _V(v)

            def y(k):
                lo = k % NF < NF // 2 and (k1 % 8 != 0 or k < 20)
                if k == 0 or k == NF // 2:
                    return (ld(k // 32, lo), _Z)
                kappa = _REP.index(k)
                return (ld(2 * kappa, lo), ld(2 * kappa + 1, lo))
            for (i2, j), v in _inv_pass_a(k1, y).items():
                last = _val(v)
                ytmp[tb, i2, j] = last
            return pltpu.bitcast(last, jnp.uint32)

        def y_pass_b(is_g, ct, g, h, tb, i2, dep=None):
            r0 = pl.multiple_of(g * 16 + 8 * h, 8)
            v = [ytmp[tb, i2, j] for j in range(8)]
            if dep is not None and DEPY:
                v = [x if (j < 2 and DEPY == 1) else pltpu.bitcast(pltpu.bitcast(x, jnp.uint32) | dep, jnp.float32)
                     for j, x in enumerate(v)]
            for t, hv in _inv_pass_b(i2, [_V(x) for x in v]).items():
                if not is_g:
                    z = 0.5 * jnp.tanh(_val(hv))
                    tf[t, pl.ds(r0, 8), :] = z
                    continue
                hf = tf[t, pl.ds(r0, 8), :]
                z = hf + hf * jnp.tanh(_val(_mul(hv, 0.5)))
                if h == 0:
                    ztmp[t] = z
                else:
                    both = jnp.concatenate([ztmp[t], z], axis=0).astype(jnp.bfloat16)
                    xs[ct, pl.ds(g * (8 * HOP) + t, 8, stride=HOP), :] = pltpu.bitcast(both, jnp.uint32)
            return pltpu.bitcast(z, jnp.uint32)

        def y_group(ct, g):
            for h in range(2):
                for k1 in _PASS2:
                    y_pass_a(yh1, 2 * g + h, h, k1)
            for h in range(2):
                for i2 in range(8):
                    y_pass_b(True, ct, g, h, h, i2)

        def x_all(i, _):
            ct, k = i // 3, i % 3
            with sc('xwait'):
                for kk in range(3):
                    @pl.when(k == kk)
                    def _():
                        for c in x_copies(ct, kk):
                            c.wait()
            x_stage(ct, k)
            return 0
        jax.lax.fori_loop(0, 3 * NCT, x_all, 0)
        for n in range(NCT * NG, NF):
            yh1[n] = jnp.zeros((NG * 16, 128), jnp.float32)
        w_stage_mxu()

        w_copy(2).start()
        wo_copy.start()
        with sc('w1wait'):
            w_piece(1, *W1[0], 4).wait()
        for i2 in range(8):
            w_pass1(0, 1, 0, i2)

        def wait_next2(jj):
            @pl.when(jj == 0)
            def _():
                w_piece(1, *W1[1], 5).wait()
            w_copy(2 * jj + 2).wait()

        def tile(jj, _):
            cw_stage(0, jnp.maximum(jj - 1, 0), jj + 1 < NCT, lambda: wait_next2(jj))

            @pl.when(jj + 1 < NCT)
            def _():
                w_copy(2 * jj + 3).start()
            cw_stage(1, 0, jj + 1 < NCT, lambda: w_copy(2 * jj + 3).wait())

            @pl.when(jj + 2 < NCT)
            def _():
                w_copy(2 * jj + 4).start()
            return 0
        jax.lax.fori_loop(0, NCT, tile, 0)

        GR = 8 * HOP
        wo_copy.wait()

        def o_copies(g, slot):
            def cp(src_lo, n, b, dst_lo, k):
                return pltpu.make_async_copy(ost.at[slot, pl.ds(src_lo, n), :],
                                             o_hbm.at[b, pl.ds(dst_lo, n), :], osem.at[slot, k])
            out = []
            for b in range(B):
                lo, hi = max(GR * g, PITCH * b), min(GR * (g + 1), PITCH * b + TH)
                if lo < hi:
                    out.append(cp(2 * (lo - GR * g), 2 * (hi - lo), b, 2 * (lo - PITCH * b), len(out)))
            return out

        def o_body(g, _):
            slot = g % 2

            if g >= 2:
                for c in o_copies(g - 2, slot):
                    c.wait()
            r0 = g * GR
            z = jnp.concatenate([_unpack(xs[ct, pl.ds(r0, GR), :]) for ct in range(NCT)], axis=1)
            res = jnp.dot(z, wo_ref[...], preferred_element_type=jnp.float32)
            ost[slot] = res.astype(jnp.bfloat16)
            tasks = [lambda dep, h=h, k1=k1: y_pass_a(yh1, 2 * g + 2 + h, h, k1, dep)
                     for h in range(2) for k1 in _PASS2]
            tasks += [lambda dep, h=h, i2=i2: y_pass_b(True, NCT - 1, g + 1, h, h, i2, dep)
                      for h in range(2) for i2 in range(8)]
            if g + 1 == NG:
                tasks = []
            zero = zref[...]
            outs = []
            for n, t in enumerate(tasks):
                v = (n * (4 * 2 * HOP)) // len(tasks)
                col, row = divmod(v, 2 * HOP)
                bits = pltpu.bitcast(res[8 * row:8 * row + 8, 128 * col:128 * col + 128], jnp.uint32)
                if len(outs) >= CH:
                    bits = bits | outs[-CH]
                outs.append(t(bits & zero))
            for c in o_copies(g, slot):
                c.start()
        with sc('O'):
            y_group(NCT - 1, 0)
            for g in range(NG):
                o_body(g, 0)
        with sc('owait'):
            for k in (NG - 2, NG - 1):
                for c in o_copies(k, k % 2):
                    c.wait()

    def f(x, w, w_o):
        lw, lx = _constants(K)
        vm = pl.BlockSpec(memory_space=pltpu.VMEM)
        anyspec = pl.BlockSpec(memory_space=pl.ANY)
        return pl.pallas_call(
            kernel,
            in_specs=[anyspec, anyspec, anyspec, vm, vm],
            out_specs=anyspec,
            out_shape=jax.ShapeDtypeStruct((B, T, D), jnp.bfloat16),
            scratch_shapes=[
                pltpu.VMEM((NCT, XROWS, 128), jnp.uint32),
                pltpu.VMEM((2, K, D, 128), jnp.bfloat16),
                pltpu.VMEM((NPROD, NCT, NG * 16, 128), jnp.bfloat16),
                pltpu.VMEM((NPROD, D, 128), jnp.bfloat16),
                pltpu.VMEM((NPROD, D, 128), jnp.bfloat16),
                pltpu.VMEM((NF, NG * 16, 128), jnp.float32),
                pltpu.VMEM((NF, NG * 16, 128), jnp.float32),
                pltpu.VMEM((HOP, NG * 16 + 16, 128), jnp.float32),
                pltpu.VMEM((2, 2, 8, 8, 8, 128), jnp.float32),
                pltpu.VMEM((2, 8, 8, 8, 128), jnp.float32),
                pltpu.VMEM((HOP, 8, 128), jnp.float32),
                pltpu.VMEM((8, 128), jnp.uint32),
                pltpu.VMEM((2, 16 * HOP, D), jnp.bfloat16),
                pltpu.VMEM((D, D), jnp.bfloat16),
                pltpu.SemaphoreType.DMA((NCT, 3, 2)),
                pltpu.SemaphoreType.DMA((2,)),
                pltpu.SemaphoreType.DMA((7,)),
                pltpu.SemaphoreType.DMA((2, 2)),
            ],
            compiler_params=pltpu.CompilerParams(vmem_limit_bytes=VMEM * 2**20),
        )(x, w, w_o, lw, lx)
    return jax.jit(f)


_kernel = make(UC=16)


@jax.jit
def pallas_standalone__autoregressive_conv_wavenet__speech_kernel(x, w, w_o):
    return _kernel(x, w, w_o)
```

```python
import contextlib
import jax
import jax.numpy as jnp
import numpy as np
from jax.experimental import pallas as pl
from jax.experimental.pallas import tpu as pltpu

NF = 64
HOP = 34
NPROD = 96


class _V:
    def __init__(self, a, s=1):
        self.a = a
        self.s = s


_Z = _V(None)


def _add(x, y):
    if x.a is None:
        return y
    if y.a is None:
        return x
    if x.s == y.s:
        return _V(x.a + y.a, x.s)
    return _V(x.a - y.a) if x.s > 0 else _V(y.a - x.a)


def _neg(x):
    return x if x.a is None else _V(x.a, -x.s)


def _sub(x, y):
    return _add(x, _neg(y))


def _mul(x, c):
    if x.a is None or c == 0:
        return _Z
    if c == 1:
        return x
    if c == -1:
        return _neg(x)
    return _V(x.a * float(c * x.s))


def _val(x, like=None):
    if x.a is None:
        return jnp.zeros_like(like)
    return x.a if x.s > 0 else -x.a


def _cadd(x, y):
    return (_add(x[0], y[0]), _add(x[1], y[1]))


def _csub(x, y):
    return (_sub(x[0], y[0]), _sub(x[1], y[1]))


def _conj(x):
    return (x[0], _neg(x[1]))


def _ctw(x, k, n):
    k %= n
    a, b = x
    if k == 0:
        return x
    if 4 * k == n:
        return (b, _neg(a))
    if 2 * k == n:
        return (_neg(a), _neg(b))
    if 4 * k == 3 * n:
        return (_neg(b), a)
    c, s = np.cos(2 * np.pi * k / n), -np.sin(2 * np.pi * k / n)
    if (8 * k) % n == 0:
        pa, pb = (a if c > 0 else _neg(a)), (b if c > 0 else _neg(b))
        qa, qb = (a if s > 0 else _neg(a)), (b if s > 0 else _neg(b))
        r = float(np.sqrt(0.5))
        return (_mul(_sub(pa, qb), r), _mul(_add(qa, pb), r))
    return (_sub(_mul(a, c), _mul(b, s)), _add(_mul(a, s), _mul(b, c)))


def _cdft(x):
    n = len(x)
    if n == 1:
        return list(x)
    if n == 2:
        return [_cadd(x[0], x[1]), _csub(x[0], x[1])]
    ev, o1, o3 = _cdft(x[0::2]), _cdft(x[1::4]), _cdft(x[3::4])
    out = [None] * n
    for k in range(n // 4):
        a, b = _ctw(o1[k], k, n), _ctw(o3[k], 3 * k, n)
        p, m = _cadd(a, b), _csub(a, b)
        mi = (m[1], _neg(m[0]))
        out[k], out[k + n // 2] = _cadd(ev[k], p), _csub(ev[k], p)
        out[k + n // 4], out[k + 3 * n // 4] = _cadd(ev[k + n // 4], mi), _csub(ev[k + n // 4], mi)
    return out


def _rdft(x):
    n = len(x)
    if n == 2:
        return {0: (_add(x[0], x[1]), _Z), 1: (_sub(x[0], x[1]), _Z)}
    h, q = n // 2, n // 4
    s = [_add(x[i], x[i + h]) for i in range(h)]
    d = [_sub(x[i], x[i + h]) for i in range(h)]
    out = {2 * k: v for k, v in _rdft(s).items()}
    u = _cdft([_ctw((d[i], _neg(d[i + q])), i, n) for i in range(q)])
    for k in range(q):
        out[4 * k + 1] = u[k]
    return out


def _pass1(i2, a, b, c, d):
    s1, s2, d1, d2 = _add(a, c), _add(b, d), _sub(a, c), _sub(b, d)
    r = float(np.sqrt(0.5))
    t1, t2 = _mul(d2, r), _mul(s2, r)
    g1 = (_add(a, t1), _neg(_add(c, t2)))
    g2 = (d1, _neg(d2))
    g3 = (_sub(a, t1), _sub(c, t2))
    out = [_add(s1, s2), _sub(s1, s2)]
    for k, g in ((1, g1), (2, g2), (3, g3)):
        out.extend(_ctw(g, i2 * k, NF))
    return out


def _pass2(k1, v):
    if k1 == 0:
        return {8 * k: x for k, x in _rdft([v(i, 0) for i in range(8)]).items()}
    if k1 == 4:
        g = [v(i, 1) for i in range(8)]
        u = _cdft([_ctw((g[i], _neg(g[i + 4])), i, 16) for i in range(4)])
        return {4 + 16 * k: u[k] for k in range(4)}
    k1, par = k1 % 8, k1 // 8
    x = [(lambda i=i: (v(i, 2 * k1), v(i, 2 * k1 + 1))) for i in range(8)]
    if par == 0:
        u = _cdft([_cadd(x[n](), x[n + 4]()) for n in range(4)])
    else:
        u = _cdft([_ctw(_csub(x[n](), x[n + 4]()), n, 8) for n in range(4)])
    return {k1 + 8 * (2 * k + par): u[k] for k in range(4)}


_PASS2 = (1, 9, 2, 10, 3, 11, 0, 4)


def _bin_keys():
    keys = sorted(k for k1 in (0, 1, 2, 3, 4, 9, 10, 11) for k in _pass2(k1, lambda i, j: _Z))
    rep = {}
    for k in keys:
        rep[k if k <= NF // 2 else NF - k] = k
    return [rep[k] for k in range(NF // 2 + 1)]


_REP = _bin_keys()


def _fwd_coef(q, nm):
    m = 4 * np.arange(nm) + q
    c = np.zeros((16, nm))
    c[0] = 1.0
    th8 = -2 * np.pi * 8 * m / NF
    c[1] = np.sin(th8) if q == 2 else np.cos(th8)
    for kp in range(1, 8):
        th = -2 * np.pi * kp * m / NF
        c[2 * kp] = np.cos(th)
        c[2 * kp + 1] = np.sin(th)
    return c


def _snap(c):
    return np.where(np.abs(c) < 1e-12, 0.0, c)


def _to_words(a):
    b = np.asarray(a, dtype=np.float32).astype(jnp.bfloat16).view(np.uint16).astype(np.uint32)
    return b[..., 0::2, :] | (b[..., 1::2, :] << 16)


def _constants(taps):
    lw, lx = [], []
    for q in range(4):
        cw = _fwd_coef(q, 8)
        for mp in range(8):
            if 4 * mp + q >= taps:
                cw[:, mp] = 0.0
        lw.append(np.kron(_snap(cw), np.eye(16)))
        lx.append(np.kron(_snap(_fwd_coef(q, 16)) * (2.0 / NF), np.eye(8)))
    return _to_words(np.stack(lw)), _to_words(np.stack(lx))


def _fwd_bins(T):
    t0 = [_V(T[q][0]) for q in range(4)]
    u0, u1 = _add(t0[0], t0[2]), _sub(t0[0], t0[2])
    v0, v1 = _add(t0[1], t0[3]), _sub(t0[1], t0[3])
    out = {0: (_add(u0, v0), _Z), 32: (_sub(u0, v0), _Z), 16: (u1, _neg(v1))}
    a0, a1, b2, a3 = (_V(T[q][1]) for q in range(4))
    s, d = _add(a1, a3), _sub(a3, a1)
    out[8] = (_add(a0, s), _add(b2, d))
    out[24] = (_sub(a0, s), _sub(d, b2))
    for kp in range(1, 8):
        t = [(_V(T[q][2 * kp]), _V(T[q][2 * kp + 1])) for q in range(4)]
        u0, u1 = _cadd(t[0], t[2]), _csub(t[0], t[2])
        v0, v1 = _cadd(t[1], t[3]), _csub(t[1], t[3])
        mi = (v1[1], _neg(v1[0]))
        out[kp] = _cadd(u0, v0)
        out[kp + 16] = _cadd(u1, mi)
        out[kp + 32] = _csub(u0, v0)
        out[kp + 48] = _csub(u1, mi)
    return out


def _rep_bin(bins, kappa):
    k = _REP[kappa]
    return bins[k] if k in bins else _conj(bins[NF - k])


def _operands(bins, is_w, like):
    ops = []
    for kappa in range(NF // 2):
        if kappa == 0:
            r0, r32 = bins[0][0], bins[NF // 2][0]
            forms = [_Z, r32, _neg(r0)] if is_w else [_Z, _mul(r32, 0.5), _mul(r0, 0.5)]
        else:
            re, im = _rep_bin(bins, kappa)
            forms = [re, _sub(im, re), _add(re, im)] if is_w else [_add(re, im), re, im]
        ops.extend(_val(v, like) for v in forms)
    return ops


def _icdft(x):
    return [_conj(v) for v in _cdft([_conj(v) for v in x])]


def _inv_pass_a(k1, y):
    if k1 == 0:
        (g0, _), (g4, _) = y(0), y(32)
        out = _inv_real8(g0, g4, y(8), y(16), _conj(y(40)), range(8))
        return {(i, 0): out[i] for i in range(8)}
    if k1 == 4:
        s = _icdft([y(4 + 16 * k) for k in range(4)])
        out = {}
        for i in range(4):
            re, im = _conj(_ctw(_conj(s[i]), i, 16))
            out[(i, 1)], out[(i + 4, 1)] = re, _neg(im)
        return out
    k1, par = k1 % 8, k1 // 8
    x = [y(k1 + 8 * k2) for k2 in range(8)]
    if par == 0:
        u = _icdft([_cadd(x[n], x[n + 4]) for n in range(4)])
    else:
        u = _icdft([_ctw(_csub(x[n], x[n + 4]), -n, 8) for n in range(4)])
    out = {}
    for k in range(4):
        out[(2 * k + par, 2 * k1)], out[(2 * k + par, 2 * k1 + 1)] = u[k]
    return out


def _inv_real8(g0, g4, t1, t2, t3, outs):
    r = float(np.sqrt(0.5))
    a, b = _add(g0, g4), _sub(g0, g4)
    p, s = _sub(t1[0], t3[0]), _add(t1[1], t3[1])
    base = [_add(a, t2[0]), _sub(b, t2[1]), _sub(a, t2[0]), _add(b, t2[1])]
    lazy = [lambda: _add(t1[0], t3[0]), lambda: _mul(_sub(p, s), r),
            lambda: _sub(t3[1], t1[1]), lambda: _neg(_mul(_add(s, p), r))]
    out, cache = {}, {}
    for i in outs:
        if i % 4 not in cache:
            cache[i % 4] = lazy[i % 4]()
        out[i] = _add(base[i % 4], cache[i % 4]) if i < 4 else _sub(base[i % 4], cache[i % 4])
    return out


def _inv_pass_b(i2, v):
    t = [_conj(_ctw(_conj((v[2 * k], v[2 * k + 1])), i2 * k, NF)) for k in (1, 2, 3)]
    outs = [i1 for i1 in range(8) if 8 * i1 + i2 >= NF - HOP]
    y = _inv_real8(v[0], v[1], t[0], t[1], t[2], outs)
    return {8 * i1 + i2 - (NF - HOP): y[i1] for i1 in outs}


def _rows16(v):
    return pltpu.bitcast(v, jnp.bfloat16).astype(jnp.float32)


def _unpack(v):
    return pltpu.bitcast(v, jnp.bfloat16)


def make(UW=8, UC=4, UY=5, UX=5, RC=400, scopes=False, WV=True, VMEM=112):
    sc = (lambda n: jax.named_scope(n)) if scopes else (lambda n: contextlib.nullcontext())
    B, T, D, K = 2, 4000, 512, 31
    NB = 60
    PITCH = NB * HOP
    TH = T // 2
    NG = B * NB // 8
    OFF = 32
    XROWS = 4392
    NCT = D // 128

    def kernel(x_hbm, w_hbm, wo_hbm, lw_ref, lx_ref, o_hbm,
               xs, wbuf, xh, wh0, wh1, yh0, yh1, tf, wtmp, ytmp, ztmp, zref, ost, wo_ref, xsem, wsem, psem, osem):
        whs = (wh0, wh1)
        xs_bf = xs.bitcast(jnp.bfloat16)
        wv = wbuf.bitcast(jnp.uint32)

        XP = (((0, 0, 1440),), ((0, 1440, TH), (1, 0, 720)), ((1, 720, TH),))

        def x_copies(ct, k):
            return [pltpu.make_async_copy(
                x_hbm.at[b, pl.ds(2 * lo, 2 * (hi - lo)), pl.ds(pl.multiple_of(ct * 128, 128), 128)],
                xs_bf.at[ct, pl.ds(2 * (OFF + b * PITCH + lo), 2 * (hi - lo)), :],
                xsem.at[ct, k, n]) for n, (b, lo, hi) in enumerate(XP[k])]

        def col_of(j):
            return (j % 2) * D + (j // 2) * 128

        def w_copy(j, ):
            return pltpu.make_async_copy(
                w_hbm.at[:, :, pl.ds(pl.multiple_of(col_of(j), 128), 128)],
                wbuf.at[j % 2], wsem.at[j % 2])

        def w_piece(j, lo, n, k):
            return pltpu.make_async_copy(
                w_hbm.at[:, pl.ds(lo, n), pl.ds(col_of(j), 128)],
                wbuf.at[j % 2, :, pl.ds(lo, n), :], psem.at[k])

        W1 = ((0, 272), (272, D - 272))
        wo_copy = pltpu.make_async_copy(wo_hbm, wo_ref, psem.at[6])

        with sc('pro0'):
            for ct in range(NCT):
                for k in range(3):
                    for c in x_copies(ct, k):
                        c.start()
            for k in range(4):
                w_piece(0, 128 * k, 128, k).start()
            for k, (lo, n) in enumerate(W1):
                w_piece(1, lo, n, 4 + k).start()

            for ct in range(NCT):
                xs[ct, 0:OFF, :] = jnp.zeros((OFF, 128), jnp.uint32)
                for b in range(B):
                    lo = OFF + b * PITCH + TH
                    hi = OFF + (b + 1) * PITCH if b + 1 < B else OFF + B * PITCH + 16
                    xs[ct, lo:hi, :] = jnp.zeros((hi - lo, 128), jnp.uint32)

        wh0[0] = jnp.zeros((D, 128), jnp.bfloat16)
        wh1[0] = jnp.zeros((D, 128), jnp.bfloat16)
        zref[...] = jnp.zeros((8, 128), jnp.uint32)
        ytmp[...] = jnp.zeros(ytmp.shape, jnp.float32)
        ztmp[...] = jnp.zeros(ztmp.shape, jnp.float32)


        def w_stage_mxu():
            def body(cg, _):
                r0 = pl.multiple_of(cg * 8, 8)
                Tq = []
                for q in range(4):
                    rows = [wv[0, min(4 * m + q, K - 1), pl.ds(r0, 8), :] for m in range(8)]
                    rhs = _unpack(jnp.concatenate(rows, axis=0))
                    res = jnp.dot(_unpack(lw_ref[q]), rhs, preferred_element_type=jnp.float32)
                    Tq.append([res[16 * j:16 * j + 16] for j in range(16)])
                ops = _operands(_fwd_bins(Tq), True, Tq[0][0])
                r1 = pl.multiple_of(cg * 16, 16)
                for p in range(NPROD):
                    wh0[p, pl.ds(r1, 16), :] = ops[p].astype(jnp.bfloat16)
                return 0
            def quarter(k, _):
                with sc('w0wait'):
                    w_piece(0, pl.multiple_of(k * 128, 128), 128, k).wait()
                for cg in range(8):
                    body(k * 8 + cg, 0)
                return 0
            with sc('W'):
                jax.lax.fori_loop(0, 4, quarter, 0)

        def w_pass1(cg, src, tb, i2, dep=None):
            r0 = pl.multiple_of(cg * 8, 8)
            words = [wv[src, i, pl.ds(r0, 8), :] if i < K else None for i in range(i2, 32, 8)]
            if dep is not None:
                words = [v if v is None else v | dep for v in words]
            rows = [None if v is None else _rows16(v) for v in words]
            for h in range(2):
                vals = _pass1(i2, *[_Z if v is None else _V(v[8 * h:8 * h + 8]) for v in rows])
                for j in range(8):
                    last = _val(vals[j])
                    wtmp[tb, h, i2, j] = last
            return pltpu.bitcast(last, jnp.uint32)

        def w_pass2(cg, whn, tb, k1, dep=None):
            forms = []

            def ld(h, i, j):
                v = wtmp[tb, h, i, j]
                if dep is not None and (i < 4 if DEP2 == 1 else DEP2 == 2):
                    v = pltpu.bitcast(pltpu.bitcast(v, jnp.uint32) | dep, jnp.float32)
                return _V(v)
            for h in range(2):
                bins = _pass2(k1, lambda i, j: ld(h, i, j))
                fh = {}
                for kappa in range(NF // 2 + 1):
                    if _REP[kappa] in bins:
                        re, im = bins[_REP[kappa]]
                        if kappa == 0:
                            fh[2] = _val(_neg(re))
                        elif kappa == NF // 2:
                            fh[1] = _val(re)
                        else:
                            fh[3 * kappa] = _val(re)
                            fh[3 * kappa + 1] = _val(_sub(im, re))
                            fh[3 * kappa + 2] = _val(_add(re, im))
                forms.append(fh)
            r1 = pl.multiple_of(cg * 16, 16)
            for p in forms[0]:
                both = jnp.concatenate([forms[0][p], forms[1][p]], axis=0)
                whn[p, pl.ds(r1, 16), :] = both.astype(jnp.bfloat16)
            return pltpu.bitcast(forms[1][p], jnp.uint32)

        def x_stage(ct, k):
            def body(g, _):
                base = g * (8 * HOP) + (OFF - 30)
                Tq = []
                for q in range(4):
                    xf = [_rows16(xs[ct, pl.ds(base + 4 * m + q, 8, stride=HOP), :]) for m in range(16)]
                    halves = []
                    for h in range(2):
                        rhs = jnp.concatenate([v[8 * h:8 * h + 8] for v in xf], axis=0).astype(jnp.bfloat16)
                        halves.append(jnp.dot(_unpack(lx_ref[q]), rhs, preferred_element_type=jnp.float32))
                    Tq.append([jnp.concatenate([halves[0][8 * j:8 * j + 8], halves[1][8 * j:8 * j + 8]], axis=0)
                               for j in range(16)])
                ops = _operands(_fwd_bins(Tq), False, Tq[0][0])
                r0 = pl.multiple_of(g * 16, 16)
                for p in range(NPROD):
                    xh[p, ct, pl.ds(r0, 16), :] = ops[p].astype(jnp.bfloat16)
                n = ct * NG + g
                yh1[n] = jnp.zeros((NG * 16, 128), jnp.float32)
                tf[jnp.minimum(n, HOP - 1)] = jnp.zeros((NG * 16 + 16, 128), jnp.float32)
                return 0
            with sc('X'):
                for gi in range(NG // 3):
                    body(k * (NG // 3) + gi, 0)

        def cw_stage(par, ct, has_next2, wait_next2):
            xhu = xh.bitcast(jnp.uint32)
            whc = whs[par].bitcast(jnp.uint32)
            whn = whs[1 - par]
            src = 1 - par
            yh, yprev = (yh0, yh1) if par == 0 else (yh1, yh0)
            is_g = par == 0

            def prod(p, r):
                lhs = jnp.concatenate([_unpack(xhu[p, ct, r // 2:(r + MC) // 2, :]) for ct in range(NCT)], axis=1)
                return jnp.dot(lhs, _unpack(whc[p]), preferred_element_type=jnp.float32)

            def w_tasks(b, tb):
                t2 = [lambda dep, k1=k1: w_pass2(b, whn, tb, k1, dep) for k1 in _PASS2]
                src1 = jnp.where(b == NF // 2 - 1, 1 - src, src)
                t1 = [lambda dep, i2=i2: w_pass1((b + 1) % (NF // 2), src1, 1 - tb, i2, dep) for i2 in range(8)]
                tw = [t for pair in zip(t2, t1) for t in pair]
                half_a = jnp.minimum(b, 2 * NG - 1)
                g_b = jnp.where(b == 0, NG, (b - 1) // 2)
                ya = [lambda dep, k1=k1: y_pass_a(yprev, half_a, tb, k1, dep) for k1 in _PASS2]
                yb = [lambda dep, i2=i2: y_pass_b(is_g, ct, g_b, 1 - tb, 1 - tb, i2, dep) for i2 in range(8)]
                ty = [t for pair in zip(yb, ya) for t in pair]
                return [t for pair in zip(tw, ty) for t in pair]

            def body(i, _):
                @pl.when(jnp.logical_and(i == (NF // 2) // UC - 1, has_next2))
                def _():
                    wait_next2()
                zero = zref[...]
                outs = []
                for u in range(UC):
                    b = i * UC + u
                    p = 3 * b
                    tasks = w_tasks(b, u % 2)
                    nv = 3 * NG * 2
                    state = [0, 0]

                    def seen(k):
                        for v in range(k.shape[0] // 8):
                            while state[1] < len(tasks) and state[0] >= (state[1] * nv) // len(tasks):
                                bits = pltpu.bitcast(k[8 * v:8 * v + 8], jnp.uint32)
                                if CH and len(outs) >= CH:
                                    bits = bits | outs[-CH]
                                outs.append(tasks[state[1]](bits & zero))
                                state[1] += 1
                            state[0] += 1
                        return k
                    for r in range(0, NG * 16, MC):
                        k1 = seen(prod(p, r))
                        yh[2 * b, r:r + MC, :] = k1 - seen(prod(p + 2, r))
                        yh[2 * b + 1, r:r + MC, :] = k1 + seen(prod(p + 1, r))
                return 0
            with sc('C%d' % par):
                jax.lax.fori_loop(0, (NF // 2) // UC, body, 0)

        def y_pass_a(yh, half, tb, k1, dep=None):
            r0 = pl.multiple_of(half * 8, 8)

            def ld(idx, use_dep):
                v = yh[idx, pl.ds(r0, 8), :]
                if dep is not None and use_dep:
                    v = pltpu.bitcast(pltpu.bitcast(v, jnp.uint32) | dep, jnp.float32)
                return _V(v)

            def y(k):
                lo = k % NF < NF // 2 and (k1 % 8 != 0 or k < 20)
                if k == 0 or k == NF // 2:
                    return (ld(k // 32, lo), _Z)
                kappa = _REP.index(k)
                return (ld(2 * kappa, lo), ld(2 * kappa + 1, lo))
            for (i2, j), v in _inv_pass_a(k1, y).items():
                last = _val(v)
                ytmp[tb, i2, j] = last
            return pltpu.bitcast(last, jnp.uint32)

        def y_pass_b(is_g, ct, g, h, tb, i2, dep=None):
            r0 = pl.multiple_of(g * 16 + 8 * h, 8)
            v = [ytmp[tb, i2, j] for j in range(8)]
            if dep is not None and DEPY:
                v = [x if (j < 2 and DEPY == 1) else pltpu.bitcast(pltpu.bitcast(x, jnp.uint32) | dep, jnp.float32)
                     for j, x in enumerate(v)]
            for t, hv in _inv_pass_b(i2, [_V(x) for x in v]).items():
                if not is_g:
                    z = 0.5 * jnp.tanh(_val(hv))
                    tf[t, pl.ds(r0, 8), :] = z
                    continue
                hf = tf[t, pl.ds(r0, 8), :]
                z = hf + hf * jnp.tanh(_val(_mul(hv, 0.5)))
                if h == 0:
                    ztmp[t] = z
                else:
                    both = jnp.concatenate([ztmp[t], z], axis=0).astype(jnp.bfloat16)
                    xs[ct, pl.ds(g * (8 * HOP) + t, 8, stride=HOP), :] = pltpu.bitcast(both, jnp.uint32)
            return pltpu.bitcast(z, jnp.uint32)

        def y_group(ct, g):
            for h in range(2):
                for k1 in _PASS2:
                    y_pass_a(yh1, 2 * g + h, h, k1)
            for h in range(2):
                for i2 in range(8):
                    y_pass_b(True, ct, g, h, h, i2)

        def x_all(i, _):
            ct, k = i // 3, i % 3
            with sc('xwait'):
                for kk in range(3):
                    @pl.when(k == kk)
                    def _():
                        for c in x_copies(ct, kk):
                            c.wait()
            x_stage(ct, k)
            return 0
        jax.lax.fori_loop(0, 3 * NCT, x_all, 0)
        for n in range(NCT * NG, NF):
            yh1[n] = jnp.zeros((NG * 16, 128), jnp.float32)
        w_stage_mxu()

        w_copy(2).start()
        wo_copy.start()
        with sc('w1wait'):
            w_piece(1, *W1[0], 4).wait()
        for i2 in range(8):
            w_pass1(0, 1, 0, i2)

        def wait_next2(jj):
            @pl.when(jj == 0)
            def _():
                w_piece(1, *W1[1], 5).wait()
            w_copy(2 * jj + 2).wait()

        def tile(jj, _):
            cw_stage(0, jnp.maximum(jj - 1, 0), jj + 1 < NCT, lambda: wait_next2(jj))

            @pl.when(jj + 1 < NCT)
            def _():
                w_copy(2 * jj + 3).start()
            cw_stage(1, 0, jj + 1 < NCT, lambda: w_copy(2 * jj + 3).wait())

            @pl.when(jj + 2 < NCT)
            def _():
                w_copy(2 * jj + 4).start()
            return 0
        jax.lax.fori_loop(0, NCT, tile, 0)

        GR = 8 * HOP
        wo_copy.wait()

        parts = []
        for g in range(NG):
            for b in range(B):
                lo, hi = max(GR * g, PITCH * b), min(GR * (g + 1), PITCH * b + TH)
                if lo < hi:
                    parts.append((g, lo, hi))
        g, lo, hi = parts.pop()
        parts += [(g, lo, hi - 88), (g, hi - 88, hi)]

        def o_copy(n):
            _, lo, hi = parts[n]
            b = lo // PITCH
            return pltpu.make_async_copy(ost.at[pl.ds(2 * lo, 2 * (hi - lo)), :],
                                         o_hbm.at[b, pl.ds(2 * (lo - PITCH * b), 2 * (hi - lo)), :], osem.at[n])

        def o_part(n):
            g, lo, hi = parts[n]
            z = jnp.concatenate([_unpack(xs[ct, lo:hi, :]) for ct in range(NCT)], axis=1)
            res = jnp.dot(z, wo_ref[...], preferred_element_type=jnp.float32)
            if n >= 1:
                o_copy(n - 1).start()
            ost[2 * lo:2 * hi, :] = res.astype(jnp.bfloat16)
            if g + 1 == NG or (n + 1 < len(parts) and parts[n + 1][0] == g):
                return
            tasks = [lambda dep, h=h, k1=k1: y_pass_a(yh1, 2 * g + 2 + h, h, k1, dep)
                     for h in range(2) for k1 in _PASS2]
            tasks += [lambda dep, h=h, i2=i2: y_pass_b(True, NCT - 1, g + 1, h, h, i2, dep)
                      for h in range(2) for i2 in range(8)]
            zero = zref[...]
            outs = []
            rows = (hi - lo) // 4
            for k, t in enumerate(tasks):
                col, row = divmod(int(k * 4 * rows * OF) // len(tasks), rows)
                bits = pltpu.bitcast(res[8 * row:8 * row + 8, 128 * col:128 * col + 128], jnp.uint32)
                if len(outs) >= CH:
                    bits = bits | outs[-CH]
                outs.append(t(bits & zero))

        with sc('O'):
            y_group(NCT - 1, 0)
            for n in range(len(parts)):
                o_part(n)
            o_copy(len(parts) - 1).start()
        with sc('owait'):
            for n in range(len(parts)):
                o_copy(n).wait()

    def f(x, w, w_o):
        lw, lx = _constants(K)
        vm = pl.BlockSpec(memory_space=pltpu.VMEM)
        anyspec = pl.BlockSpec(memory_space=pl.ANY)
        return pl.pallas_call(
            kernel,
            in_specs=[anyspec, anyspec, anyspec, vm, vm],
            out_specs=anyspec,
            out_shape=jax.ShapeDtypeStruct((B, T, D), jnp.bfloat16),
            scratch_shapes=[
                pltpu.VMEM((NCT, XROWS, 128), jnp.uint32),
                pltpu.VMEM((2, K, D, 128), jnp.bfloat16),
                pltpu.VMEM((NPROD, NCT, NG * 16, 128), jnp.bfloat16),
                pltpu.VMEM((NPROD, D, 128), jnp.bfloat16),
                pltpu.VMEM((NPROD, D, 128), jnp.bfloat16),
                pltpu.VMEM((NF, NG * 16, 128), jnp.float32),
                pltpu.VMEM((NF, NG * 16, 128), jnp.float32),
                pltpu.VMEM((HOP, NG * 16 + 16, 128), jnp.float32),
                pltpu.VMEM((2, 2, 8, 8, 8, 128), jnp.float32),
                pltpu.VMEM((2, 8, 8, 8, 128), jnp.float32),
                pltpu.VMEM((HOP, 8, 128), jnp.float32),
                pltpu.VMEM((8, 128), jnp.uint32),
                pltpu.VMEM((2 * B * PITCH, D), jnp.bfloat16),
                pltpu.VMEM((D, D), jnp.bfloat16),
                pltpu.SemaphoreType.DMA((NCT, 3, 2)),
                pltpu.SemaphoreType.DMA((2,)),
                pltpu.SemaphoreType.DMA((7,)),
                pltpu.SemaphoreType.DMA((NG + 2,)),
            ],
            compiler_params=pltpu.CompilerParams(vmem_limit_bytes=VMEM * 2**20),
        )(x, w, w_o, lw, lx)
    return jax.jit(f)


_kernel = make(UC=16)


@jax.jit
def pallas_standalone__autoregressive_conv_wavenet__speech_kernel(x, w, w_o):
    return _kernel(x, w, w_o)
```

```python
import jax
import jax.numpy as jnp
import numpy as np
from jax.experimental import pallas as pl
from jax.experimental.pallas import tpu as pltpu

NF = 64
HOP = 34
NPROD = 96
B, T, D, K = 2, 4000, 512, 31
TH = T // 2
NB = 60
PITCH = NB * HOP
NG = B * NB // 8
NR = NG * 16
GR = 8 * HOP
OFF = 32
XROWS = 4392
NCT = D // 128
UC = 16
CHAIN = 2


class _V:
    def __init__(self, a, s=1):
        self.a = a
        self.s = s


_Z = _V(None)


def _add(x, y):
    if x.a is None:
        return y
    if y.a is None:
        return x
    if x.s == y.s:
        return _V(x.a + y.a, x.s)
    return _V(x.a - y.a) if x.s > 0 else _V(y.a - x.a)


def _neg(x):
    return x if x.a is None else _V(x.a, -x.s)


def _sub(x, y):
    return _add(x, _neg(y))


def _mul(x, c):
    return _Z if x.a is None else _V(x.a * float(c * x.s))


def _val(x, like=None):
    if x.a is None:
        return jnp.zeros_like(like)
    return x.a if x.s > 0 else -x.a


def _cadd(x, y):
    return (_add(x[0], y[0]), _add(x[1], y[1]))


def _csub(x, y):
    return (_sub(x[0], y[0]), _sub(x[1], y[1]))


def _conj(x):
    return (x[0], _neg(x[1]))


def _ctw(x, k, n):
    k %= n
    a, b = x
    if k == 0:
        return x
    if 4 * k == n:
        return (b, _neg(a))
    if 2 * k == n:
        return (_neg(a), _neg(b))
    if 4 * k == 3 * n:
        return (_neg(b), a)
    c, s = np.cos(2 * np.pi * k / n), -np.sin(2 * np.pi * k / n)
    if (8 * k) % n == 0:
        pa, pb = (a if c > 0 else _neg(a)), (b if c > 0 else _neg(b))
        qa, qb = (a if s > 0 else _neg(a)), (b if s > 0 else _neg(b))
        r = float(np.sqrt(0.5))
        return (_mul(_sub(pa, qb), r), _mul(_add(qa, pb), r))
    return (_sub(_mul(a, c), _mul(b, s)), _add(_mul(a, s), _mul(b, c)))


def _cdft(x):
    n = len(x)
    if n == 1:
        return list(x)
    if n == 2:
        return [_cadd(x[0], x[1]), _csub(x[0], x[1])]
    ev, o1, o3 = _cdft(x[0::2]), _cdft(x[1::4]), _cdft(x[3::4])
    out = [None] * n
    for k in range(n // 4):
        a, b = _ctw(o1[k], k, n), _ctw(o3[k], 3 * k, n)
        p, m = _cadd(a, b), _csub(a, b)
        mi = (m[1], _neg(m[0]))
        out[k], out[k + n // 2] = _cadd(ev[k], p), _csub(ev[k], p)
        out[k + n // 4], out[k + 3 * n // 4] = _cadd(ev[k + n // 4], mi), _csub(ev[k + n // 4], mi)
    return out


def _icdft(x):
    return [_conj(v) for v in _cdft([_conj(v) for v in x])]


def _rdft(x):
    n = len(x)
    if n == 2:
        return {0: (_add(x[0], x[1]), _Z), 1: (_sub(x[0], x[1]), _Z)}
    h, q = n // 2, n // 4
    s = [_add(x[i], x[i + h]) for i in range(h)]
    d = [_sub(x[i], x[i + h]) for i in range(h)]
    out = {2 * k: v for k, v in _rdft(s).items()}
    u = _cdft([_ctw((d[i], _neg(d[i + q])), i, n) for i in range(q)])
    for k in range(q):
        out[4 * k + 1] = u[k]
    return out


def _fwd_pass1(i2, a, b, c, d):
    r = float(np.sqrt(0.5))
    s1, s2, d1, d2 = _add(a, c), _add(b, d), _sub(a, c), _sub(b, d)
    t1, t2 = _mul(d2, r), _mul(s2, r)
    g1 = (_add(a, t1), _neg(_add(c, t2)))
    g2 = (d1, _neg(d2))
    g3 = (_sub(a, t1), _sub(c, t2))
    out = [_add(s1, s2), _sub(s1, s2)]
    for k, g in ((1, g1), (2, g2), (3, g3)):
        out.extend(_ctw(g, i2 * k, NF))
    return out


def _fwd_pass2(cls, v):
    if cls == 0:
        return {8 * k: x for k, x in _rdft([v(i, 0) for i in range(8)]).items()}
    if cls == 4:
        g = [v(i, 1) for i in range(8)]
        u = _cdft([_ctw((g[i], _neg(g[i + 4])), i, 16) for i in range(4)])
        return {4 + 16 * k: u[k] for k in range(4)}
    k1, odd = cls % 8, cls // 8
    x = [(v(i, 2 * k1), v(i, 2 * k1 + 1)) for i in range(8)]
    if odd:
        u = _cdft([_ctw(_csub(x[n], x[n + 4]), n, 8) for n in range(4)])
    else:
        u = _cdft([_cadd(x[n], x[n + 4]) for n in range(4)])
    return {k1 + 8 * (2 * k + odd): u[k] for k in range(4)}


_CLASSES = (1, 9, 2, 10, 3, 11, 0, 4)


def _representatives():
    rep = {}
    for cls in _CLASSES:
        for k in _fwd_pass2(cls, lambda i, j: _Z):
            rep[min(k, NF - k)] = k
    return [rep[k] for k in range(NF // 2 + 1)]


_REP = _representatives()


def _gauss_forms(kappa, re, im, is_w):
    return [re, _sub(im, re), _add(re, im)] if is_w else [_add(re, im), re, im]


def _inv_real8(g0, g4, t1, t2, t3, outs):
    r = float(np.sqrt(0.5))
    a, b = _add(g0, g4), _sub(g0, g4)
    p, s = _sub(t1[0], t3[0]), _add(t1[1], t3[1])
    base = [_add(a, t2[0]), _sub(b, t2[1]), _sub(a, t2[0]), _add(b, t2[1])]
    lazy = [lambda: _add(t1[0], t3[0]), lambda: _mul(_sub(p, s), r),
            lambda: _sub(t3[1], t1[1]), lambda: _neg(_mul(_add(s, p), r))]
    out, cache = {}, {}
    for i in outs:
        if i % 4 not in cache:
            cache[i % 4] = lazy[i % 4]()
        out[i] = _add(base[i % 4], cache[i % 4]) if i < 4 else _sub(base[i % 4], cache[i % 4])
    return out


def _inv_pass_a(cls, y):
    if cls == 0:
        (g0, _), (g4, _) = y(0), y(32)
        out = _inv_real8(g0, g4, y(8), y(16), _conj(y(40)), range(8))
        return {(i, 0): out[i] for i in range(8)}
    if cls == 4:
        s = _icdft([y(4 + 16 * k) for k in range(4)])
        out = {}
        for i in range(4):
            re, im = _conj(_ctw(_conj(s[i]), i, 16))
            out[(i, 1)], out[(i + 4, 1)] = re, _neg(im)
        return out
    k1, odd = cls % 8, cls // 8
    x = [y(k1 + 8 * k2) for k2 in range(8)]
    if odd:
        u = _icdft([_ctw(_csub(x[n], x[n + 4]), -n, 8) for n in range(4)])
    else:
        u = _icdft([_cadd(x[n], x[n + 4]) for n in range(4)])
    out = {}
    for k in range(4):
        out[(2 * k + odd, 2 * k1)], out[(2 * k + odd, 2 * k1 + 1)] = u[k]
    return out


def _inv_pass_b(i2, v):
    t = [_conj(_ctw(_conj((v[2 * k], v[2 * k + 1])), i2 * k, NF)) for k in (1, 2, 3)]
    outs = [i1 for i1 in range(8) if 8 * i1 + i2 >= NF - HOP]
    y = _inv_real8(v[0], v[1], t[0], t[1], t[2], outs)
    return {8 * i1 + i2 - (NF - HOP): y[i1] for i1 in outs}


def _radix4_bins(tq):
    t0 = [_V(tq[q][0]) for q in range(4)]
    u0, u1 = _add(t0[0], t0[2]), _sub(t0[0], t0[2])
    v0, v1 = _add(t0[1], t0[3]), _sub(t0[1], t0[3])
    out = {0: (_add(u0, v0), _Z), 32: (_sub(u0, v0), _Z), 16: (u1, _neg(v1))}
    a0, a1, b2, a3 = (_V(tq[q][1]) for q in range(4))
    s, d = _add(a1, a3), _sub(a3, a1)
    out[8] = (_add(a0, s), _add(b2, d))
    out[24] = (_sub(a0, s), _sub(d, b2))
    for kp in range(1, 8):
        t = [(_V(tq[q][2 * kp]), _V(tq[q][2 * kp + 1])) for q in range(4)]
        u0, u1 = _cadd(t[0], t[2]), _csub(t[0], t[2])
        v0, v1 = _cadd(t[1], t[3]), _csub(t[1], t[3])
        mi = (v1[1], _neg(v1[0]))
        out[kp] = _cadd(u0, v0)
        out[kp + 16] = _cadd(u1, mi)
        out[kp + 32] = _csub(u0, v0)
        out[kp + 48] = _csub(u1, mi)
    return out


def _operands(bins, is_w, like):
    r0, r32 = bins[0][0], bins[NF // 2][0]
    ops = [_Z, r32, _neg(r0)] if is_w else [_Z, _mul(r32, 0.5), _mul(r0, 0.5)]
    for kappa in range(1, NF // 2):
        k = _REP[kappa]
        re, im = bins[k] if k in bins else _conj(bins[NF - k])
        ops.extend(_gauss_forms(kappa, re, im, is_w))
    return [_val(v, like) for v in ops]


def _sub_dft(q, nm, taps):
    n = 4 * np.arange(nm) + q
    c = np.zeros((16, nm))
    c[0] = 1.0
    th = -2 * np.pi * 8 * n / NF
    c[1] = np.sin(th) if q == 2 else np.cos(th)
    for kp in range(1, 8):
        th = -2 * np.pi * kp * n / NF
        c[2 * kp], c[2 * kp + 1] = np.cos(th), np.sin(th)
    c[:, n >= taps] = 0.0
    return np.where(np.abs(c) < 1e-12, 0.0, c)


def _as_words(a):
    b = np.asarray(a, dtype=np.float32).astype(jnp.bfloat16).view(np.uint16).astype(np.uint32)
    return b[..., 0::2, :] | (b[..., 1::2, :] << 16)


def _bf16(words):
    return pltpu.bitcast(words, jnp.bfloat16)


def _bits(v):
    return pltpu.bitcast(v, jnp.uint32)


def _after(v, dep):
    return v if dep is None else pltpu.bitcast(_bits(v) | dep, jnp.float32)


def _kernel(x_hbm, w_hbm, wo_hbm, lw_ref, lx_ref, o_hbm,
            xs, wbuf, xh, wh0, wh1, yh0, yh1, tf, wtmp, ytmp, ztmp, zref, ost, wo_ref,
            xsem, wsem, psem, osem):
    whs = (wh0, wh1)
    xs_bf = xs.bitcast(jnp.bfloat16)
    wv = wbuf.bitcast(jnp.uint32)

    x_parts = (((0, 0, 1440),), ((0, 1440, TH), (1, 0, 720)), ((1, 720, TH),))

    def x_copies(ct, k):
        return [pltpu.make_async_copy(
            x_hbm.at[b, pl.ds(2 * lo, 2 * (hi - lo)), pl.ds(pl.multiple_of(ct * 128, 128), 128)],
            xs_bf.at[ct, pl.ds(2 * (OFF + b * PITCH + lo), 2 * (hi - lo)), :],
            xsem.at[ct, k, n]) for n, (b, lo, hi) in enumerate(x_parts[k])]

    def col_of(j):
        return (j % 2) * D + (j // 2) * 128

    def w_copy(j):
        return pltpu.make_async_copy(
            w_hbm.at[:, :, pl.ds(pl.multiple_of(col_of(j), 128), 128)], wbuf.at[j % 2], wsem.at[j % 2])

    def w_part(j, lo, n, k):
        return pltpu.make_async_copy(
            w_hbm.at[:, pl.ds(lo, n), pl.ds(col_of(j), 128)], wbuf.at[j % 2, :, pl.ds(lo, n), :], psem.at[k])

    w1_parts = ((0, 16 * (UC + 1)), (16 * (UC + 1), D - 16 * (UC + 1)))
    wo_copy = pltpu.make_async_copy(wo_hbm, wo_ref, psem.at[6])

    for ct in range(NCT):
        for k in range(3):
            for c in x_copies(ct, k):
                c.start()
    for k in range(4):
        w_part(0, 128 * k, 128, k).start()
    for k, (lo, n) in enumerate(w1_parts):
        w_part(1, lo, n, 4 + k).start()

    for ct in range(NCT):
        xs[ct, 0:OFF, :] = jnp.zeros((OFF, 128), jnp.uint32)
        for b in range(B):
            lo = OFF + b * PITCH + TH
            hi = OFF + (b + 1) * PITCH + (16 if b == B - 1 else 0)
            xs[ct, lo:hi, :] = jnp.zeros((hi - lo, 128), jnp.uint32)
    wh0[0] = jnp.zeros((D, 128), jnp.bfloat16)
    wh1[0] = jnp.zeros((D, 128), jnp.bfloat16)
    zref[...] = jnp.zeros((8, 128), jnp.uint32)
    ytmp[...] = jnp.zeros(ytmp.shape, jnp.float32)
    ztmp[...] = jnp.zeros(ztmp.shape, jnp.float32)

    def x_group(ct, g):
        base = g * GR + (OFF - (K - 1))
        tq = []
        for q in range(4):
            rows = [_bf16(xs[ct, pl.ds(base + 4 * m + q, 8, stride=HOP), :]).astype(jnp.float32)
                    for m in range(16)]
            res = []
            for h in range(2):
                rhs = jnp.concatenate([v[8 * h:8 * h + 8] for v in rows], axis=0).astype(jnp.bfloat16)
                res.append(jnp.dot(_bf16(lx_ref[q]), rhs, preferred_element_type=jnp.float32))
            tq.append([jnp.concatenate([r[8 * j:8 * j + 8] for r in res], axis=0) for j in range(16)])
        ops = _operands(_radix4_bins(tq), False, tq[0][0])
        r0 = pl.multiple_of(g * 16, 16)
        for p in range(NPROD):
            xh[p, ct, pl.ds(r0, 16), :] = ops[p].astype(jnp.bfloat16)
        n = ct * NG + g
        yh1[n] = jnp.zeros((NR, 128), jnp.float32)
        tf[jnp.minimum(n, HOP - 1)] = jnp.zeros((NR + 16, 128), jnp.float32)

    def x_step(i, carry):
        ct, k = i // 3, i % 3
        for kk in range(3):
            @pl.when(k == kk)
            def _():
                for c in x_copies(ct, kk):
                    c.wait()
        for gi in range(NG // 3):
            x_group(ct, k * (NG // 3) + gi)
        return carry

    lax_loop = jax.lax.fori_loop
    lax_loop(0, 3 * NCT, x_step, 0)
    for n in range(NCT * NG, NF):
        yh1[n] = jnp.zeros((NR, 128), jnp.float32)

    def w_group_mxu(cg):
        r0 = pl.multiple_of(cg * 8, 8)
        tq = []
        for q in range(4):
            rhs = _bf16(jnp.concatenate(
                [wv[0, min(4 * m + q, K - 1), pl.ds(r0, 8), :] for m in range(8)], axis=0))
            res = jnp.dot(_bf16(lw_ref[q]), rhs, preferred_element_type=jnp.float32)
            tq.append([res[16 * j:16 * j + 16] for j in range(16)])
        ops = _operands(_radix4_bins(tq), True, tq[0][0])
        r1 = pl.multiple_of(cg * 16, 16)
        for p in range(NPROD):
            wh0[p, pl.ds(r1, 16), :] = ops[p].astype(jnp.bfloat16)

    def w_step_mxu(k, carry):
        w_part(0, pl.multiple_of(k * 128, 128), 128, k).wait()
        for cg in range(8):
            w_group_mxu(k * 8 + cg)
        return carry

    lax_loop(0, 4, w_step_mxu, 0)

    def w_pass1(cg, src, tb, i2, dep=None):
        r0 = pl.multiple_of(cg * 8, 8)
        words = [wv[src, i, pl.ds(r0, 8), :] if i < K else None for i in range(i2, 32, 8)]
        rows = [None if v is None else _bf16(v if dep is None else v | dep).astype(jnp.float32)
                for v in words]
        for h in range(2):
            vals = _fwd_pass1(i2, *[_Z if v is None else _V(v[8 * h:8 * h + 8]) for v in rows])
            for j in range(8):
                last = _val(vals[j])
                wtmp[tb, h, i2, j] = last
        return _bits(last)

    def w_pass2(cg, whn, tb, cls, dep=None):
        forms = []
        for h in range(2):
            bins = _fwd_pass2(cls, lambda i, j: _V(_after(wtmp[tb, h, i, j], dep if i < 4 else None)))
            fh = {}
            for kappa in range(NF // 2 + 1):
                if _REP[kappa] in bins:
                    re, im = bins[_REP[kappa]]
                    if kappa == 0:
                        fh[2] = _val(_neg(re))
                    elif kappa == NF // 2:
                        fh[1] = _val(re)
                    else:
                        for n, v in enumerate(_gauss_forms(kappa, re, im, True)):
                            fh[3 * kappa + n] = _val(v)
            forms.append(fh)
        r1 = pl.multiple_of(cg * 16, 16)
        for p in forms[0]:
            whn[p, pl.ds(r1, 16), :] = jnp.concatenate([forms[0][p], forms[1][p]], axis=0).astype(jnp.bfloat16)
        return _bits(forms[1][p])

    def y_pass_a(yh, half, tb, cls, dep=None):
        r0 = pl.multiple_of(half * 8, 8)

        def y(k):
            d = dep if k < NF // 2 and (cls % 8 != 0 or k < 20) else None
            if k % (NF // 2) == 0:
                return (_V(_after(yh[k // 32, pl.ds(r0, 8), :], d)), _Z)
            kappa = _REP.index(k)
            return (_V(_after(yh[2 * kappa, pl.ds(r0, 8), :], d)),
                    _V(_after(yh[2 * kappa + 1, pl.ds(r0, 8), :], d)))
        for (i2, j), v in _inv_pass_a(cls, y).items():
            last = _val(v)
            ytmp[tb, i2, j] = last
        return _bits(last)

    def y_pass_b(is_gate, ct, g, h, tb, i2, dep=None):
        r0 = pl.multiple_of(g * 16 + 8 * h, 8)
        v = [_V(_after(ytmp[tb, i2, j], dep if j >= 2 else None)) for j in range(8)]
        for t, hv in _inv_pass_b(i2, v).items():
            if not is_gate:
                z = 0.5 * jnp.tanh(_val(hv))
                tf[t, pl.ds(r0, 8), :] = z
                continue
            hf = tf[t, pl.ds(r0, 8), :]
            z = hf + hf * jnp.tanh(_val(_mul(hv, 0.5)))
            if h == 0:
                ztmp[t] = z
            else:
                both = jnp.concatenate([ztmp[t], z], axis=0).astype(jnp.bfloat16)
                xs[ct, pl.ds(g * GR + t, 8, stride=HOP), :] = _bits(both)
        return _bits(z)

    def release(tasks, results):
        zero = zref[...]
        outs = []
        for n, task in enumerate(tasks):
            dep = _bits(results[(n * len(results)) // len(tasks)])
            if n >= CHAIN:
                dep = dep | outs[n - CHAIN]
            outs.append(task(dep & zero))
        return outs

    def products(par, ct, wait_next):
        xhu = xh.bitcast(jnp.uint32)
        whc = whs[par].bitcast(jnp.uint32)
        whn, src = whs[1 - par], 1 - par
        yh, yprev = (yh0, yh1) if par == 0 else (yh1, yh0)

        def prod(p):
            lhs = jnp.concatenate([_bf16(xhu[p, ct_]) for ct_ in range(NCT)], axis=1)
            return jnp.dot(lhs, _bf16(whc[p]), preferred_element_type=jnp.float32)

        def tasks_of(b, tb):
            t2 = [lambda dep, c=c: w_pass2(b, whn, tb, c, dep) for c in _CLASSES]
            src1 = jnp.where(b == NF // 2 - 1, 1 - src, src)
            t1 = [lambda dep, i2=i2: w_pass1((b + 1) % (NF // 2), src1, 1 - tb, i2, dep) for i2 in range(8)]
            tw = [t for pair in zip(t2, t1) for t in pair]
            half_a = jnp.minimum(b, 2 * NG - 1)
            g_b = jnp.where(b == 0, NG, (b - 1) // 2)
            ya = [lambda dep, c=c: y_pass_a(yprev, half_a, tb, c, dep) for c in _CLASSES]
            yb = [lambda dep, i2=i2: y_pass_b(par == 0, ct, g_b, 1 - tb, 1 - tb, i2, dep) for i2 in range(8)]
            ty = [t for pair in zip(yb, ya) for t in pair]
            return [t for pair in zip(tw, ty) for t in pair]

        def body(i, carry):
            @pl.when(i == NF // 2 // UC - 1)
            def _():
                wait_next()
            zero = zref[...]
            outs = []
            for u in range(UC):
                b = i * UC + u
                tasks = tasks_of(b, u % 2)
                first = len(outs)
                seen = [0]

                def emit(k):
                    for v in range(k.shape[0] // 8):
                        while (len(outs) - first < len(tasks)
                               and seen[0] >= ((len(outs) - first) * 3 * NR // 8) // len(tasks)):
                            dep = _bits(k[8 * v:8 * v + 8])
                            if len(outs) >= CHAIN:
                                dep = dep | outs[-CHAIN]
                            outs.append(tasks[len(outs) - first](dep & zero))
                        seen[0] += 1
                    return k
                k1 = emit(prod(3 * b))
                yh[2 * b] = k1 - emit(prod(3 * b + 2))
                yh[2 * b + 1] = k1 + emit(prod(3 * b + 1))
            return carry

        lax_loop(0, NF // 2 // UC, body, 0)

    w_copy(2).start()
    w_part(1, *w1_parts[0], 4).wait()
    for i2 in range(8):
        w_pass1(0, 1, 0, i2)

    def wait_tile(j, more):
        @pl.when(more)
        def _():
            w_copy(j).wait()

    def wait_first(jj):
        @pl.when(jj == 0)
        def _():
            w_part(1, *w1_parts[1], 5).wait()
        wait_tile(2 * jj + 2, jj + 1 < NCT)

    def tile_pair(jj, carry):
        products(0, jnp.maximum(jj - 1, 0), lambda: wait_first(jj))

        @pl.when(jj + 1 < NCT)
        def _():
            w_copy(2 * jj + 3).start()
        products(1, 0, lambda: wait_tile(2 * jj + 3, jj + 1 < NCT))

        @pl.when(jj + 2 < NCT)
        def _():
            w_copy(2 * jj + 4).start()

        @pl.when(jj == 1)
        def _():
            wo_copy.start()
        return carry

    lax_loop(0, NCT, tile_pair, 0)

    parts = []
    for g in range(NG):
        for b in range(B):
            lo, hi = max(GR * g, PITCH * b), min(GR * (g + 1), PITCH * b + TH)
            if lo < hi:
                parts.append((g, lo, hi))
    g, lo, hi = parts.pop()
    parts += [(g, lo, hi - 88), (g, hi - 88, hi)]

    def o_copy(n):
        _, lo, hi = parts[n]
        b = lo // PITCH
        return pltpu.make_async_copy(
            ost.at[pl.ds(2 * lo, 2 * (hi - lo)), :],
            o_hbm.at[b, pl.ds(2 * (lo - PITCH * b), 2 * (hi - lo)), :], osem.at[n])

    def last_tasks(g):
        t = [lambda dep, h=h, c=c: y_pass_a(yh1, 2 * g + h, h, c, dep) for h in range(2) for c in _CLASSES]
        return t + [lambda dep, h=h, i2=i2: y_pass_b(True, NCT - 1, g, h, h, i2, dep)
                    for h in range(2) for i2 in range(8)]

    wo_copy.wait()
    for task in last_tasks(0):
        task(None)
    for n, (g, lo, hi) in enumerate(parts):
        z = jnp.concatenate([_bf16(xs[ct, lo:hi, :]) for ct in range(NCT)], axis=1)
        res = jnp.dot(z, wo_ref[...], preferred_element_type=jnp.float32)
        if n >= 1:
            o_copy(n - 1).start()
        ost[2 * lo:2 * hi, :] = res.astype(jnp.bfloat16)
        if g + 1 < NG and parts[n + 1][0] != g:
            rows = (hi - lo) // 4
            tiles = [res[8 * r:8 * r + 8, 128 * c:128 * c + 128] for c in range(NCT) for r in range(rows)]
            release(last_tasks(g + 1), tiles[:int(0.7 * len(tiles))])
    o_copy(len(parts) - 1).start()
    for n in range(len(parts)):
        o_copy(n).wait()


@jax.jit
def pallas_standalone__autoregressive_conv_wavenet__speech_kernel(x, w, w_o):
    lw = _as_words(np.stack([np.kron(_sub_dft(q, 8, K), np.eye(16)) for q in range(4)]))
    lx = _as_words(np.stack([np.kron(_sub_dft(q, 16, NF) * (2.0 / NF), np.eye(8)) for q in range(4)]))
    hbm = pl.BlockSpec(memory_space=pl.ANY)
    vmem = pl.BlockSpec(memory_space=pltpu.VMEM)
    f32, bf16, u32 = jnp.float32, jnp.bfloat16, jnp.uint32
    return pl.pallas_call(
        _kernel,
        in_specs=[hbm, hbm, hbm, vmem, vmem],
        out_specs=hbm,
        out_shape=jax.ShapeDtypeStruct((B, T, D), bf16),
        scratch_shapes=[
            pltpu.VMEM((NCT, XROWS, 128), u32),
            pltpu.VMEM((2, K, D, 128), bf16),
            pltpu.VMEM((NPROD, NCT, NR, 128), bf16),
            pltpu.VMEM((NPROD, D, 128), bf16),
            pltpu.VMEM((NPROD, D, 128), bf16),
            pltpu.VMEM((NF, NR, 128), f32),
            pltpu.VMEM((NF, NR, 128), f32),
            pltpu.VMEM((HOP, NR + 16, 128), f32),
            pltpu.VMEM((2, 2, 8, 8, 8, 128), f32),
            pltpu.VMEM((2, 8, 8, 8, 128), f32),
            pltpu.VMEM((HOP, 8, 128), f32),
            pltpu.VMEM((8, 128), u32),
            pltpu.VMEM((2 * B * PITCH, D), bf16),
            pltpu.VMEM((D, D), bf16),
            pltpu.SemaphoreType.DMA((NCT, 3, 2)),
            pltpu.SemaphoreType.DMA((2,)),
            pltpu.SemaphoreType.DMA((7,)),
            pltpu.SemaphoreType.DMA((NG + 2,)),
        ],
        compiler_params=pltpu.CompilerParams(vmem_limit_bytes=112 * 2**20),
    )(x, w, w_o, lw, lx)
```

```python
import jax
import jax.numpy as jnp
import numpy as np
from jax.experimental import pallas as pl
from jax.experimental.pallas import tpu as pltpu

NF = 64
HOP = 34
NPROD = 96
B, T, D, K = 2, 4000, 512, 31
TH = T // 2
NB = 60
PITCH = NB * HOP
NG = B * NB // 8
NR = NG * 16
GR = 8 * HOP
OFF = 32
XROWS = 4392
NCT = D // 128
UC = 16
CHAIN = 2


class _V:
    def __init__(self, a, s=1):
        self.a = a
        self.s = s


_Z = _V(None)


def _add(x, y):
    if x.a is None:
        return y
    if y.a is None:
        return x
    if x.s == y.s:
        return _V(x.a + y.a, x.s)
    return _V(x.a - y.a) if x.s > 0 else _V(y.a - x.a)


def _neg(x):
    return x if x.a is None else _V(x.a, -x.s)


def _sub(x, y):
    return _add(x, _neg(y))


def _mul(x, c):
    return _Z if x.a is None else _V(x.a * float(c * x.s))


def _val(x, like=None):
    if x.a is None:
        return jnp.zeros_like(like)
    return x.a if x.s > 0 else -x.a


def _cadd(x, y):
    return (_add(x[0], y[0]), _add(x[1], y[1]))


def _csub(x, y):
    return (_sub(x[0], y[0]), _sub(x[1], y[1]))


def _conj(x):
    return (x[0], _neg(x[1]))


def _ctw(x, k, n):
    k %= n
    a, b = x
    if k == 0:
        return x
    if 4 * k == n:
        return (b, _neg(a))
    if 2 * k == n:
        return (_neg(a), _neg(b))
    if 4 * k == 3 * n:
        return (_neg(b), a)
    c, s = np.cos(2 * np.pi * k / n), -np.sin(2 * np.pi * k / n)
    if (8 * k) % n == 0:
        pa, pb = (a if c > 0 else _neg(a)), (b if c > 0 else _neg(b))
        qa, qb = (a if s > 0 else _neg(a)), (b if s > 0 else _neg(b))
        r = float(np.sqrt(0.5))
        return (_mul(_sub(pa, qb), r), _mul(_add(qa, pb), r))
    return (_sub(_mul(a, c), _mul(b, s)), _add(_mul(a, s), _mul(b, c)))


def _cdft(x):
    n = len(x)
    if n == 1:
        return list(x)
    if n == 2:
        return [_cadd(x[0], x[1]), _csub(x[0], x[1])]
    ev, o1, o3 = _cdft(x[0::2]), _cdft(x[1::4]), _cdft(x[3::4])
    out = [None] * n
    for k in range(n // 4):
        a, b = _ctw(o1[k], k, n), _ctw(o3[k], 3 * k, n)
        p, m = _cadd(a, b), _csub(a, b)
        mi = (m[1], _neg(m[0]))
        out[k], out[k + n // 2] = _cadd(ev[k], p), _csub(ev[k], p)
        out[k + n // 4], out[k + 3 * n // 4] = _cadd(ev[k + n // 4], mi), _csub(ev[k + n // 4], mi)
    return out


def _icdft(x):
    return [_conj(v) for v in _cdft([_conj(v) for v in x])]


def _rdft(x):
    n = len(x)
    if n == 2:
        return {0: (_add(x[0], x[1]), _Z), 1: (_sub(x[0], x[1]), _Z)}
    h, q = n // 2, n // 4
    s = [_add(x[i], x[i + h]) for i in range(h)]
    d = [_sub(x[i], x[i + h]) for i in range(h)]
    out = {2 * k: v for k, v in _rdft(s).items()}
    u = _cdft([_ctw((d[i], _neg(d[i + q])), i, n) for i in range(q)])
    for k in range(q):
        out[4 * k + 1] = u[k]
    return out


def _fwd_pass1(i2, a, b, c, d):
    r = float(np.sqrt(0.5))
    s1, s2, d1, d2 = _add(a, c), _add(b, d), _sub(a, c), _sub(b, d)
    t1, t2 = _mul(d2, r), _mul(s2, r)
    g1 = (_add(a, t1), _neg(_add(c, t2)))
    g2 = (d1, _neg(d2))
    g3 = (_sub(a, t1), _sub(c, t2))
    out = [_add(s1, s2), _sub(s1, s2)]
    for k, g in ((1, g1), (2, g2), (3, g3)):
        out.extend(_ctw(g, i2 * k, NF))
    return out


def _fwd_pass2(cls, v):
    if cls == 0:
        return {8 * k: x for k, x in _rdft([v(i, 0) for i in range(8)]).items()}
    if cls == 4:
        g = [v(i, 1) for i in range(8)]
        u = _cdft([_ctw((g[i], _neg(g[i + 4])), i, 16) for i in range(4)])
        return {4 + 16 * k: u[k] for k in range(4)}
    k1, odd = cls % 8, cls // 8
    x = [(v(i, 2 * k1), v(i, 2 * k1 + 1)) for i in range(8)]
    if odd:
        u = _cdft([_ctw(_csub(x[n], x[n + 4]), n, 8) for n in range(4)])
    else:
        u = _cdft([_cadd(x[n], x[n + 4]) for n in range(4)])
    return {k1 + 8 * (2 * k + odd): u[k] for k in range(4)}


_CLASSES = (1, 9, 2, 10, 3, 11, 0, 4)


def _representatives():
    rep = {}
    for cls in _CLASSES:
        for k in _fwd_pass2(cls, lambda i, j: _Z):
            rep[min(k, NF - k)] = k
    return [rep[k] for k in range(NF // 2 + 1)]


_REP = _representatives()


def _gauss_forms(kappa, re, im, is_w):
    return [re, _sub(im, re), _add(re, im)] if is_w else [_add(re, im), re, im]


def _inv_real8(g0, g4, t1, t2, t3, outs):
    r = float(np.sqrt(0.5))
    a, b = _add(g0, g4), _sub(g0, g4)
    p, s = _sub(t1[0], t3[0]), _add(t1[1], t3[1])
    base = [_add(a, t2[0]), _sub(b, t2[1]), _sub(a, t2[0]), _add(b, t2[1])]
    lazy = [lambda: _add(t1[0], t3[0]), lambda: _mul(_sub(p, s), r),
            lambda: _sub(t3[1], t1[1]), lambda: _neg(_mul(_add(s, p), r))]
    out, cache = {}, {}
    for i in outs:
        if i % 4 not in cache:
            cache[i % 4] = lazy[i % 4]()
        out[i] = _add(base[i % 4], cache[i % 4]) if i < 4 else _sub(base[i % 4], cache[i % 4])
    return out


def _inv_pass_a(cls, y):
    if cls == 0:
        (g0, _), (g4, _) = y(0), y(32)
        out = _inv_real8(g0, g4, y(8), y(16), _conj(y(40)), range(8))
        return {(i, 0): out[i] for i in range(8)}
    if cls == 4:
        s = _icdft([y(4 + 16 * k) for k in range(4)])
        out = {}
        for i in range(4):
            re, im = _conj(_ctw(_conj(s[i]), i, 16))
            out[(i, 1)], out[(i + 4, 1)] = re, _neg(im)
        return out
    k1, odd = cls % 8, cls // 8
    x = [y(k1 + 8 * k2) for k2 in range(8)]
    if odd:
        u = _icdft([_ctw(_csub(x[n], x[n + 4]), -n, 8) for n in range(4)])
    else:
        u = _icdft([_cadd(x[n], x[n + 4]) for n in range(4)])
    out = {}
    for k in range(4):
        out[(2 * k + odd, 2 * k1)], out[(2 * k + odd, 2 * k1 + 1)] = u[k]
    return out


def _inv_pass_b(i2, v):
    t = [_conj(_ctw(_conj((v[2 * k], v[2 * k + 1])), i2 * k, NF)) for k in (1, 2, 3)]
    outs = [i1 for i1 in range(8) if 8 * i1 + i2 >= NF - HOP]
    y = _inv_real8(v[0], v[1], t[0], t[1], t[2], outs)
    return {8 * i1 + i2 - (NF - HOP): y[i1] for i1 in outs}


def _radix4_bins(tq):
    t0 = [_V(tq[q][0]) for q in range(4)]
    u0, u1 = _add(t0[0], t0[2]), _sub(t0[0], t0[2])
    v0, v1 = _add(t0[1], t0[3]), _sub(t0[1], t0[3])
    out = {0: (_add(u0, v0), _Z), 32: (_sub(u0, v0), _Z), 16: (u1, _neg(v1))}
    a0, a1, b2, a3 = (_V(tq[q][1]) for q in range(4))
    s, d = _add(a1, a3), _sub(a3, a1)
    out[8] = (_add(a0, s), _add(b2, d))
    out[24] = (_sub(a0, s), _sub(d, b2))
    for kp in range(1, 8):
        t = [(_V(tq[q][2 * kp]), _V(tq[q][2 * kp + 1])) for q in range(4)]
        u0, u1 = _cadd(t[0], t[2]), _csub(t[0], t[2])
        v0, v1 = _cadd(t[1], t[3]), _csub(t[1], t[3])
        mi = (v1[1], _neg(v1[0]))
        out[kp] = _cadd(u0, v0)
        out[kp + 16] = _cadd(u1, mi)
        out[kp + 32] = _csub(u0, v0)
        out[kp + 48] = _csub(u1, mi)
    return out


def _operands(bins, is_w, like):
    r0, r32 = bins[0][0], bins[NF // 2][0]
    ops = [_Z, r32, _neg(r0)] if is_w else [_Z, _mul(r32, 0.5), _mul(r0, 0.5)]
    for kappa in range(1, NF // 2):
        k = _REP[kappa]
        re, im = bins[k] if k in bins else _conj(bins[NF - k])
        ops.extend(_gauss_forms(kappa, re, im, is_w))
    return [_val(v, like) for v in ops]


def _sub_dft(q, nm, taps):
    n = 4 * np.arange(nm) + q
    c = np.zeros((16, nm))
    c[0] = 1.0
    th = -2 * np.pi * 8 * n / NF
    c[1] = np.sin(th) if q == 2 else np.cos(th)
    for kp in range(1, 8):
        th = -2 * np.pi * kp * n / NF
        c[2 * kp], c[2 * kp + 1] = np.cos(th), np.sin(th)
    c[:, n >= taps] = 0.0
    return np.where(np.abs(c) < 1e-12, 0.0, c)


def _bf16(words):
    return pltpu.bitcast(words, jnp.bfloat16)


def _bits(v):
    return pltpu.bitcast(v, jnp.uint32)


def _after(v, dep):
    return v if dep is None else pltpu.bitcast(_bits(v) | dep, jnp.float32)


def _kernel(x_hbm, w_hbm, wo_hbm, coef_ref, o_hbm,
            xs, wbuf, xh, wh0, wh1, yh0, yh1, tf, wtmp, ytmp, ztmp, zref, ost, wo_ref, lw_bf, lx_bf,
            xsem, wsem, psem, osem):
    whs = (wh0, wh1)
    xs_bf = xs.bitcast(jnp.bfloat16)
    wv = wbuf.bitcast(jnp.uint32)
    lw_ref, lx_ref = lw_bf.bitcast(jnp.uint32), lx_bf.bitcast(jnp.uint32)

    x_parts = (((0, 0, 1440),), ((0, 1440, TH), (1, 0, 720)), ((1, 720, TH),))

    def x_copies(ct, k):
        return [pltpu.make_async_copy(
            x_hbm.at[b, pl.ds(2 * lo, 2 * (hi - lo)), pl.ds(pl.multiple_of(ct * 128, 128), 128)],
            xs_bf.at[ct, pl.ds(2 * (OFF + b * PITCH + lo), 2 * (hi - lo)), :],
            xsem.at[ct, k, n]) for n, (b, lo, hi) in enumerate(x_parts[k])]

    def col_of(j):
        return (j % 2) * D + (j // 2) * 128

    def w_copy(j, rest):
        lo, n = (16, D - 16) if rest else (0, 16)
        return pltpu.make_async_copy(
            w_hbm.at[:, pl.ds(lo, n), pl.ds(pl.multiple_of(col_of(j), 128), 128)],
            wbuf.at[j % 2, :, pl.ds(lo, n), :], wsem.at[j % 2, int(rest)])

    def w_start(j):
        w_copy(j, False).start()
        w_copy(j, True).start()

    def w_part(j, lo, n, k):
        return pltpu.make_async_copy(
            w_hbm.at[:, pl.ds(lo, n), pl.ds(col_of(j), 128)], wbuf.at[j % 2, :, pl.ds(lo, n), :], psem.at[k])

    w1_parts = ((0, 16 * (UC + 1)), (16 * (UC + 1), D - 16 * (UC + 1)))
    wo_copy = pltpu.make_async_copy(wo_hbm, wo_ref, psem.at[6])

    for ct in range(NCT):
        for k in range(3):
            for c in x_copies(ct, k):
                c.start()
    for k in range(4):
        w_part(0, 128 * k, 128, k).start()
    for k, (lo, n) in enumerate(w1_parts):
        w_part(1, lo, n, 4 + k).start()

    for first, rep, dst in ((0, 8, lx_bf), (4, 16, lw_bf)):
        shape = (16 * rep, 128)
        diag = (jax.lax.broadcasted_iota(jnp.int32, shape, 0) % rep
                == jax.lax.broadcasted_iota(jnp.int32, shape, 1) % rep)
        for q in range(4):
            c = coef_ref[first + q]
            full = jnp.concatenate([jnp.broadcast_to(c[j:j + 1], (rep, 128)) for j in range(16)], axis=0)
            dst[q] = jnp.where(diag, full, 0.0).astype(jnp.bfloat16)

    for ct in range(NCT):
        xs[ct, 0:OFF, :] = jnp.zeros((OFF, 128), jnp.uint32)
        for b in range(B):
            lo = OFF + b * PITCH + TH
            hi = OFF + (b + 1) * PITCH + (16 if b == B - 1 else 0)
            xs[ct, lo:hi, :] = jnp.zeros((hi - lo, 128), jnp.uint32)
    wh0[0] = jnp.zeros((D, 128), jnp.bfloat16)
    wh1[0] = jnp.zeros((D, 128), jnp.bfloat16)
    zref[...] = jnp.zeros((8, 128), jnp.uint32)
    ytmp[...] = jnp.zeros(ytmp.shape, jnp.float32)
    ztmp[...] = jnp.zeros(ztmp.shape, jnp.float32)

    def x_group(ct, g):
        base = g * GR + (OFF - (K - 1))
        tq = []
        for q in range(4):
            rows = [_bf16(xs[ct, pl.ds(base + 4 * m + q, 8, stride=HOP), :]).astype(jnp.float32)
                    for m in range(16)]
            res = []
            for h in range(2):
                rhs = jnp.concatenate([v[8 * h:8 * h + 8] for v in rows], axis=0).astype(jnp.bfloat16)
                res.append(jnp.dot(_bf16(lx_ref[q]), rhs, preferred_element_type=jnp.float32))
            tq.append([jnp.concatenate([r[8 * j:8 * j + 8] for r in res], axis=0) for j in range(16)])
        ops = _operands(_radix4_bins(tq), False, tq[0][0])
        r0 = pl.multiple_of(g * 16, 16)
        for p in range(NPROD):
            xh[p, ct, pl.ds(r0, 16), :] = ops[p].astype(jnp.bfloat16)
        n = ct * NG + g
        yh1[n] = jnp.zeros((NR, 128), jnp.float32)
        tf[jnp.minimum(n, HOP - 1)] = jnp.zeros((NR + 16, 128), jnp.float32)

    def x_step(i, carry):
        ct, k = i // 3, i % 3
        for kk in range(3):
            @pl.when(k == kk)
            def _():
                for c in x_copies(ct, kk):
                    c.wait()
        for gi in range(NG // 3):
            x_group(ct, k * (NG // 3) + gi)
        return carry

    lax_loop = jax.lax.fori_loop
    lax_loop(0, 3 * NCT, x_step, 0)
    for n in range(NCT * NG, NF):
        yh1[n] = jnp.zeros((NR, 128), jnp.float32)

    def w_group_mxu(cg):
        r0 = pl.multiple_of(cg * 8, 8)
        tq = []
        for q in range(4):
            rhs = _bf16(jnp.concatenate(
                [wv[0, min(4 * m + q, K - 1), pl.ds(r0, 8), :] for m in range(8)], axis=0))
            res = jnp.dot(_bf16(lw_ref[q]), rhs, preferred_element_type=jnp.float32)
            tq.append([res[16 * j:16 * j + 16] for j in range(16)])
        ops = _operands(_radix4_bins(tq), True, tq[0][0])
        r1 = pl.multiple_of(cg * 16, 16)
        for p in range(NPROD):
            wh0[p, pl.ds(r1, 16), :] = ops[p].astype(jnp.bfloat16)

    def w_step_mxu(k, carry):
        w_part(0, pl.multiple_of(k * 128, 128), 128, k).wait()
        for cg in range(8):
            w_group_mxu(k * 8 + cg)
        return carry

    lax_loop(0, 4, w_step_mxu, 0)

    def w_pass1(cg, src, tb, i2, dep=None):
        r0 = pl.multiple_of(cg * 8, 8)
        words = [wv[src, i, pl.ds(r0, 8), :] if i < K else None for i in range(i2, 32, 8)]
        rows = [None if v is None else _bf16(v if dep is None else v | dep).astype(jnp.float32)
                for v in words]
        for h in range(2):
            vals = _fwd_pass1(i2, *[_Z if v is None else _V(v[8 * h:8 * h + 8]) for v in rows])
            for j in range(8):
                last = _val(vals[j])
                wtmp[tb, h, i2, j] = last
        return _bits(last)

    def w_pass2(cg, whn, tb, cls, dep=None):
        forms = []
        for h in range(2):
            bins = _fwd_pass2(cls, lambda i, j: _V(_after(wtmp[tb, h, i, j], dep if i < 4 else None)))
            fh = {}
            for kappa in range(NF // 2 + 1):
                if _REP[kappa] in bins:
                    re, im = bins[_REP[kappa]]
                    if kappa == 0:
                        fh[2] = _val(_neg(re))
                    elif kappa == NF // 2:
                        fh[1] = _val(re)
                    else:
                        for n, v in enumerate(_gauss_forms(kappa, re, im, True)):
                            fh[3 * kappa + n] = _val(v)
            forms.append(fh)
        r1 = pl.multiple_of(cg * 16, 16)
        for p in forms[0]:
            whn[p, pl.ds(r1, 16), :] = jnp.concatenate([forms[0][p], forms[1][p]], axis=0).astype(jnp.bfloat16)
        return _bits(forms[1][p])

    def y_pass_a(yh, half, tb, cls, dep=None):
        r0 = pl.multiple_of(half * 8, 8)

        def y(k):
            d = dep if k < NF // 2 and (cls % 8 != 0 or k < 20) else None
            if k % (NF // 2) == 0:
                return (_V(_after(yh[k // 32, pl.ds(r0, 8), :], d)), _Z)
            kappa = _REP.index(k)
            return (_V(_after(yh[2 * kappa, pl.ds(r0, 8), :], d)),
                    _V(_after(yh[2 * kappa + 1, pl.ds(r0, 8), :], d)))
        for (i2, j), v in _inv_pass_a(cls, y).items():
            last = _val(v)
            ytmp[tb, i2, j] = last
        return _bits(last)

    def y_pass_b(is_gate, ct, g, h, tb, i2, dep=None):
        r0 = pl.multiple_of(g * 16 + 8 * h, 8)
        v = [_V(_after(ytmp[tb, i2, j], dep if j >= 2 else None)) for j in range(8)]
        for t, hv in _inv_pass_b(i2, v).items():
            if not is_gate:
                z = 0.5 * jnp.tanh(_val(hv))
                tf[t, pl.ds(r0, 8), :] = z
                continue
            hf = tf[t, pl.ds(r0, 8), :]
            z = hf + hf * jnp.tanh(_val(_mul(hv, 0.5)))
            if h == 0:
                ztmp[t] = z
            else:
                both = jnp.concatenate([ztmp[t], z], axis=0).astype(jnp.bfloat16)
                xs[ct, pl.ds(g * GR + t, 8, stride=HOP), :] = _bits(both)
        return _bits(z)

    def release(tasks, results):
        zero = zref[...]
        outs = []
        for n, task in enumerate(tasks):
            dep = _bits(results[(n * len(results)) // len(tasks)])
            if n >= CHAIN:
                dep = dep | outs[n - CHAIN]
            outs.append(task(dep & zero))
        return outs

    def products(par, ct, wait_next):
        xhu = xh.bitcast(jnp.uint32)
        whc = whs[par].bitcast(jnp.uint32)
        whn, src = whs[1 - par], 1 - par
        yh, yprev = (yh0, yh1) if par == 0 else (yh1, yh0)

        def prod(p):
            lhs = jnp.concatenate([_bf16(xhu[p, ct_]) for ct_ in range(NCT)], axis=1)
            return jnp.dot(lhs, _bf16(whc[p]), preferred_element_type=jnp.float32)

        def tasks_of(b, tb):
            t2 = [lambda dep, c=c: w_pass2(b, whn, tb, c, dep) for c in _CLASSES]
            src1 = jnp.where(b == NF // 2 - 1, 1 - src, src)
            t1 = [lambda dep, i2=i2: w_pass1((b + 1) % (NF // 2), src1, 1 - tb, i2, dep) for i2 in range(8)]
            tw = [t for pair in zip(t2, t1) for t in pair]
            half_a = jnp.minimum(b, 2 * NG - 1)
            g_b = jnp.where(b == 0, NG, (b - 1) // 2)
            ya = [lambda dep, c=c: y_pass_a(yprev, half_a, tb, c, dep) for c in _CLASSES]
            yb = [lambda dep, i2=i2: y_pass_b(par == 0, ct, g_b, 1 - tb, 1 - tb, i2, dep) for i2 in range(8)]
            ty = [t for pair in zip(ya, yb) for t in pair]
            return [t for pair in zip(tw, ty) for t in pair]

        def body(i, carry):
            @pl.when(i == NF // 2 // UC - 1)
            def _():
                wait_next()
            zero = zref[...]
            outs = []
            for u in range(UC):
                b = i * UC + u
                tasks = tasks_of(b, u % 2)
                first = len(outs)
                seen = [0]

                def emit(k):
                    for v in range(k.shape[0] // 8):
                        while (len(outs) - first < len(tasks)
                               and seen[0] >= ((len(outs) - first) * 3 * NR // 8) // len(tasks)):
                            dep = _bits(k[8 * v:8 * v + 8])
                            if len(outs) >= CHAIN:
                                dep = dep | outs[-CHAIN]
                            outs.append(tasks[len(outs) - first](dep & zero))
                        seen[0] += 1
                    return k
                k1 = emit(prod(3 * b))
                yh[2 * b] = k1 - emit(prod(3 * b + 2))
                yh[2 * b + 1] = k1 + emit(prod(3 * b + 1))
            return carry

        lax_loop(0, NF // 2 // UC, body, 0)

    w_start(2)
    w_part(1, *w1_parts[0], 4).wait()
    for i2 in range(8):
        w_pass1(0, 1, 0, i2)

    def wait_tile(j, more):
        @pl.when(more)
        def _():
            w_copy(j, False).wait()

    def wait_first(jj):
        @pl.when(jj == 0)
        def _():
            w_part(1, *w1_parts[1], 5).wait()
        wait_tile(2 * jj + 2, jj + 1 < NCT)

    def tile_pair(jj, carry):
        products(0, jnp.maximum(jj - 1, 0), lambda: wait_first(jj))

        @pl.when(jj + 1 < NCT)
        def _():
            w_start(2 * jj + 3)
            w_copy(2 * jj + 2, True).wait()
        products(1, 0, lambda: wait_tile(2 * jj + 3, jj + 1 < NCT))

        @pl.when(jj + 2 < NCT)
        def _():
            w_start(2 * jj + 4)

        @pl.when(jj + 1 < NCT)
        def _():
            w_copy(2 * jj + 3, True).wait()

        @pl.when(jj == 1)
        def _():
            wo_copy.start()
        return jj

    ct_last = lax_loop(0, NCT, tile_pair, 0)

    parts = []
    for g in range(NG):
        for b in range(B):
            lo, hi = max(GR * g, PITCH * b), min(GR * (g + 1), PITCH * b + TH)
            if lo < hi:
                parts.append((g, lo, hi))
    g, lo, hi = parts.pop()
    parts += [(g, lo, hi - 88), (g, hi - 88, hi)]

    def o_copy(n):
        _, lo, hi = parts[n]
        b = lo // PITCH
        return pltpu.make_async_copy(
            ost.at[pl.ds(2 * lo, 2 * (hi - lo)), :],
            o_hbm.at[b, pl.ds(2 * (lo - PITCH * b), 2 * (hi - lo)), :], osem.at[n])

    def last_tasks(g):
        t = [lambda dep, h=h, c=c: y_pass_a(yh1, 2 * g + h, h, c, dep) for h in range(2) for c in _CLASSES]
        return t + [lambda dep, h=h, i2=i2: y_pass_b(True, ct_last, g, h, h, i2, dep)
                    for h in range(2) for i2 in range(8)]

    wo_copy.wait()
    for task in last_tasks(0):
        task(None)
    for n, (g, lo, hi) in enumerate(parts):
        z = jnp.concatenate([_bf16(xs[ct, lo:hi, :]) for ct in range(NCT)], axis=1)
        res = jnp.dot(z, wo_ref[...], preferred_element_type=jnp.float32)
        if n >= 1:
            o_copy(n - 1).start()
        ost[2 * lo:2 * hi, :] = res.astype(jnp.bfloat16)
        if g + 1 < NG and parts[n + 1][0] != g:
            rows = (hi - lo) // 4
            tiles = [res[8 * r:8 * r + 8, 128 * c:128 * c + 128] for c in range(NCT) for r in range(rows)]
            release(last_tasks(g + 1), tiles[:int(0.7 * len(tiles))])
    o_copy(len(parts) - 1).start()
    for n in range(len(parts)):
        o_copy(n).wait()


@jax.jit
def pallas_standalone__autoregressive_conv_wavenet__speech_kernel(x, w, w_o):
    coef = np.stack([np.repeat(_sub_dft(q, 16, NF) * (2.0 / NF), 8, axis=1) for q in range(4)]
                    + [np.repeat(_sub_dft(q, 8, K), 16, axis=1) for q in range(4)]).astype(np.float32)
    hbm = pl.BlockSpec(memory_space=pl.ANY)
    vmem = pl.BlockSpec(memory_space=pltpu.VMEM)
    f32, bf16, u32 = jnp.float32, jnp.bfloat16, jnp.uint32
    return pl.pallas_call(
        _kernel,
        in_specs=[hbm, hbm, hbm, vmem],
        out_specs=hbm,
        out_shape=jax.ShapeDtypeStruct((B, T, D), bf16),
        scratch_shapes=[
            pltpu.VMEM((NCT, XROWS, 128), u32),
            pltpu.VMEM((2, K, D, 128), bf16),
            pltpu.VMEM((NPROD, NCT, NR, 128), bf16),
            pltpu.VMEM((NPROD, D, 128), bf16),
            pltpu.VMEM((NPROD, D, 128), bf16),
            pltpu.VMEM((NF, NR, 128), f32),
            pltpu.VMEM((NF, NR, 128), f32),
            pltpu.VMEM((HOP, NR + 16, 128), f32),
            pltpu.VMEM((2, 2, 8, 8, 8, 128), f32),
            pltpu.VMEM((2, 8, 8, 8, 128), f32),
            pltpu.VMEM((HOP, 8, 128), f32),
            pltpu.VMEM((8, 128), u32),
            pltpu.VMEM((2 * B * PITCH, D), bf16),
            pltpu.VMEM((D, D), bf16),
            pltpu.VMEM((4, 256, 128), bf16),
            pltpu.VMEM((4, 128, 128), bf16),
            pltpu.SemaphoreType.DMA((NCT, 3, 2)),
            pltpu.SemaphoreType.DMA((2, 2)),
            pltpu.SemaphoreType.DMA((7,)),
            pltpu.SemaphoreType.DMA((NG + 2,)),
        ],
        compiler_params=pltpu.CompilerParams(vmem_limit_bytes=112 * 2**20),
    )(x, w, w_o, coef)
```

```python
import jax
import jax.numpy as jnp
import numpy as np
from jax.experimental import pallas as pl
from jax.experimental.pallas import tpu as pltpu

NF = 64
HOP = 34
NPROD = 96
B, T, D, K = 2, 4000, 512, 31
TH = T // 2
NB = 60
PITCH = NB * HOP
NG = B * NB // 8
NR = NG * 16
GR = 8 * HOP
OFF = 32
XROWS = 4392
NCT = D // 128
UC = 16
CHAIN = 2


class _V:
    def __init__(self, a, s=1):
        self.a = a
        self.s = s


_Z = _V(None)


def _add(x, y):
    if x.a is None:
        return y
    if y.a is None:
        return x
    if x.s == y.s:
        return _V(x.a + y.a, x.s)
    return _V(x.a - y.a) if x.s > 0 else _V(y.a - x.a)


def _neg(x):
    return x if x.a is None else _V(x.a, -x.s)


def _sub(x, y):
    return _add(x, _neg(y))


def _mul(x, c):
    return _Z if x.a is None else _V(x.a * float(c * x.s))


def _val(x, like=None):
    if x.a is None:
        return jnp.zeros_like(like)
    return x.a if x.s > 0 else -x.a


def _cadd(x, y):
    return (_add(x[0], y[0]), _add(x[1], y[1]))


def _csub(x, y):
    return (_sub(x[0], y[0]), _sub(x[1], y[1]))


def _conj(x):
    return (x[0], _neg(x[1]))


def _ctw(x, k, n):
    k %= n
    a, b = x
    if k == 0:
        return x
    if 4 * k == n:
        return (b, _neg(a))
    if 2 * k == n:
        return (_neg(a), _neg(b))
    if 4 * k == 3 * n:
        return (_neg(b), a)
    c, s = np.cos(2 * np.pi * k / n), -np.sin(2 * np.pi * k / n)
    if (8 * k) % n == 0:
        pa, pb = (a if c > 0 else _neg(a)), (b if c > 0 else _neg(b))
        qa, qb = (a if s > 0 else _neg(a)), (b if s > 0 else _neg(b))
        r = float(np.sqrt(0.5))
        return (_mul(_sub(pa, qb), r), _mul(_add(qa, pb), r))
    return (_sub(_mul(a, c), _mul(b, s)), _add(_mul(a, s), _mul(b, c)))


def _cdft(x):
    n = len(x)
    if n == 1:
        return list(x)
    if n == 2:
        return [_cadd(x[0], x[1]), _csub(x[0], x[1])]
    ev, o1, o3 = _cdft(x[0::2]), _cdft(x[1::4]), _cdft(x[3::4])
    out = [None] * n
    for k in range(n // 4):
        a, b = _ctw(o1[k], k, n), _ctw(o3[k], 3 * k, n)
        p, m = _cadd(a, b), _csub(a, b)
        mi = (m[1], _neg(m[0]))
        out[k], out[k + n // 2] = _cadd(ev[k], p), _csub(ev[k], p)
        out[k + n // 4], out[k + 3 * n // 4] = _cadd(ev[k + n // 4], mi), _csub(ev[k + n // 4], mi)
    return out


def _icdft(x):
    return [_conj(v) for v in _cdft([_conj(v) for v in x])]


def _rdft(x):
    n = len(x)
    if n == 2:
        return {0: (_add(x[0], x[1]), _Z), 1: (_sub(x[0], x[1]), _Z)}
    h, q = n // 2, n // 4
    s = [_add(x[i], x[i + h]) for i in range(h)]
    d = [_sub(x[i], x[i + h]) for i in range(h)]
    out = {2 * k: v for k, v in _rdft(s).items()}
    u = _cdft([_ctw((d[i], _neg(d[i + q])), i, n) for i in range(q)])
    for k in range(q):
        out[4 * k + 1] = u[k]
    return out


def _fwd_pass1(i2, a, b, c, d):
    r = float(np.sqrt(0.5))
    s1, s2, d1, d2 = _add(a, c), _add(b, d), _sub(a, c), _sub(b, d)
    t1, t2 = _mul(d2, r), _mul(s2, r)
    g1 = (_add(a, t1), _neg(_add(c, t2)))
    g2 = (d1, _neg(d2))
    g3 = (_sub(a, t1), _sub(c, t2))
    out = [_add(s1, s2), _sub(s1, s2)]
    for k, g in ((1, g1), (2, g2), (3, g3)):
        out.extend(_ctw(g, i2 * k, NF))
    return out


def _fwd_pass2(cls, v):
    if cls == 0:
        return {8 * k: x for k, x in _rdft([v(i, 0) for i in range(8)]).items()}
    if cls == 4:
        g = [v(i, 1) for i in range(8)]
        u = _cdft([_ctw((g[i], _neg(g[i + 4])), i, 16) for i in range(4)])
        return {4 + 16 * k: u[k] for k in range(4)}
    k1, odd = cls % 8, cls // 8
    x = [(v(i, 2 * k1), v(i, 2 * k1 + 1)) for i in range(8)]
    if odd:
        u = _cdft([_ctw(_csub(x[n], x[n + 4]), n, 8) for n in range(4)])
    else:
        u = _cdft([_cadd(x[n], x[n + 4]) for n in range(4)])
    return {k1 + 8 * (2 * k + odd): u[k] for k in range(4)}


_CLASSES = (1, 9, 2, 10, 3, 11, 0, 4)


def _representatives():
    rep = {}
    for cls in _CLASSES:
        for k in _fwd_pass2(cls, lambda i, j: _Z):
            rep[min(k, NF - k)] = k
    return [rep[k] for k in range(NF // 2 + 1)]


_REP = _representatives()


def _gauss_forms(kappa, re, im, is_w):
    return [re, _sub(im, re), _add(re, im)] if is_w else [_add(re, im), re, im]


def _inv_real8(g0, g4, t1, t2, t3, outs):
    r = float(np.sqrt(0.5))
    a, b = _add(g0, g4), _sub(g0, g4)
    p, s = _sub(t1[0], t3[0]), _add(t1[1], t3[1])
    base = [_add(a, t2[0]), _sub(b, t2[1]), _sub(a, t2[0]), _add(b, t2[1])]
    lazy = [lambda: _add(t1[0], t3[0]), lambda: _mul(_sub(p, s), r),
            lambda: _sub(t3[1], t1[1]), lambda: _neg(_mul(_add(s, p), r))]
    out, cache = {}, {}
    for i in outs:
        if i % 4 not in cache:
            cache[i % 4] = lazy[i % 4]()
        out[i] = _add(base[i % 4], cache[i % 4]) if i < 4 else _sub(base[i % 4], cache[i % 4])
    return out


def _inv_pass_a(cls, y):
    if cls == 0:
        (g0, _), (g4, _) = y(0), y(32)
        out = _inv_real8(g0, g4, y(8), y(16), _conj(y(40)), range(8))
        return {(i, 0): out[i] for i in range(8)}
    if cls == 4:
        s = _icdft([y(4 + 16 * k) for k in range(4)])
        out = {}
        for i in range(4):
            re, im = _conj(_ctw(_conj(s[i]), i, 16))
            out[(i, 1)], out[(i + 4, 1)] = re, _neg(im)
        return out
    k1, odd = cls % 8, cls // 8
    x = [y(k1 + 8 * k2) for k2 in range(8)]
    if odd:
        u = _icdft([_ctw(_csub(x[n], x[n + 4]), -n, 8) for n in range(4)])
    else:
        u = _icdft([_cadd(x[n], x[n + 4]) for n in range(4)])
    out = {}
    for k in range(4):
        out[(2 * k + odd, 2 * k1)], out[(2 * k + odd, 2 * k1 + 1)] = u[k]
    return out


def _inv_pass_b(i2, v):
    t = [_conj(_ctw(_conj((v[2 * k], v[2 * k + 1])), i2 * k, NF)) for k in (1, 2, 3)]
    outs = [i1 for i1 in range(8) if 8 * i1 + i2 >= NF - HOP]
    y = _inv_real8(v[0], v[1], t[0], t[1], t[2], outs)
    return {8 * i1 + i2 - (NF - HOP): y[i1] for i1 in outs}


def _radix4_bins(tq):
    t0 = [_V(tq[q][0]) for q in range(4)]
    u0, u1 = _add(t0[0], t0[2]), _sub(t0[0], t0[2])
    v0, v1 = _add(t0[1], t0[3]), _sub(t0[1], t0[3])
    out = {0: (_add(u0, v0), _Z), 32: (_sub(u0, v0), _Z), 16: (u1, _neg(v1))}
    a0, a1, b2, a3 = (_V(tq[q][1]) for q in range(4))
    s, d = _add(a1, a3), _sub(a3, a1)
    out[8] = (_add(a0, s), _add(b2, d))
    out[24] = (_sub(a0, s), _sub(d, b2))
    for kp in range(1, 8):
        t = [(_V(tq[q][2 * kp]), _V(tq[q][2 * kp + 1])) for q in range(4)]
        u0, u1 = _cadd(t[0], t[2]), _csub(t[0], t[2])
        v0, v1 = _cadd(t[1], t[3]), _csub(t[1], t[3])
        mi = (v1[1], _neg(v1[0]))
        out[kp] = _cadd(u0, v0)
        out[kp + 16] = _cadd(u1, mi)
        out[kp + 32] = _csub(u0, v0)
        out[kp + 48] = _csub(u1, mi)
    return out


def _operands(bins, is_w, like):
    r0, r32 = bins[0][0], bins[NF // 2][0]
    ops = [_Z, r32, _neg(r0)] if is_w else [_Z, _mul(r32, 0.5), _mul(r0, 0.5)]
    for kappa in range(1, NF // 2):
        k = _REP[kappa]
        re, im = bins[k] if k in bins else _conj(bins[NF - k])
        ops.extend(_gauss_forms(kappa, re, im, is_w))
    return [_val(v, like) for v in ops]


def _sub_dft(q, nm, taps):
    n = 4 * np.arange(nm) + q
    c = np.zeros((16, nm))
    c[0] = 1.0
    th = -2 * np.pi * 8 * n / NF
    c[1] = np.sin(th) if q == 2 else np.cos(th)
    for kp in range(1, 8):
        th = -2 * np.pi * kp * n / NF
        c[2 * kp], c[2 * kp + 1] = np.cos(th), np.sin(th)
    c[:, n >= taps] = 0.0
    return np.where(np.abs(c) < 1e-12, 0.0, c)


def _bf16(words):
    return pltpu.bitcast(words, jnp.bfloat16)


def _bits(v):
    return pltpu.bitcast(v, jnp.uint32)


def _after(v, dep):
    return v if dep is None else pltpu.bitcast(_bits(v) | dep, jnp.float32)


def _kernel(x_hbm, w_hbm, wo_hbm, coef_ref, o_hbm,
            xs, wbuf, xh, wh0, wh1, yh0, yh1, tf, wtmp, ytmp, ztmp, zref, ost, wo_ref, lw_bf, lx_bf,
            xsem, wsem, psem, osem):
    whs = (wh0, wh1)
    xs_bf = xs.bitcast(jnp.bfloat16)
    wv = wbuf.bitcast(jnp.uint32)
    lw_ref, lx_ref = lw_bf.bitcast(jnp.uint32), lx_bf.bitcast(jnp.uint32)

    x_parts = (((0, 0, 1440),), ((0, 1440, TH), (1, 0, 720)), ((1, 720, TH),))

    def x_copies(ct, k):
        return [pltpu.make_async_copy(
            x_hbm.at[b, pl.ds(2 * lo, 2 * (hi - lo)), pl.ds(pl.multiple_of(ct * 128, 128), 128)],
            xs_bf.at[ct, pl.ds(2 * (OFF + b * PITCH + lo), 2 * (hi - lo)), :],
            xsem.at[ct, k, n]) for n, (b, lo, hi) in enumerate(x_parts[k])]

    def col_of(j):
        return (j % 2) * D + (j // 2) * 128

    def w_copy(j, rest):
        lo, n = (16, D - 16) if rest else (0, 16)
        return pltpu.make_async_copy(
            w_hbm.at[:, pl.ds(lo, n), pl.ds(pl.multiple_of(col_of(j), 128), 128)],
            wbuf.at[j % 2, :, pl.ds(lo, n), :], wsem.at[j % 2, int(rest)])

    def w_start(j):
        w_copy(j, False).start()
        w_copy(j, True).start()

    def w_part(j, lo, n, k):
        return pltpu.make_async_copy(
            w_hbm.at[:, pl.ds(lo, n), pl.ds(col_of(j), 128)], wbuf.at[j % 2, :, pl.ds(lo, n), :], psem.at[k])

    w1_parts = ((0, 144), (144, 128), (272, 128), (400, 112))
    wo_copy = pltpu.make_async_copy(wo_hbm, wo_ref, psem.at[8])

    for ct in range(NCT):
        for k in range(3):
            for c in x_copies(ct, k):
                c.start()
    for k in range(4):
        w_part(0, 128 * k, 128, k).start()
    for k, (lo, n) in enumerate(w1_parts):
        w_part(1, lo, n, 4 + k).start()

    for first, rep, dst in ((0, 8, lx_bf), (4, 16, lw_bf)):
        shape = (16 * rep, 128)
        diag = (jax.lax.broadcasted_iota(jnp.int32, shape, 0) % rep
                == jax.lax.broadcasted_iota(jnp.int32, shape, 1) % rep)
        for q in range(4):
            c = coef_ref[first + q]
            full = jnp.concatenate([jnp.broadcast_to(c[j:j + 1], (rep, 128)) for j in range(16)], axis=0)
            dst[q] = jnp.where(diag, full, 0.0).astype(jnp.bfloat16)

    for ct in range(NCT):
        xs[ct, 0:OFF, :] = jnp.zeros((OFF, 128), jnp.uint32)
        for b in range(B):
            lo = OFF + b * PITCH + TH
            hi = OFF + (b + 1) * PITCH + (16 if b == B - 1 else 0)
            xs[ct, lo:hi, :] = jnp.zeros((hi - lo, 128), jnp.uint32)
    wh0[0] = jnp.zeros((D, 128), jnp.bfloat16)
    wh1[0] = jnp.zeros((D, 128), jnp.bfloat16)
    zref[...] = jnp.zeros((8, 128), jnp.uint32)
    ytmp[...] = jnp.zeros(ytmp.shape, jnp.float32)
    ztmp[...] = jnp.zeros(ztmp.shape, jnp.float32)

    def x_group(ct, g):
        base = g * GR + (OFF - (K - 1))
        tq = []
        for q in range(4):
            rows = [_bf16(xs[ct, pl.ds(base + 4 * m + q, 8, stride=HOP), :]).astype(jnp.float32)
                    for m in range(16)]
            res = []
            for h in range(2):
                rhs = jnp.concatenate([v[8 * h:8 * h + 8] for v in rows], axis=0).astype(jnp.bfloat16)
                res.append(jnp.dot(_bf16(lx_ref[q]), rhs, preferred_element_type=jnp.float32))
            tq.append([jnp.concatenate([r[8 * j:8 * j + 8] for r in res], axis=0) for j in range(16)])
        ops = _operands(_radix4_bins(tq), False, tq[0][0])
        r0 = pl.multiple_of(g * 16, 16)
        for p in range(NPROD):
            xh[p, ct, pl.ds(r0, 16), :] = ops[p].astype(jnp.bfloat16)

    NG3 = NG // 3

    def x_step(i, carry):
        ct, k = i // 3, i % 3
        for kk in range(3):
            @pl.when(k == kk)
            def _():
                for c in x_copies(ct, kk):
                    c.wait()
        for gi in range(NG3):
            x_group(ct, k * NG3 + gi)
        return carry

    jax.lax.fori_loop(0, 3 * NCT, x_step, 0)

    def w_group_mxu(cg):
        r0 = pl.multiple_of(cg * 8, 8)
        tq = []
        for q in range(4):
            rhs = _bf16(jnp.concatenate(
                [wv[0, min(4 * m + q, K - 1), pl.ds(r0, 8), :] for m in range(8)], axis=0))
            res = jnp.dot(_bf16(lw_ref[q]), rhs, preferred_element_type=jnp.float32)
            tq.append([res[16 * j:16 * j + 16] for j in range(16)])
        ops = _operands(_radix4_bins(tq), True, tq[0][0])
        r1 = pl.multiple_of(cg * 16, 16)
        for p in range(NPROD):
            wh0[p, pl.ds(r1, 16), :] = ops[p].astype(jnp.bfloat16)

    def w_step_mxu(k, carry):
        w_part(0, pl.multiple_of(k * 128, 128), 128, k).wait()
        for cg in range(8):
            w_group_mxu(k * 8 + cg)
        return carry

    jax.lax.fori_loop(0, 4, w_step_mxu, 0)

    def w_pass1(cg, src, tb, i2, dep=None):
        r0 = pl.multiple_of(cg * 8, 8)
        words = [wv[src, i, pl.ds(r0, 8), :] if i < K else None for i in range(i2, 32, 8)]
        rows = [None if v is None else _bf16(v if dep is None else v | dep).astype(jnp.float32)
                for v in words]
        for h in range(2):
            vals = _fwd_pass1(i2, *[_Z if v is None else _V(v[8 * h:8 * h + 8]) for v in rows])
            for j in range(8):
                last = _val(vals[j])
                wtmp[tb, h, i2, j] = last
        return _bits(last)

    def w_pass2(cg, whn, tb, cls, dep=None):
        forms = []
        for h in range(2):
            bins = _fwd_pass2(cls, lambda i, j: _V(_after(wtmp[tb, h, i, j], dep if i < 4 else None)))
            fh = {}
            for kappa in range(NF // 2 + 1):
                if _REP[kappa] in bins:
                    re, im = bins[_REP[kappa]]
                    if kappa == 0:
                        fh[2] = _val(_neg(re))
                    elif kappa == NF // 2:
                        fh[1] = _val(re)
                    else:
                        for n, v in enumerate(_gauss_forms(kappa, re, im, True)):
                            fh[3 * kappa + n] = _val(v)
            forms.append(fh)
        r1 = pl.multiple_of(cg * 16, 16)
        for p in forms[0]:
            whn[p, pl.ds(r1, 16), :] = jnp.concatenate([forms[0][p], forms[1][p]], axis=0).astype(jnp.bfloat16)
        return _bits(forms[1][p])

    def y_pass_a(yh, half, tb, cls, dep=None):
        r0 = pl.multiple_of(half * 8, 8)

        def y(k):
            d = dep if k < NF // 2 and (cls % 8 != 0 or k < 20) else None
            if k % (NF // 2) == 0:
                return (_V(_after(yh[k // 32, pl.ds(r0, 8), :], d)), _Z)
            kappa = _REP.index(k)
            return (_V(_after(yh[2 * kappa, pl.ds(r0, 8), :], d)),
                    _V(_after(yh[2 * kappa + 1, pl.ds(r0, 8), :], d)))
        for (i2, j), v in _inv_pass_a(cls, y).items():
            last = _val(v)
            ytmp[tb, i2, j] = last
        return _bits(last)

    def y_pass_b(is_gate, ct, g, h, tb, i2, dep=None):
        r0 = pl.multiple_of(g * 16 + 8 * h, 8)
        v = [_V(_after(ytmp[tb, i2, j], dep if j >= 2 else None)) for j in range(8)]
        for t, hv in _inv_pass_b(i2, v).items():
            if not is_gate:
                z = 0.5 * jnp.tanh(_val(hv))
                tf[t, pl.ds(r0, 8), :] = z
                continue
            hf = tf[t, pl.ds(r0, 8), :]
            z = hf + hf * jnp.tanh(_val(_mul(hv, 0.5)))
            if h == 0:
                ztmp[t] = z
            else:
                both = jnp.concatenate([ztmp[t], z], axis=0).astype(jnp.bfloat16)
                xs[ct, pl.ds(g * GR + t, 8, stride=HOP), :] = _bits(both)
        return _bits(z)

    def release(tasks, results):
        zero = zref[...]
        outs = []
        for n, task in enumerate(tasks):
            dep = _bits(results[(n * len(results)) // len(tasks)])
            if n >= CHAIN:
                dep = dep | outs[n - CHAIN]
            outs.append(task(dep & zero))
        return outs

    def bin_products(prod, yh, b, rows, tasks, outs, zero):
        first, seen = len(outs), [0]
        total = 3 * rows.size // 8

        def emit(k):
            for v in range(k.shape[0] // 8):
                while len(outs) - first < len(tasks) and seen[0] >= ((len(outs) - first) * total) // len(tasks):
                    dep = _bits(k[8 * v:8 * v + 8])
                    if len(outs) >= CHAIN:
                        dep = dep | outs[-CHAIN]
                    outs.append(tasks[len(outs) - first](dep & zero))
                seen[0] += 1
            return k
        k1 = emit(prod(3 * b))
        yh[2 * b, rows, :] = k1 - emit(prod(3 * b + 2))
        yh[2 * b + 1, rows, :] = k1 + emit(prod(3 * b + 1))

    def products(par, ct, wait_next):
        xhu = xh.bitcast(jnp.uint32)
        whc = whs[par].bitcast(jnp.uint32)
        whn, src = whs[1 - par], 1 - par
        yh, yprev = (yh0, yh1) if par == 0 else (yh1, yh0)

        def prod(p):
            lhs = jnp.concatenate([_bf16(xhu[p, ct_]) for ct_ in range(NCT)], axis=1)
            return jnp.dot(lhs, _bf16(whc[p]), preferred_element_type=jnp.float32)

        def tasks_of(b, tb):
            t2 = [lambda dep, c=c: w_pass2(b, whn, tb, c, dep) for c in _CLASSES]
            src1 = jnp.where(b == NF // 2 - 1, 1 - src, src)
            t1 = [lambda dep, i2=i2: w_pass1((b + 1) % (NF // 2), src1, 1 - tb, i2, dep) for i2 in range(8)]
            tw = [t for pair in zip(t2, t1) for t in pair]
            half_a = jnp.minimum(b, 2 * NG - 1)
            g_b = jnp.where(b == 0, NG, (b - 1) // 2)
            ya = [lambda dep, c=c: y_pass_a(yprev, half_a, tb, c, dep) for c in _CLASSES]
            yb = [lambda dep, i2=i2: y_pass_b(par == 0, ct, g_b, 1 - tb, 1 - tb, i2, dep) for i2 in range(8)]
            ty = [t for pair in zip(ya, yb) for t in pair]
            return [t for pair in zip(tw, ty) for t in pair]

        def body(i, carry):
            @pl.when(i == NF // 2 // UC - 1)
            def _():
                wait_next()
            zero = zref[...]
            outs = []
            for u in range(UC):
                b = i * UC + u
                bin_products(prod, yh, b, pl.ds(0, NR), tasks_of(b, u % 2), outs, zero)
            return carry

        jax.lax.fori_loop(0, NF // 2 // UC, body, 0)

    def first_products():
        xhu, whc = xh.bitcast(jnp.uint32), wh0.bitcast(jnp.uint32)

        def prod(p):
            lhs = jnp.concatenate([_bf16(xhu[p, ct_]) for ct_ in range(NCT)], axis=1)
            return jnp.dot(lhs, _bf16(whc[p]), preferred_element_type=jnp.float32)

        def tasks_of(b, tb):
            t2 = [lambda dep, c=c: w_pass2(b, wh1, tb, c, dep) for c in _CLASSES]
            src1 = jnp.where(b == NF // 2 - 1, 0, 1)
            t1 = [lambda dep, i2=i2: w_pass1((b + 1) % (NF // 2), src1, 1 - tb, i2, dep) for i2 in range(8)]
            return [t for pair in zip(t2, t1) for t in pair]

        def body(i, carry):
            for k in range(1, 4):
                @pl.when(i == k)
                def _():
                    w_part(1, *w1_parts[k], 4 + k).wait()
                    if k == 3:
                        w_copy(2, False).wait()
            zero = zref[...]
            outs = []
            for u in range(8):
                b = i * 8 + u
                bin_products(prod, yh0, b, pl.ds(0, NR), tasks_of(b, u % 2), outs, zero)
            return carry

        jax.lax.fori_loop(0, 4, body, 0)

    w_start(2)
    w_part(1, *w1_parts[0], 4).wait()
    for i2 in range(8):
        w_pass1(0, 1, 0, i2)
    first_products()

    def wait_tile(j, more):
        @pl.when(more)
        def _():
            w_copy(j, False).wait()

    def tile_pair(jj, carry):
        @pl.when(jj > 0)
        def _():
            products(0, jnp.maximum(jj - 1, 0), lambda: wait_tile(2 * jj + 2, jj + 1 < NCT))

        @pl.when(jj + 1 < NCT)
        def _():
            w_start(2 * jj + 3)
            w_copy(2 * jj + 2, True).wait()
        products(1, 0, lambda: wait_tile(2 * jj + 3, jj + 1 < NCT))

        @pl.when(jj + 2 < NCT)
        def _():
            w_start(2 * jj + 4)

        @pl.when(jj + 1 < NCT)
        def _():
            w_copy(2 * jj + 3, True).wait()

        @pl.when(jj == 1)
        def _():
            wo_copy.start()
        return jj

    ct_last = jax.lax.fori_loop(0, NCT, tile_pair, 0)

    parts = []
    for g in range(NG):
        for b in range(B):
            lo, hi = max(GR * g, PITCH * b), min(GR * (g + 1), PITCH * b + TH)
            if lo < hi:
                parts.append((g, lo, hi))
    g, lo, hi = parts.pop()
    parts += [(g, lo, hi - 88), (g, hi - 88, hi)]

    def o_copy(n):
        _, lo, hi = parts[n]
        b = lo // PITCH
        return pltpu.make_async_copy(
            ost.at[pl.ds(2 * lo, 2 * (hi - lo)), :],
            o_hbm.at[b, pl.ds(2 * (lo - PITCH * b), 2 * (hi - lo)), :], osem.at[n])

    def last_tasks(g):
        t = [lambda dep, h=h, c=c: y_pass_a(yh1, 2 * g + h, h, c, dep) for h in range(2) for c in _CLASSES]
        return t + [lambda dep, h=h, i2=i2: y_pass_b(True, ct_last, g, h, h, i2, dep)
                    for h in range(2) for i2 in range(8)]

    wo_copy.wait()
    for task in last_tasks(0):
        task(None)
    for n, (g, lo, hi) in enumerate(parts):
        z = jnp.concatenate([_bf16(xs[ct, lo:hi, :]) for ct in range(NCT)], axis=1)
        res = jnp.dot(z, wo_ref[...], preferred_element_type=jnp.float32)
        if n >= 1:
            o_copy(n - 1).start()
        ost[2 * lo:2 * hi, :] = res.astype(jnp.bfloat16)
        if g + 1 < NG and parts[n + 1][0] != g:
            rows = (hi - lo) // 4
            tiles = [res[8 * r:8 * r + 8, 128 * c:128 * c + 128] for c in range(NCT) for r in range(rows)]
            release(last_tasks(g + 1), tiles[:int(0.7 * len(tiles))])
    o_copy(len(parts) - 1).start()
    for n in range(len(parts)):
        o_copy(n).wait()


@jax.jit
def pallas_standalone__autoregressive_conv_wavenet__speech_kernel(x, w, w_o):
    coef = np.stack([np.repeat(_sub_dft(q, 16, NF) * (2.0 / NF), 8, axis=1) for q in range(4)]
                    + [np.repeat(_sub_dft(q, 8, K), 16, axis=1) for q in range(4)]).astype(np.float32)
    hbm = pl.BlockSpec(memory_space=pl.ANY)
    vmem = pl.BlockSpec(memory_space=pltpu.VMEM)
    f32, bf16, u32 = jnp.float32, jnp.bfloat16, jnp.uint32
    return pl.pallas_call(
        _kernel,
        in_specs=[hbm, hbm, hbm, vmem],
        out_specs=hbm,
        out_shape=jax.ShapeDtypeStruct((B, T, D), bf16),
        scratch_shapes=[
            pltpu.VMEM((NCT, XROWS, 128), u32),
            pltpu.VMEM((2, K, D, 128), bf16),
            pltpu.VMEM((NPROD, NCT, NR, 128), bf16),
            pltpu.VMEM((NPROD, D, 128), bf16),
            pltpu.VMEM((NPROD, D, 128), bf16),
            pltpu.VMEM((NF, NR, 128), f32),
            pltpu.VMEM((NF, NR, 128), f32),
            pltpu.VMEM((HOP, NR + 16, 128), f32),
            pltpu.VMEM((2, 2, 8, 8, 8, 128), f32),
            pltpu.VMEM((2, 8, 8, 8, 128), f32),
            pltpu.VMEM((HOP, 8, 128), f32),
            pltpu.VMEM((8, 128), u32),
            pltpu.VMEM((2 * B * PITCH, D), bf16),
            pltpu.VMEM((D, D), bf16),
            pltpu.VMEM((4, 256, 128), bf16),
            pltpu.VMEM((4, 128, 128), bf16),
            pltpu.SemaphoreType.DMA((NCT, 3, 2)),
            pltpu.SemaphoreType.DMA((2, 2)),
            pltpu.SemaphoreType.DMA((9,)),
            pltpu.SemaphoreType.DMA((NG + 2,)),
        ],
        compiler_params=pltpu.CompilerParams(vmem_limit_bytes=112 * 2**20),
    )(x, w, w_o, coef)
```
